```python
import jax
import jax.numpy as jnp

def _softmax(x, axis=-1):
    return jax.nn.softmax(x, axis=axis)

def _gelu(x):
    return jax.nn.gelu(x, approximate=True)

def _silu(x):
    return jax.nn.silu(x)

def _sigmoid(x):
    return jax.nn.sigmoid(x)

def _layernorm(x, axis=-1, eps=1e-05):
    m = jnp.mean(x, axis=axis, keepdims=True)
    v = jnp.var(x, axis=axis, keepdims=True)
    return (x - m) / jnp.sqrt(v + eps)

def _scatter_add(tgt, idx, src, axis=0):
    return tgt.at[idx].add(src)

def _segment_sum(src, seg, n):
    return jax.ops.segment_sum(src, seg, n)

class _Rng:

    def __init__(self, key):
        self._k = key

    def _next(self):
        self._k, sub = jax.random.split(self._k)
        return sub

    def normal(self, shape):
        return jax.random.normal(self._next(), shape, dtype=jnp.bfloat16)

    def randint(self, lo, hi, shape):
        return jax.random.randint(self._next(), shape, lo, hi, dtype=jnp.int32)

    def uniform(self, shape, lo=0.0, hi=1.0):
        return jax.random.uniform(self._next(), shape, jnp.bfloat16, lo, hi)

    def permutation(self, n):
        return jax.random.permutation(self._next(), n)
kernel_name = 'adaLN_cond__ssm_conv_h3__dense_activation_gelu__prompt'

def setup_inputs():
    _rng = _Rng(jax.random.key(int.from_bytes(__import__("os").urandom(4), "little")))
    _w = lambda a: (lambda t: t.astype(jnp.bfloat16) if jnp.issubdtype(t.dtype, jnp.floating) else t)(jnp.asarray(a))

    def _A_setup():
        B, S, D = (1, 2048, 640)
        ks = 4
        return {'q': _w((lambda *s: _rng.normal(s) * 0.05)(B, S, D)), 'k': _w((lambda *s: _rng.normal(s) * 0.05)(B, S, D)), 'v': _w((lambda *s: _rng.normal(s) * 0.05)(B, S, D)), 'shift_k': _w((lambda *s: _rng.normal(s) * 0.05)(D, ks) * 0.5), 'ssm_k': _w((lambda *s: _rng.normal(s) * 0.05)(D, S) * (1.0 / S ** 0.5)), 'ssm_D': _w((lambda *s: _rng.normal(s) * 0.05)(D))}
    _A_in = _A_setup()

    def _B_setup():
        B, S, D, F = (1, 2048, 640, 1728)
        return {'x': _w((lambda *s: _rng.normal(s) * 0.05)(B, S, D)), 'w1': _w((lambda *s: _rng.normal(s) * 0.05)(D, F) * D ** (-0.5)), 'b1': _w((lambda *s: _rng.normal(s) * 0.05)(F) * 0.01), 'w2': _w((lambda *s: _rng.normal(s) * 0.05)(F, D) * F ** (-0.5)), 'b2': _w((lambda *s: _rng.normal(s) * 0.05)(D) * 0.01)}
    _B_in = _B_setup()
    return {'A_q': _A_in['q'], 'A_k': _A_in['k'], 'A_v': _A_in['v'], 'A_shift_k': _A_in['shift_k'], 'A_ssm_k': _A_in['ssm_k'], 'A_ssm_D': _A_in['ssm_D'], 'B_x': _B_in['x'], 'B_w1': _B_in['w1'], 'B_b1': _B_in['b1'], 'B_w2': _B_in['w2'], 'B_b2': _B_in['b2'], 'c': _w((lambda *s: _rng.normal(s) * 0.05)(1, 640)), 'w_mod': _w((lambda *s: _rng.normal(s) * 0.05)(640, 6 * 640) * 640 ** (-0.5))}

def reference(A_q, A_k, A_v, A_shift_k, A_ssm_k, A_ssm_D, B_x, B_w1, B_b1, B_w2, B_b2, c, w_mod):

    def _A_ref(q, k, v, shift_k, ssm_k, ssm_D):
        B, S, D = q.shape
        ks = shift_k.shape[-1]
        k_pad = jnp.pad(k, ((0, 0), (ks - 1, 0), (0, 0)))
        k_shift = jnp.zeros_like(k)
        for t in range(ks):
            k_shift = k_shift + k_pad[:, t:t + S, :] * shift_k[:, ks - 1 - t][None, None, :]
        kv = k_shift * v
        L = 2 * S
        kv_pad = jnp.pad(kv, ((0, 0), (0, S), (0, 0)))
        kf_pad = jnp.pad(ssm_k, ((0, 0), (0, S)))
        kv_f = (lambda x, axes=(-2, -1): jnp.fft.rfft2(x.astype(jnp.float32), axes=axes))(kv_pad[:, None, :, :], axes=(1, 2))
        kf_f = (lambda x, axes=(-2, -1): jnp.fft.rfft2(x.astype(jnp.float32), axes=axes))(kf_pad[:, None, :], axes=(1, 2))
        kf_f = (lambda x, *d: x.transpose(*d))(kf_f, 1, 2, 0)
        y_f = kv_f * kf_f[None, :, :, :]
        y = (lambda x, s, axes=(-2, -1): jnp.fft.irfft2(x, s=s, axes=axes).astype(jnp.bfloat16))(y_f, (1, L), axes=(1, 2))[:, 0, :S, :]
        y = y + kv * ssm_D[None, None, :]
        return q * y

    def _B_ref(x, w1, b1, w2, b2):
        h = jnp.einsum('bsd,df->bsf', x, w1) + b1
        h = _gelu(h)
        return jnp.einsum('bsf,fd->bsd', h, w2) + b2
    x = A_q
    mod = (_silu(c) @ w_mod).reshape(c.shape[0], 6, 1, -1)
    sa, ca, ga, sb, cb, gb = (mod[:, 0].copy(), mod[:, 1].copy(), mod[:, 2].copy(), mod[:, 3].copy(), mod[:, 4].copy(), mod[:, 5].copy())
    h = _layernorm(x, axis=-1) * (1 + ca) + sa
    x = x + ga * _A_ref(h, A_k, A_v, A_shift_k, A_ssm_k, A_ssm_D)
    h = _layernorm(x, axis=-1) * (1 + cb) + sb
    x = x + gb * _B_ref(h, B_w1, B_b1, B_w2, B_b2)
    return x
```

```python
import numpy as np
import jax
import jax.numpy as jnp
from jax import lax
import jax.experimental.pallas as pl
import jax.experimental.pallas.tpu as pltpu

S = 2048
D = 640
F = 1728
BLK = 128
NB = S // BLK
NL = D // 128
TM = 256
EPS = 1e-5
BF = jnp.bfloat16
F32 = jnp.float32


def _dft_mats():
    n = 2 * BLK
    ks = np.concatenate([np.arange(0, BLK, 2), np.arange(1, BLK, 2)])
    t = np.arange(BLK)
    ang = 2.0 * np.pi * (ks[:, None] + 0.5) * t[None, :] / n
    fwd = np.concatenate([np.cos(ang), -np.sin(ang)], axis=0)
    c = (2.0 / n) * np.cos(ang).T
    s = -(2.0 / n) * np.sin(ang).T
    inv = np.zeros((BLK, n))
    for g in range(BLK // 8):
        inv[:, 16 * g:16 * g + 8] = c[:, 8 * g:8 * g + 8]
        inv[:, 16 * g + 8:16 * g + 16] = s[:, 8 * g:8 * g + 8]
    return fwd.astype(np.float32), inv.astype(np.float32)


def _ln(x):
    m = jnp.mean(x, axis=-1, keepdims=True)
    xc = x - m
    v = jnp.mean(xc * xc, axis=-1, keepdims=True)
    return xc * lax.rsqrt(v + EPS)


def _gelu(x):
    c0 = 0.7978845608028654
    u = x * (c0 + (c0 * 0.044715) * (x * x))
    hx = 0.5 * x
    return hx + hx * jnp.tanh(u)


def _kernel(q_hbm, k_hbm, v_hbm, sh_ref, h_hbm, dvec_ref, w1_hbm, b1_ref, w2_hbm,
            b2_ref, c_ref, wm_hbm, fwd_ref, inv_ref, o_hbm,
            qb, kb, vb, hb, wmb, w1b, w2b, ob, kf, x3, h3, hp, yf, yb, modb,
            sem_kv, sem_h, sem_w, sem_o):
    def k_cp(j):
        return pltpu.make_async_copy(k_hbm.at[0, pl.ds(BLK * j, BLK)],
                                     kb.at[pl.ds(BLK * j, BLK)], sem_kv.at[2 * j])

    def v_cp(j):
        return pltpu.make_async_copy(v_hbm.at[0, pl.ds(BLK * j, BLK)],
                                     vb.at[pl.ds(BLK * j, BLK)], sem_kv.at[2 * j + 1])

    def h_cp(j):
        return pltpu.make_async_copy(h_hbm.at[:, pl.ds(BLK * j, BLK)],
                                     hb.at[j], sem_h.at[j])

    wm_cp = pltpu.make_async_copy(wm_hbm, wmb, sem_w.at[0])
    q_cp = pltpu.make_async_copy(q_hbm.at[0], qb, sem_w.at[1])
    w1_cp = pltpu.make_async_copy(w1_hbm, w1b, sem_w.at[2])
    w2_cp = pltpu.make_async_copy(w2_hbm, w2b, sem_w.at[3])

    for j in range(NB):
        k_cp(j).start()
        v_cp(j).start()
        h_cp(j).start()
    wm_cp.start()
    w1_cp.start()
    q_cp.start()
    w2_cp.start()

    sh = sh_ref[...].astype(F32)
    dvec = dvec_ref[...].astype(F32).reshape(1, D)
    kf[0:8, :] = jnp.zeros((8, D), F32)
    hp[...] = jnp.zeros_like(hp)

    def fwd_block(j, carry):
        r0 = pl.multiple_of(j * BLK, BLK)
        k_cp(j).wait()
        v_cp(j).wait()
        kf[8:8 + BLK, :] = kb[pl.ds(r0, BLK), :].astype(F32)
        ks = kf[8:8 + BLK, :] * sh[0:1, :]
        for t in range(1, 4):
            ks = ks + kf[8 - t:8 - t + BLK, :] * sh[t:t + 1, :]
        kv = (ks * vb[pl.ds(r0, BLK), :].astype(F32)).astype(BF)
        kf[0:8, :] = kf[BLK:BLK + 8, :]
        xf = jnp.dot(fwd_ref[...], kv, preferred_element_type=F32)
        xr = xf[:BLK]
        xi = xf[BLK:]
        x3[j, 0] = xr + xi
        x3[j, 1] = xr
        x3[j, 2] = xi

        h_cp(j).wait()
        hf = lax.dot_general(fwd_ref[...], hb[j], (((1,), (1,)), ((), ())),
                             preferred_element_type=F32)
        hr = hf[:BLK]
        hi = hf[BLK:]
        pr = hp[0]
        pi = hp[1]
        half = BLK // 2
        cr = jnp.concatenate([hr[:half] - pi[:half], hr[half:] + pi[half:]], axis=0)
        ci = jnp.concatenate([hi[:half] + pr[:half], hi[half:] - pr[half:]], axis=0)
        cr = cr + jnp.where(j == 0, dvec, 0.0)
        hp[0] = hr
        hp[1] = hi
        h3[j, 0] = cr
        h3[j, 1] = ci - cr
        h3[j, 2] = cr + ci
        return carry

    with jax.named_scope("fwd"):
        lax.fori_loop(0, NB, fwd_block, 0)

    def mac_group(g, carry):
        r0 = pl.multiple_of(g * 8, 8)
        y0 = pl.multiple_of(g * 16, 16)
        for l in range(NL):
            ls = slice(128 * l, 128 * (l + 1))
            for a0 in range(0, NB, 4):
                acc = [[None] * 3 for _ in range(4)]
                for m in range(a0 + 4):
                    hm = [h3[m, c, pl.ds(r0, 8), ls] for c in range(3)]
                    for da in range(4):
                        jx = a0 + da - m
                        if jx < 0:
                            continue
                        for c in range(3):
                            p = x3[jx, c, pl.ds(r0, 8), ls] * hm[c]
                            acc[da][c] = p if acc[da][c] is None else acc[da][c] + p
                for da in range(4):
                    s1, s2, s3 = acc[da]
                    yf[a0 + da, pl.ds(y0, 16), ls] = jnp.concatenate(
                        [s1 - s3, s1 + s2], axis=0).astype(BF)
        return carry

    with jax.named_scope("mac"):
        lax.fori_loop(0, BLK // 8, mac_group, 0)

    def inv_block(j, carry):
        r0 = pl.multiple_of(j * BLK, BLK)
        yb[pl.ds(r0, BLK), :] = jnp.dot(inv_ref[...], yf[j], preferred_element_type=F32)
        return carry

    with jax.named_scope("inv"):
        lax.fori_loop(0, NB, inv_block, 0)

    with jax.named_scope("mod"):
        wm_cp.wait()
        c = c_ref[...].astype(F32)
        sc = (c * jax.nn.sigmoid(c)).astype(BF)
        modb[...] = jnp.dot(jnp.broadcast_to(sc, (16, D)), wmb[...],
                            preferred_element_type=F32)[0:8]
        w1_cp.wait()
        q_cp.wait()
        w2_cp.wait()

    b1 = b1_ref[...].astype(F32).reshape(1, F)
    b2 = b2_ref[...].astype(F32).reshape(1, D)

    def o_cp(i):
        r0 = pl.multiple_of(i * TM, TM)
        return pltpu.make_async_copy(ob.at[pl.ds(r0, TM)], o_hbm.at[0, pl.ds(r0, TM)],
                                     sem_o.at[i])

    def mlp_step(i, carry):
        r0 = pl.multiple_of(i * TM, TM)
        sa = modb[0:1, 0 * D:1 * D]
        ca = modb[0:1, 1 * D:2 * D]
        ga = modb[0:1, 2 * D:3 * D]
        sb = modb[0:1, 3 * D:4 * D]
        cb = modb[0:1, 4 * D:5 * D]
        gb = modb[0:1, 5 * D:6 * D]
        x = qb[pl.ds(r0, TM), :].astype(F32)
        h = _ln(x) * (1.0 + ca) + sa
        x1 = x + ga * (h * yb[pl.ds(r0, TM), :])
        h2 = (_ln(x1) * (1.0 + cb) + sb).astype(BF)
        g = lax.dot_general(h2, w1b[...], (((1,), (1,)), ((), ())),
                            preferred_element_type=F32) + b1
        g = _gelu(g).astype(BF)
        o = jnp.dot(g, w2b[...], preferred_element_type=F32) + b2
        ob[pl.ds(r0, TM), :] = (x1 + gb * o).astype(BF)
        o_cp(i).start()
        return carry

    with jax.named_scope("mlp"):
        lax.fori_loop(0, S // TM, mlp_step, 0)
    for i in range(S // TM):
        o_cp(i).wait()


@jax.jit
def pallas_adaLN_cond__ssm_conv_h3__dense_activation_gelu__prompt_kernel(
    A_q: jax.Array,
    A_k: jax.Array,
    A_v: jax.Array,
    A_shift_k: jax.Array,
    A_ssm_k: jax.Array,
    A_ssm_D: jax.Array,
    B_x: jax.Array,
    B_w1: jax.Array,
    B_b1: jax.Array,
    B_w2: jax.Array,
    B_b2: jax.Array,
    c: jax.Array,
    w_mod: jax.Array,
):
    del B_x
    fwd, inv = _dft_mats()
    fwd = jnp.asarray(fwd, dtype=BF)
    inv = jnp.asarray(inv, dtype=BF)
    any_spec = pl.BlockSpec(memory_space=pl.ANY)
    vmem_spec = pl.BlockSpec(memory_space=pltpu.VMEM)
    in_specs = [any_spec, any_spec, any_spec, vmem_spec, any_spec, vmem_spec, any_spec,
                vmem_spec, any_spec, vmem_spec, vmem_spec, any_spec, vmem_spec, vmem_spec]
    scratch = [
        pltpu.VMEM((S, D), BF),
        pltpu.VMEM((S, D), BF),
        pltpu.VMEM((S, D), BF),
        pltpu.VMEM((NB, D, BLK), BF),
        pltpu.VMEM((D, 6 * D), BF),
        pltpu.VMEM((F, D), BF),
        pltpu.VMEM((F, D), BF),
        pltpu.VMEM((S, D), BF),
        pltpu.VMEM((BLK + 8, D), F32),
        pltpu.VMEM((NB, 3, BLK, D), F32),
        pltpu.VMEM((NB, 3, BLK, D), F32),
        pltpu.VMEM((2, BLK, D), F32),
        pltpu.VMEM((NB, 2 * BLK, D), BF),
        pltpu.VMEM((S, D), F32),
        pltpu.VMEM((8, 6 * D), F32),
        pltpu.SemaphoreType.DMA((2 * NB,)),
        pltpu.SemaphoreType.DMA((NB,)),
        pltpu.SemaphoreType.DMA((4,)),
        pltpu.SemaphoreType.DMA((S // TM,)),
    ]
    return pl.pallas_call(
        _kernel,
        in_specs=in_specs,
        out_specs=any_spec,
        out_shape=jax.ShapeDtypeStruct((1, S, D), BF),
        scratch_shapes=scratch,
        compiler_params=pltpu.CompilerParams(vmem_limit_bytes=100 * 1024 * 1024),
    )(A_q, A_k, A_v, A_shift_k.T, A_ssm_k, A_ssm_D, B_w1.T, B_b1, B_w2, B_b2, c, w_mod,
      fwd, inv)
```

```python
LINK = 2
NACC = 2
HOPS = 8
NOMAC = 0
import numpy as np
import jax
import jax.numpy as jnp
from jax import lax
import jax.experimental.pallas as pl
import jax.experimental.pallas.tpu as pltpu

S = 2048
D = 640
F = 1728
BLK = 128
NB = S // BLK
NG = BLK // 8
NL = D // 128
TM = 256
NS = S // TM
EPS = 1e-5
BF = jnp.bfloat16
F32 = jnp.float32
U32 = jnp.uint32


def _pack_rows(a):
    u = np.ascontiguousarray(a, dtype=np.float32).view(np.uint32)
    u = (u + 0x7FFF + ((u >> 16) & 1)) >> 16
    return (u[0::2] | (u[1::2] << 16)).astype(np.uint32)


def _dft_mats():
    n = 2 * BLK
    th = 2.0 * np.arange(BLK) + 0.5
    t = np.arange(BLK)
    ang = 2.0 * np.pi * th[:, None] * t[None, :] / n
    re, im = np.cos(ang), -np.sin(ang)
    fx = np.zeros((2 * BLK, BLK))
    inv = np.zeros((BLK, n))
    for g in range(NG):
        r, i = re[8 * g:8 * g + 8], im[8 * g:8 * g + 8]
        fx[16 * g:16 * g + 8] = r
        fx[16 * g + 8:16 * g + 16] = i
        inv[:, 16 * g:16 * g + 8] = (2.0 / n) * r.T
        inv[:, 16 * g + 8:16 * g + 16] = (2.0 / n) * i.T
    return _pack_rows(fx), _pack_rows(inv)


def _gelu(x):
    c0 = 0.7978845608028654
    u = x * (c0 + (c0 * 0.044715) * (x * x))
    hx = 0.5 * x
    return hx + hx * jnp.tanh(u)


def _kernel(q_hbm, k_hbm, v_hbm, sh_ref, h_hbm, dvec_ref, w1_hbm, b1_ref, w2_hbm,
            b2_ref, c_ref, wm_hbm, fx_ref, inv_ref, o_hbm,
            qb, kb, vb, hb, wmb, w1b, w2b, ob, kf, wb, kvb, hp,
            xh0, xh1, xh2, xh3, yf0, yf1, yf2, yf3,
            qp, yb, modb, h2r, x1r, gbuf, zs,
            sem, sem_o):
    xhq = (xh0, xh1, xh2, xh3)
    yfq = (yf0, yf1, yf2, yf3)

    def k_cp(j):
        return pltpu.make_async_copy(k_hbm.at[0, pl.ds(BLK * j, BLK)],
                                     kb.at[pl.ds(BLK * j, BLK)], sem.at[3 * j])

    def v_cp(j):
        return pltpu.make_async_copy(v_hbm.at[0, pl.ds(BLK * j, BLK)],
                                     vb.at[pl.ds(BLK * j, BLK)], sem.at[3 * j + 1])

    def h_cp(j):
        return pltpu.make_async_copy(h_hbm.at[:, pl.ds(BLK * j, BLK)],
                                     hb.at[j], sem.at[3 * j + 2])

    def wm_cp(n):
        return pltpu.make_async_copy(wm_hbm.at[:, pl.ds(D * n, D)], wmb.at[n],
                                     sem.at[3 * NB + n])

    def q_cp(i):
        r0 = i * TM if isinstance(i, int) else pl.multiple_of(i * TM, TM)
        return pltpu.make_async_copy(q_hbm.at[0, pl.ds(r0, TM)], qb.at[pl.ds(r0, TM)],
                                     sem.at[3 * NB + 8 + i])

    w1_cp = pltpu.make_async_copy(w1_hbm, w1b, sem.at[3 * NB + 6])
    w2_cp = pltpu.make_async_copy(w2_hbm, w2b, sem.at[3 * NB + 7])

    for j in range(NB):
        k_cp(j).start()
        v_cp(j).start()
        h_cp(j).start()
    q_cp(0).start()
    for n in range(5):
        wm_cp(n).start()
    w1_cp.start()
    q_cp(1).start()
    w2_cp.start()
    wm_cp(5).start()
    for i in range(2, NS):
        q_cp(i).start()

    for n in range(8):
        zs[n] = 0
    sh = sh_ref[...].astype(F32)
    for t in range(4):
        wb[t] = jnp.broadcast_to(sh[t:t + 1, :], (8, D))
    kf[:, 0:8, :] = jnp.zeros((NL, 8, 128), F32)

    def wait_block(j):
        k_cp(j).wait()
        v_cp(j).wait()
        h_cp(j).wait()

    def stage_v(j, kvv, hpv):
        r0 = pl.multiple_of(j * BLK, BLK)
        for l in range(NL):
            ls = slice(128 * l, 128 * (l + 1))
            w = [jnp.concatenate([wb[t, :, ls]] * 2, axis=0) for t in range(4)]
            for rc in range(BLK // 16):
                r = pl.multiple_of(r0 + 16 * rc, 16)
                k = kb[pl.ds(r, 16), ls].astype(F32)
                v = vb[pl.ds(r, 16), ls].astype(F32)
                kf[l, pl.ds(r + 8, 16), :] = k
                ks = k * w[0]
                for t in range(1, 4):
                    ks = ks + kf[l, pl.ds(j * BLK + 16 * rc + (8 - t), 16), :] * w[t]
                kvv[64 + 8 * rc:64 + 8 * rc + 8, ls] = pltpu.bitcast((ks * v).astype(BF), U32)
        hpv[1] = pltpu.bitcast(hb[j], U32)

    def stage_a(p, i, kvv, hpv):
        kv = pltpu.bitcast(kvv[0:64, :], BF)
        xf = jnp.dot(pltpu.bitcast(fx_ref[...], BF), kv, preferred_element_type=F32)
        xhq[p][i] = xf.reshape(4, 64, D)
        hf = lax.dot_general(pltpu.bitcast(fx_ref[...], BF), pltpu.bitcast(hpv[0], BF),
                             (((1,), (1,)), ((), ())), preferred_element_type=F32)
        xhq[p][4 + i] = hf.reshape(4, 64, D)

    def stage_b(q, i, gg, lanes=tuple(range(NL))):
        y0 = 8 * gg
        yfv = [yfq[q].at[pl.ds(32 * i + BLK * da if isinstance(i, int) else pl.multiple_of(32 * i + BLK * da, 32), 32)] for da in range(4)]
        a0 = 4 * q
        for l in lanes:
            ls = slice(128 * l, 128 * (l + 1))
            acc = [[None] * 3 for _ in range(4)]
            xs = {}
            for m in range(a0 + 4):
                hr = xhq[m // 4][4 + m % 4, i, pl.ds(16 * gg, 8), ls]
                hi = xhq[m // 4][4 + m % 4, i, pl.ds(16 * gg + 8, 8), ls]
                hm = (hr + hi, hr, hi)
                for da in range(4):
                    jx = a0 + da - m
                    if jx < 0:
                        continue
                    if jx not in xs:
                        xr = xhq[jx // 4][jx % 4, i, pl.ds(16 * gg, 8), ls]
                        xi = xhq[jx // 4][jx % 4, i, pl.ds(16 * gg + 8, 8), ls]
                        xs[jx] = (xr + xi, xr, xi)
                    for c in range(3):
                        p = xs[jx][c] * hm[c]
                        acc[da][c] = p if acc[da][c] is None else acc[da][c] + p
            if q > 0:
                pr = qp[i, 0, pl.ds(y0, 8), ls]
                pi = qp[i, 1, pl.ds(y0, 8), ls]
            for da in range(4):
                s3, s1, s2 = acc[da]
                re = s1 - s2
                im = s3 - (s1 + s2)
                if q == 0 and da == 0:
                    ore, oim = re, im
                else:
                    ore, oim = re - pi, im + pr
                yfv[da][pl.ds(y0, 8), ls] = pltpu.bitcast(
                    jnp.concatenate([ore, oim], axis=0).astype(BF), U32)
                pr, pi = re, im
            if q < 3:
                qp[i, 0, pl.ds(y0, 8), ls] = pr
                qp[i, 1, pl.ds(y0, 8), ls] = pi

    def link(v, n):
        for q in range(4):
            xhq[q][8, 0, 8 * n:8 * n + 8, 0:128] = v

    def stage_b3(ls):
        for g in range(NG):
            i, gg = g // 4, g % 4
            pr = qp[i, 0, 8 * gg:8 * gg + 8, ls]
            pi = qp[i, 1, 8 * gg:8 * gg + 8, ls]
            for a0 in range(12, 16, NACC):
                acc = [[None] * 3 for _ in range(NACC)]
                xs = {}
                for m in range(a0 + NACC):
                    hr = xhq[m // 4][4 + m % 4, i, 16 * gg:16 * gg + 8, ls]
                    hi = xhq[m // 4][4 + m % 4, i, 16 * gg + 8:16 * gg + 16, ls]
                    hm = (hr + hi, hr, hi)
                    for da in range(NACC):
                        jx = a0 + da - m
                        if jx < 0:
                            continue
                        if jx not in xs:
                            xr = xhq[jx // 4][jx % 4, i, 16 * gg:16 * gg + 8, ls]
                            xi = xhq[jx // 4][jx % 4, i, 16 * gg + 8:16 * gg + 16, ls]
                            xs[jx] = (xr + xi, xr, xi)
                        for c in range(3):
                            p = xs[jx][c] * hm[c]
                            acc[da][c] = p if acc[da][c] is None else acc[da][c] + p
                for da in range(NACC):
                    s3, s1, s2 = acc[da]
                    re = s1 - s2
                    im = s3 - (s1 + s2)
                    r = BLK * (a0 - 12 + da) + 8 * g
                    oim = im + pr
                    yf3[r:r + 8, ls] = pltpu.bitcast(
                        jnp.concatenate([re - pi, oim], axis=0).astype(BF), U32)
                    pr, pi = re, im
                v = oim
                for _ in range(HOPS):
                    v = jnp.tanh(v)
                link(v, 0)

    def stage_c3(ls):
        for i in range(4):
            for hh in range(2):
                yf = yf3[BLK * i + 64 * hh:BLK * i + 64 * hh + 64, ls]
                yb[hh, (12 + i) * BLK:(13 + i) * BLK, ls] = jnp.dot(
                    pltpu.bitcast(inv_ref[:, 128 * hh:128 * (hh + 1)], BF),
                    pltpu.bitcast(yf, BF), preferred_element_type=F32)

    def stage_c(q, i):
        mo = (lambda v, n: v) if isinstance(i, int) else pl.multiple_of
        r0 = mo((4 * q + i) * BLK, BLK)
        for hh in range(2):
            yf = yfq[q][pl.ds(mo(i * BLK + 64 * hh, 64), 64), :]
            yb[hh, pl.ds(r0, BLK), :] = jnp.dot(
                pltpu.bitcast(inv_ref[:, 128 * hh:128 * (hh + 1)], BF),
                pltpu.bitcast(yf, BF), preferred_element_type=F32)

    def phase(p):
        def body(i, carry):
            t = 4 * p + i + 1
            if p < 3:
                wait_block(t)
            elif p == 3:
                @pl.when(t < NB)
                def _():
                    wait_block(t)
            if p < 4:
                kvv = kvb.at[pl.ds(pl.multiple_of(t * 64, 64), 128)]
                hpv = hp.at[pl.ds(t, 2)]
                stage_a(p, i, kvv, hpv)
            if p >= 2:
                stage_c(p - 2, i)
            if p < 4:
                stage_v(jnp.minimum(t, NB - 1) if p == 3 else t, kvv, hpv)
            if 1 <= p <= 4:
                for gg in range(4):
                    stage_b(p - 1, i, gg)
            return carry
        with jax.named_scope("p%d" % p):
            lax.fori_loop(0, 4, body, 0)

    wait_block(0)
    stage_v(jnp.int32(0), kvb.at[pl.ds(0, 128)], hp.at[pl.ds(0, 2)])
    phase(0)
    dvec = jnp.broadcast_to(dvec_ref[...].astype(F32).reshape(1, D), (8, D))
    for g in range(NG):
        a, r = g // 4, 16 * (g % 4)
        xh0[4, a, r:r + 8, :] = xh0[4, a, r:r + 8, :] + dvec
    for p in range(1, 4):
        phase(p)
    with jax.named_scope("p4"):
        for i in range(4):
            stage_c(2, i)

    zero = jnp.minimum(pl.program_id(0), 0)
    c = c_ref[...].astype(F32)
    sc = jnp.broadcast_to((c * jax.nn.sigmoid(c)).astype(BF), (16, D))

    def mod_chunk(n):
        wm_cp(n).wait()
        m = jnp.dot(sc, wmb[n], preferred_element_type=F32)[0:8]
        modb[n] = m + 1.0 if n in (1, 4) else m

    with jax.named_scope("mod"):
        q_cp(0).wait()
        for n in range(5):
            mod_chunk(n)

    b1 = b1_ref[...].astype(F32).reshape(1, F)
    b2 = b2_ref[...].astype(F32).reshape(1, D)

    def o_cp(i):
        r0 = pl.multiple_of(i * TM, TM)
        return pltpu.make_async_copy(ob.at[pl.ds(r0, TM)], o_hbm.at[0, pl.ds(r0, TM)],
                                     sem_o.at[i])

    def stats(x):
        m = jnp.sum(x, axis=-1, keepdims=True) * (1.0 / D)
        m2 = jnp.sum(x * x, axis=-1, keepdims=True) * (1.0 / D)
        return m, lax.rsqrt(jnp.maximum(m2 - m * m, 0.0) + EPS)

    def prep(i, h2v, x1v, xoff, chain=True):
        ra = i * TM + zs[0] * 16
        rb = i * TM + zs[1] * 16
        rc_ = i * TM + zs[2] * 16
        for g0 in range(0, TM // 16, LINK):
            grp = range(g0, g0 + LINK)
            xs = [qb[pl.ds(pl.multiple_of(ra + 16 * rc, 16), 16), :] for rc in grp]
            st1 = [stats(x.astype(F32)) for x in xs]
            st2 = []
            for rc in grp:
                r = pl.multiple_of(rb + 16 * rc, 16)
                sa, ca, ga = [jnp.concatenate([modb[n]] * 2, axis=0) for n in range(3)]
                m, rs = st1[rc - g0]
                x = qb[pl.ds(r, 16), :].astype(F32)
                h = ((x - m) * rs) * ca + sa
                x1 = x + ga * (h * (yb[0, pl.ds(r, 16), :] + yb[1, pl.ds(r, 16), :]))
                x1v[xoff + 16 * rc:xoff + 16 * rc + 16, :] = x1
                st2.append(stats(x1))
            for rc in grp:
                sb, cb = [jnp.concatenate([modb[n]] * 2, axis=0) for n in (3, 4)]
                m, rs = st2[rc - g0]
                x1 = x1r[pl.ds(pl.multiple_of(rc_ + 16 * rc, 16), 16), :]
                h2 = ((x1 - m) * rs) * cb + sb
                h2v[8 * rc:8 * rc + 8, :] = pltpu.bitcast(h2.astype(BF), U32)
                if chain and g0 + LINK < TM // 16:
                    qb[S:S + 8, 128 * (rc - g0):128 * (rc - g0 + 1)] = h2[8:16, D - 128:D].astype(BF)
                elif chain:
                    xh3[8, 1, 8 * (rc - g0):8 * (rc - g0) + 8, 0:128] = h2[8:16, D - 128:D]

    def mm1(h2v, off):
        h2 = pltpu.bitcast(h2v[off * TM // 2:(off + 1) * TM // 2, :], BF)
        g = lax.dot_general(h2, w1b[...], (((1,), (1,)), ((), ())),
                            preferred_element_type=F32) + b1
        gbuf[...] = pltpu.bitcast(_gelu(g).astype(BF), U32)

    def mm2(i, x1v, off):
        r0 = pl.multiple_of(i * TM, TM)
        gb = modb[5][0:1]
        o = jnp.dot(pltpu.bitcast(gbuf[...], BF), w2b[...], preferred_element_type=F32) + b2
        ob[pl.ds(r0, TM), :] = (x1v[off * TM:(off + 1) * TM, :] + gb * o).astype(BF)
        o_cp(i).start()

    with jax.named_scope("prep0"):
        prep(0, h2r, x1r, 0, False)
    with jax.named_scope("first"):
        w1_cp.wait()
        mm1(h2r, 0)
    with jax.named_scope("w2wait"):
        w2_cp.wait()
        mod_chunk(5)

    def step(k, carry):
        h2v = h2r.at[pl.ds(pl.multiple_of(k * (TM // 2), TM // 2), TM // 2)]
        x1o = x1r.at[pl.ds(pl.multiple_of((k - 1) * TM, TM), 2 * TM)]
        q_cp(k).wait()
        lc = pl.ds(pl.multiple_of(jnp.minimum(k - 1, NL - 1) * 128, 128), 128)
        mm2(k - 1, x1o, 0)
        prep(k, h2v, x1o, TM)
        if not NOMAC:
            stage_b3(lc)
        mm1(h2v, 0)
        stage_c3(lc)
        return carry

    with jax.named_scope("mlp"):
        lax.fori_loop(1, NS, step, 0)
    with jax.named_scope("last"):
        mm2(NS - 1, x1r, NS - 1)
    for i in range(NS):
        o_cp(i).wait()


@jax.jit
def pallas_adaLN_cond__ssm_conv_h3__dense_activation_gelu__prompt_kernel(
    A_q, A_k, A_v, A_shift_k, A_ssm_k, A_ssm_D, B_x, B_w1, B_b1, B_w2, B_b2, c, w_mod,
):
    del B_x
    fx, inv = _dft_mats()
    any_spec = pl.BlockSpec(memory_space=pl.ANY)
    vmem_spec = pl.BlockSpec(memory_space=pltpu.VMEM)
    in_specs = [any_spec, any_spec, any_spec, vmem_spec, any_spec, vmem_spec, any_spec,
                vmem_spec, any_spec, vmem_spec, vmem_spec, any_spec, vmem_spec, vmem_spec]
    scratch = [
        pltpu.VMEM((S + 16, D), BF),
        pltpu.VMEM((S, D), BF),
        pltpu.VMEM((S, D), BF),
        pltpu.VMEM((NB, D, BLK), BF),
        pltpu.VMEM((6, D, D), BF),
        pltpu.VMEM((F, D), BF),
        pltpu.VMEM((F, D), BF),
        pltpu.VMEM((S, D), BF),
        pltpu.VMEM((NL, S + 8, 128), F32),
        pltpu.VMEM((4, 8, D), F32),
        pltpu.VMEM(((NB + 2) * 64, D), U32),
        pltpu.VMEM((NB + 2, D // 2, BLK), U32),
    ] + [pltpu.VMEM((9, 4, 64, D), F32)] * 4 + [pltpu.VMEM((4 * BLK, D), U32)] * 4 + [
        pltpu.VMEM((4, 2, 32, D), F32),
        pltpu.VMEM((2, S, D), F32),
        pltpu.VMEM((6, 8, D), F32),
        pltpu.VMEM(((NS + 1) * TM // 2, D), U32),
        pltpu.VMEM(((NS + 1) * TM, D), F32),
        pltpu.VMEM((TM // 2, F), U32),
        pltpu.SMEM((8,), jnp.int32),
        pltpu.SemaphoreType.DMA((3 * NB + 8 + NS,)),
        pltpu.SemaphoreType.DMA((NS,)),
    ]
    return pl.pallas_call(
        _kernel,
        grid=(1,),
        in_specs=in_specs,
        out_specs=any_spec,
        out_shape=jax.ShapeDtypeStruct((1, S, D), BF),
        scratch_shapes=scratch,
        compiler_params=pltpu.CompilerParams(vmem_limit_bytes=110 * 1024 * 1024),
    )(A_q, A_k, A_v, A_shift_k.T, A_ssm_k, A_ssm_D, B_w1.T, B_b1, B_w2, B_b2, c, w_mod,
      jnp.asarray(fx), jnp.asarray(inv))
```

```python
import numpy as np
import jax
import jax.numpy as jnp
from jax import lax
import jax.experimental.pallas as pl
import jax.experimental.pallas.tpu as pltpu

S = 2048
D = 640
F = 1728
BLK = 128
NB = S // BLK
NG = BLK // 8
NL = D // 128
TM = 256
TH = TM // 2
NS = S // TM
F0 = 512
EPS = 1e-5
BF = jnp.bfloat16
F32 = jnp.float32
U32 = jnp.uint32
LINK = 2
NACC = 2
HOPS = 8
HOPSB = 16
MUL4 = 0
L0 = 'p4'
SPLIT = 0
FM = 1280
VAR = 'b'
NT = (((1,), (1,)), ((), ()))


def _pack_rows(a):
    u = np.ascontiguousarray(a, dtype=np.float32).view(np.uint32)
    u = (u + 0x7FFF + ((u >> 16) & 1)) >> 16
    return (u[0::2] | (u[1::2] << 16)).astype(np.uint32)


def _dft_mats():
    n = 2 * BLK
    th = 2.0 * np.arange(BLK) + 0.5
    t = np.arange(BLK)
    ang = 2.0 * np.pi * th[:, None] * t[None, :] / n
    re, im = np.cos(ang), -np.sin(ang)
    fx = np.zeros((2 * BLK, BLK))
    inv = np.zeros((BLK, n))
    for g in range(NG):
        r, i = re[8 * g:8 * g + 8], im[8 * g:8 * g + 8]
        fx[16 * g:16 * g + 8] = r
        fx[16 * g + 8:16 * g + 16] = i
        inv[:, 16 * g:16 * g + 8] = (2.0 / n) * r.T
        inv[:, 16 * g + 8:16 * g + 16] = (2.0 / n) * i.T
    inv = _pack_rows(inv)
    return np.concatenate([_pack_rows(fx), inv[:, :BLK], inv[:, BLK:]], axis=0)


def _gelu(x):
    c0 = 0.7978845608028654
    u = x * (c0 + (c0 * 0.044715) * (x * x))
    hx = 0.5 * x
    return hx + hx * jnp.tanh(u)


def _stats(x):
    m = jnp.sum(x, axis=-1, keepdims=True) * (1.0 / D)
    m2 = jnp.sum(x * x, axis=-1, keepdims=True) * (1.0 / D)
    return m, lax.rsqrt(jnp.maximum(m2 - m * m, 0.0) + EPS)


def _mo(v, n):
    return v if isinstance(v, int) else pl.multiple_of(v, n)


def _kernel(q_hbm, k_hbm, v_hbm, sh_hbm, h_hbm, dv_hbm, w1_hbm, b1_hbm, w2_hbm,
            b2_hbm, c_hbm, wm_hbm, dft_hbm, o_hbm,
            qb, kb, vb, hb, wmb, w1b, w2b, ob, shb, dvb, b1b, b2b, cb_, dft,
            kf, wb, kvb, hp, xh0, xh1, xh2, xh3, yf0, yf1, yf2, yf3,
            qp, yb, modb, h2r, x1r, gr, zs, sem, sem_o):
    xhq = (xh0, xh1, xh2, xh3)
    yfq = (yf0, yf1, yf2, yf3)
    cp = pltpu.make_async_copy
    n0 = 3 * NB

    def k_cp(j):
        return cp(k_hbm.at[0, pl.ds(BLK * j, BLK)], kb.at[pl.ds(BLK * j, BLK)], sem.at[3 * j])

    def v_cp(j):
        return cp(v_hbm.at[0, pl.ds(BLK * j, BLK)], vb.at[pl.ds(BLK * j, BLK)], sem.at[3 * j + 1])

    def h_cp(j):
        return cp(h_hbm.at[:, pl.ds(BLK * j, BLK)], hb.at[j], sem.at[3 * j + 2])

    def wm_cp(n):
        return cp(wm_hbm.at[:, pl.ds(D * n, D)], wmb.at[n], sem.at[n0 + n])

    def q_cp(i):
        r0 = _mo(i * TM, TM)
        return cp(q_hbm.at[0, pl.ds(r0, TM)], qb.at[pl.ds(r0, TM)], sem.at[n0 + 6 + i])

    n1 = n0 + 6 + NS
    w1a_cp = cp(w1_hbm.at[pl.ds(0, F0)], w1b.at[pl.ds(0, F0)], sem.at[n1])
    w1b_cp = cp(w1_hbm.at[pl.ds(F0, F - F0)], w1b.at[pl.ds(F0, F - F0)], sem.at[n1 + 1])
    w2_cp = cp(w2_hbm, w2b, sem.at[n1 + 2])
    sh_cp = cp(sh_hbm, shb, sem.at[n1 + 3])
    dft_cp = cp(dft_hbm, dft, sem.at[n1 + 4])
    small = [cp(dv_hbm, dvb, sem.at[n1 + 5]), cp(c_hbm, cb_, sem.at[n1 + 6]),
             cp(b1_hbm, b1b, sem.at[n1 + 7]), cp(b2_hbm, b2b, sem.at[n1 + 8])]

    sh_cp.start()
    for j in range(NB):
        k_cp(j).start()
        v_cp(j).start()
        h_cp(j).start()
        if j == 0:
            dft_cp.start()
        if j == 1:
            for c_ in small:
                c_.start()
    q_cp(0).start()
    if VAR == 'b':
        q_cp(1).start()
    for n in range(5):
        wm_cp(n).start()
    w1a_cp.start()
    if VAR != 'b':
        q_cp(1).start()
    w1b_cp.start()
    w2_cp.start()
    wm_cp(5).start()
    for i in range(2, NS):
        q_cp(i).start()

    for n in range(4):
        zs[n] = 0
    kf[:, 0:8, :] = jnp.zeros((NL, 8, 128), F32)
    sh_cp.wait()
    sh = shb[...].astype(F32)
    for t in range(4):
        wb[t] = jnp.broadcast_to(sh[t:t + 1, :], (8, D))

    def wait_block(j):
        k_cp(j).wait()
        v_cp(j).wait()
        h_cp(j).wait()

    def stage_v(j, kvv, hpv):
        r0 = pl.multiple_of(j * BLK, BLK)
        for l in range(NL):
            ls = slice(128 * l, 128 * (l + 1))
            w = [jnp.concatenate([wb[t, :, ls]] * 2, axis=0) for t in range(4)]
            for rc in range(BLK // 16):
                r = pl.multiple_of(r0 + 16 * rc, 16)
                k = kb[pl.ds(r, 16), ls].astype(F32)
                v = vb[pl.ds(r, 16), ls].astype(F32)
                kf[l, pl.ds(r + 8, 16), :] = k
                ks = k * w[0]
                for t in range(1, 4):
                    ks = ks + kf[l, pl.ds(j * BLK + 16 * rc + (8 - t), 16), :] * w[t]
                kvv[64 + 8 * rc:64 + 8 * rc + 8, ls] = pltpu.bitcast((ks * v).astype(BF), U32)
        hpv[1] = pltpu.bitcast(hb[j], U32)

    def stage_a(p, i, kvv, hpv):
        fx = pltpu.bitcast(dft[0:BLK, :], BF)
        xf = jnp.dot(fx, pltpu.bitcast(kvv[0:64, :], BF), preferred_element_type=F32)
        for l in range(NL):
            xhq[p][l, i] = xf[:, 128 * l:128 * (l + 1)].reshape(4, 64, 128)
        hf = lax.dot_general(fx, pltpu.bitcast(hpv[0], BF), NT, preferred_element_type=F32)
        for l in range(NL):
            xhq[p][l, 4 + i] = hf[:, 128 * l:128 * (l + 1)].reshape(4, 64, 128)

    all_lanes = list(range(NL))

    def link(v):
        for q in range(4):
            xhq[q][zs[3], 8, 0, 0:8, :] = v

    def stage_b(a0, n, i, lanes, hops):
        q = a0 // 4
        yfv = [yfq[q].at[pl.ds(_mo(32 * i + BLK * ((a0 + da) % 4), 32), 32)] for da in range(n)]
        for gg in range(4):
            y0 = 8 * gg
            for l in lanes:
                ls = pl.ds(_mo(128 * l, 128), 128)
                if a0 > 0:
                    pr = qp[i, 0, y0:y0 + 8, ls]
                    pi = qp[i, 1, y0:y0 + 8, ls]
                acc = [[None] * 3 for _ in range(n)]
                xs = {}
                for m in range(a0 + n):
                    hr = xhq[m // 4][l, 4 + m % 4, i, 16 * gg:16 * gg + 8, :]
                    hi = xhq[m // 4][l, 4 + m % 4, i, 16 * gg + 8:16 * gg + 16, :]
                    hm = (hr + hi, hr, hi)
                    for da in range(n):
                        jx = a0 + da - m
                        if jx < 0:
                            continue
                        if jx not in xs:
                            xr = xhq[jx // 4][l, jx % 4, i, 16 * gg:16 * gg + 8, :]
                            xi = xhq[jx // 4][l, jx % 4, i, 16 * gg + 8:16 * gg + 16, :]
                            xs[jx] = (xr + xi, xr, xi)
                        for c in range(3):
                            p = xs[jx][c] * hm[c]
                            acc[da][c] = p if acc[da][c] is None else acc[da][c] + p
                for da in range(n):
                    s3, s1, s2 = acc[da]
                    re = s1 - s2
                    im = s3 - (s1 + s2)
                    if a0 + da == 0:
                        ore, oim = re, im
                    else:
                        ore, oim = re - pi, im + pr
                    yfv[da][y0:y0 + 8, ls] = pltpu.bitcast(
                        jnp.concatenate([ore, oim], axis=0).astype(BF), U32)
                    pr, pi = re, im
                if a0 + n < NB:
                    qp[i, 0, y0:y0 + 8, ls] = pr
                    qp[i, 1, y0:y0 + 8, ls] = pi
                if hops is not None:
                    v = oim
                    for _ in range(hops):
                        v = jnp.tanh(v)
                    link(v)

    def stage_c(q, i, ls=slice(None)):
        r0 = _mo((4 * q + i) * BLK, BLK)
        for hh in range(2):
            yf = yfq[q][pl.ds(_mo(i * BLK + 64 * hh, 64), 64), ls]
            g = pltpu.bitcast(dft[BLK + 64 * hh:BLK + 64 * (hh + 1), :], BF)
            yb[hh, pl.ds(r0, BLK), ls] = jnp.dot(g, pltpu.bitcast(yf, BF),
                                                 preferred_element_type=F32)

    def unit_b(a0, lane):
        for i in range(4):
            stage_b(a0, 2, i, [lane], HOPS)

    def unit_c(a0, lane):
        ls = pl.ds(_mo(lane * 128, 128), 128)
        for i in range(2):
            stage_c(3, a0 % 4 + i, ls)

    def phase(p):
        def body(i, carry):
            t = 4 * p + i + 1
            if p < 3:
                wait_block(t)
            else:
                @pl.when(t < NB)
                def _():
                    wait_block(t)
            kvv = kvb.at[pl.ds(pl.multiple_of(t * 64, 64), 128)]
            hpv = hp.at[pl.ds(t, 2)]
            stage_a(p, i, kvv, hpv)
            if p >= 2:
                stage_c(p - 2, i)
            stage_v(jnp.minimum(t, NB - 1) if p == 3 else t, kvv, hpv)
            if p >= 1:
                stage_b(4 * (p - 1), 4, i, all_lanes, None)
            return carry
        with jax.named_scope("p%d" % p):
            lax.fori_loop(0, 4, body, 0)

    with jax.named_scope("w0"):
        wait_block(0)
    with jax.named_scope("v0"):
        stage_v(jnp.int32(0), kvb.at[pl.ds(0, 128)], hp.at[pl.ds(0, 2)])
        dft_cp.wait()
    phase(0)
    for c_ in small:
        c_.wait()
    dvec = jnp.broadcast_to(dvb[...].astype(F32).reshape(1, D), (8, D))
    for g in range(NG):
        a, r = g // 4, 16 * (g % 4)
        for l in range(NL):
            xh0[l, 4, a, r:r + 8, :] = xh0[l, 4, a, r:r + 8, :] + dvec[:, 128 * l:128 * (l + 1)]
    for p in range(1, 4):
        phase(p)

    c = cb_[...].astype(F32)
    sc = jnp.broadcast_to((c * jax.nn.sigmoid(c)).astype(BF), (16, D))
    b1 = b1b[...].astype(F32).reshape(1, F)
    b2 = b2b[...].astype(F32).reshape(1, D)

    def mod_chunk(n):
        m = jnp.dot(sc, wmb[n], preferred_element_type=F32)[0:8]
        modb[n] = m + 1.0 if n in (1, 4) else m

    def mods(ns):
        return [jnp.concatenate([modb[n]] * 2, axis=0) for n in ns]

    def prep1(i, grp):
        ra = i * TM + zs[0] * 16
        xs = [qb[pl.ds(pl.multiple_of(ra + 16 * rc, 16), 16), :] for rc in grp]
        return [_stats(x.astype(F32)) for x in xs]

    def prep2(i, grp, st1, x1v, xoff):
        rb = i * TM + zs[1] * 16
        st2 = []
        for rc, (m, rs) in zip(grp, st1):
            r = pl.multiple_of(rb + 16 * rc, 16)
            sa, ca, ga = mods((0, 1, 2))
            x = qb[pl.ds(r, 16), :].astype(F32)
            h = ((x - m) * rs) * ca + sa
            x1 = x + ga * (h * (yb[0, pl.ds(r, 16), :] + yb[1, pl.ds(r, 16), :]))
            x1v[xoff + 16 * rc:xoff + 16 * rc + 16, :] = x1
            st2.append(_stats(x1))
        return st2

    def prep3(i, grp, st2, h2v, hoff, chain):
        rc_ = i * TM + zs[2] * 16
        for n, (rc, (m, rs)) in enumerate(zip(grp, st2)):
            sb, cb = mods((3, 4))
            x1 = x1r[pl.ds(pl.multiple_of(rc_ + 16 * rc, 16), 16), :]
            h2 = ((x1 - m) * rs) * cb + sb
            h2v[hoff + 8 * rc:hoff + 8 * rc + 8, :] = pltpu.bitcast(h2.astype(BF), U32)
            if chain == 1:
                qb[S:S + 8, 128 * n:128 * (n + 1)] = h2[8:16, D - 128:D].astype(BF)
            elif chain == 2:
                xh3[zs[3], 8, 1, 8 * n:8 * n + 8, :] = h2[8:16, D - 128:D]

    def prep(i, h2v, hoff, x1v, xoff, link_n):
        for g0 in range(0, TM // 16, link_n):
            grp = range(g0, g0 + link_n)
            st2 = prep2(i, grp, prep1(i, grp), x1v, xoff)
            prep3(i, grp, st2, h2v, hoff, 1 if g0 + link_n < TM // 16 else 2)

    def o_cp(i):
        r0 = _mo(i * TM, TM)
        return cp(ob.at[pl.ds(r0, TM)], o_hbm.at[0, pl.ds(r0, TM)], sem_o.at[i])

    def mm1(h2v, hoff, gv, goff, rows, f0, f1):
        h2 = pltpu.bitcast(h2v[hoff:hoff + rows // 2, :], BF)
        g = lax.dot_general(h2, w1b[f0:f1, :], NT, preferred_element_type=F32) + b1[:, f0:f1]
        gv[goff:goff + rows // 2, f0:f1] = pltpu.bitcast(_gelu(g).astype(BF), U32)

    def mm2(i, gv, goff, x1v, xoff):
        r0 = _mo(i * TM, TM)
        gb = modb[5][0:1]
        o = jnp.dot(pltpu.bitcast(gv[goff:goff + TH, :], BF), w2b[...],
                    preferred_element_type=F32) + b2
        ob[pl.ds(r0, TM), :] = (x1v[xoff:xoff + TM, :] + gb * o).astype(BF)
        o_cp(i).start()

    allg = range(TM // 16)
    with jax.named_scope("p4"):
        q_cp(0).wait()
        if VAR == 'b':
            q_cp(1).wait()
        for n in range(3):
            wm_cp(n).wait()
        for n in range(3):
            mod_chunk(n)
        for i in range(4):
            stage_c(2, i)
        st1 = prep1(0, allg)
        if VAR == 'b':
            st1b = prep1(1, allg)
    with jax.named_scope("p5"):
        wm_cp(3).wait()
        mod_chunk(3)
        st2 = prep2(0, allg, st1, x1r, 0)
    with jax.named_scope("p6"):
        wm_cp(4).wait()
        mod_chunk(4)
        prep3(0, allg, st2, h2r, 0, 0)
    with jax.named_scope("firstA"):
        w1a_cp.wait()
        if VAR != 'b':
            q_cp(1).wait()
            st1b = prep1(1, allg)
        mm1(h2r, 0, gr, 0, TM, 0, F0)
        st2 = prep2(1, allg, st1b, x1r, TM)
        prep3(1, allg, st2, h2r, TH, 0)
        mm1(h2r, TH, gr, TH, TM, 0, F0)
    with jax.named_scope("firstB"):
        w1b_cp.wait()
        unit_b(12, 0)
        mm1(h2r, 0, gr, 0, 2 * TM, F0, FM)
        unit_c(12, 0)
        if FM < F:
            mm1(h2r, 0, gr, 0, 2 * TM, FM, F)
    with jax.named_scope("w2wait"):
        w2_cp.wait()
        wm_cp(5).wait()
        mod_chunk(5)

    def step(k, units):
        if isinstance(k, int):
            x1v, xo, gv, go = x1r, (k - 2) * TM, gr, (k - 2) * TH
        else:
            x1v = x1r.at[pl.ds(pl.multiple_of((k - 2) * TM, TM), 3 * TM)]
            gv = gr.at[pl.ds(pl.multiple_of((k - 2) * TH, TH), 3 * TH)]
            xo = go = 0
        q_cp(k).wait()
        mm2(k - 2, gv, go, x1v, xo)
        prep(k, h2r, 0, x1v, xo + 2 * TM, LINK)
        for a0, lane in units:
            unit_b(a0, lane)
        mm1(h2r, 0, gv, go + 2 * TH, TM, 0, F)
        for a0, lane in units:
            unit_c(a0, lane)

    def body(k, carry):
        step(k, [(12, k - 1), (14, k - 2)])
        return carry

    with jax.named_scope("mloop"):
        lax.fori_loop(2, 6, body, 0)
    with jax.named_scope("m6"):
        step(6, [(14, NL - 1)])
    with jax.named_scope("m7"):
        step(7, [])
    with jax.named_scope("last"):
        for i in range(NS - 2, NS):
            mm2(i, gr, i * TH, x1r, i * TM)
    with jax.named_scope("owait"):
        for i in range(NS):
            o_cp(i).wait()


@jax.jit
def pallas_adaLN_cond__ssm_conv_h3__dense_activation_gelu__prompt_kernel(
    A_q, A_k, A_v, A_shift_k, A_ssm_k, A_ssm_D, B_x, B_w1, B_b1, B_w2, B_b2, c, w_mod,
):
    del B_x
    any_spec = pl.BlockSpec(memory_space=pl.ANY)
    scratch = [
        pltpu.VMEM((S + 16, D), BF),
        pltpu.VMEM((S, D), BF),
        pltpu.VMEM((S, D), BF),
        pltpu.VMEM((NB, D, BLK), BF),
        pltpu.VMEM((6, D, D), BF),
        pltpu.VMEM((F, D), BF),
        pltpu.VMEM((F, D), BF),
        pltpu.VMEM((S, D), BF),
        pltpu.VMEM((4, D), BF),
        pltpu.VMEM((D,), BF),
        pltpu.VMEM((F,), BF),
        pltpu.VMEM((D,), BF),
        pltpu.VMEM((1, D), BF),
        pltpu.VMEM((2 * BLK, BLK), U32),
        pltpu.VMEM((NL, S + 8, 128), F32),
        pltpu.VMEM((4, 8, D), F32),
        pltpu.VMEM(((NB + 2) * 64, D), U32),
        pltpu.VMEM((NB + 2, D // 2, BLK), U32),
    ] + [pltpu.VMEM((NL, 9, 4, 64, 128), F32)] * 4 + [pltpu.VMEM((4 * BLK, D), U32)] * 4 + [
        pltpu.VMEM((4, 2, 32, D), F32),
        pltpu.VMEM((2, S, D), F32),
        pltpu.VMEM((6, 8, D), F32),
        pltpu.VMEM((TM, D), U32),
        pltpu.VMEM((S, D), F32),
        pltpu.VMEM((S // 2, F), U32),
        pltpu.SMEM((8,), jnp.int32),
        pltpu.SemaphoreType.DMA((3 * NB + 6 + NS + 9,)),
        pltpu.SemaphoreType.DMA((NS,)),
    ]
    return pl.pallas_call(
        _kernel,
        in_specs=[any_spec] * 13,
        out_specs=any_spec,
        out_shape=jax.ShapeDtypeStruct((1, S, D), BF),
        scratch_shapes=scratch,
        compiler_params=pltpu.CompilerParams(vmem_limit_bytes=110 * 1024 * 1024),
    )(A_q, A_k, A_v, A_shift_k.T, A_ssm_k, A_ssm_D, B_w1.T, B_b1, B_w2, B_b2, c, w_mod,
      jnp.asarray(_dft_mats()))
```

```python
import numpy as np
import jax
import jax.numpy as jnp
from jax import lax
import jax.experimental.pallas as pl
import jax.experimental.pallas.tpu as pltpu

S = 2048
D = 640
F = 1728
BLK = 128
NB = S // BLK
NG = BLK // 8
NL = D // 128
TM = 256
TH = TM // 2
NS = S // TM
F0 = 512
EPS = 1e-5
BF = jnp.bfloat16
F32 = jnp.float32
U32 = jnp.uint32
LINK = 2
NACC = 2
HOPS = 8
HOPSB = 16
MUL4 = 0
L0 = 'p4'
SPLIT = 0
FM = 1280
DBL = 'x'
MERGE = 1
TAILR = 32
HALF = 1
FH = 1664
VAR = 'b'
NT = (((1,), (1,)), ((), ()))


def _pack_rows(a):
    u = np.ascontiguousarray(a, dtype=np.float32).view(np.uint32)
    u = (u + 0x7FFF + ((u >> 16) & 1)) >> 16
    return (u[0::2] | (u[1::2] << 16)).astype(np.uint32)


def _dft_mats():
    n = 2 * BLK
    th = 2.0 * np.arange(BLK) + 0.5
    t = np.arange(BLK)
    ang = 2.0 * np.pi * th[:, None] * t[None, :] / n
    re, im = np.cos(ang), -np.sin(ang)
    fx = np.zeros((2 * BLK, BLK))
    inv = np.zeros((BLK, n))
    for g in range(NG):
        r, i = re[8 * g:8 * g + 8], im[8 * g:8 * g + 8]
        fx[16 * g:16 * g + 8] = r
        fx[16 * g + 8:16 * g + 16] = i
        inv[:, 16 * g:16 * g + 8] = (2.0 / n) * r.T
        inv[:, 16 * g + 8:16 * g + 16] = (2.0 / n) * i.T
    inv = _pack_rows(inv)
    return np.concatenate([_pack_rows(fx), inv[:, :BLK], inv[:, BLK:]], axis=0)


def _gelu(x):
    c0 = 0.7978845608028654
    u = x * (c0 + (c0 * 0.044715) * (x * x))
    hx = 0.5 * x
    return hx + hx * jnp.tanh(u)


def _stats(x):
    m = jnp.sum(x, axis=-1, keepdims=True) * (1.0 / D)
    m2 = jnp.sum(x * x, axis=-1, keepdims=True) * (1.0 / D)
    return m, lax.rsqrt(jnp.maximum(m2 - m * m, 0.0) + EPS)


def _mo(v, n):
    return v if isinstance(v, int) else pl.multiple_of(v, n)


def _kernel(q_hbm, k_hbm, v_hbm, sh_hbm, h_hbm, dv_hbm, w1_hbm, b1_hbm, w2_hbm,
            b2_hbm, c_hbm, wm_hbm, dft_hbm, o_hbm,
            qb, kb, vb, hb, wmb, w1b, w2b, ob, shb, dvb, b1b, b2b, cb_, dft,
            kf, wb, kvb, hp, xh0, xh1, xh2, xh3, yf0, yf1, yf2, yf3,
            qp, yb, modb, h2r, x1r, gr, b1c, zs, sem, sem_o):
    xhq = (xh0, xh1, xh2, xh3)
    yfq = (yf0, yf1, yf2, yf3)
    cp = pltpu.make_async_copy
    n0 = 3 * NB

    def k_cp(j):
        return cp(k_hbm.at[0, pl.ds(BLK * j, BLK)], kb.at[pl.ds(BLK * j, BLK)], sem.at[3 * j])

    def v_cp(j):
        return cp(v_hbm.at[0, pl.ds(BLK * j, BLK)], vb.at[pl.ds(BLK * j, BLK)], sem.at[3 * j + 1])

    def h_cp(j):
        return cp(h_hbm.at[:, pl.ds(BLK * j, BLK)], hb.at[j], sem.at[3 * j + 2])

    def wm_cp(n):
        return cp(wm_hbm.at[:, pl.ds(D * n, D)], wmb.at[n], sem.at[n0 + n])

    def q_cp(i):
        r0 = _mo(i * TM, TM)
        return cp(q_hbm.at[0, pl.ds(r0, TM)], qb.at[pl.ds(r0, TM)], sem.at[n0 + 6 + i])

    n1 = n0 + 6 + NS
    w1a_cp = cp(w1_hbm.at[pl.ds(0, F0)], w1b.at[pl.ds(0, F0)], sem.at[n1])
    w1b_cp = cp(w1_hbm.at[pl.ds(F0, F - F0)], w1b.at[pl.ds(F0, F - F0)], sem.at[n1 + 1])
    w2_cp = cp(w2_hbm, w2b, sem.at[n1 + 2])
    sh_cp = cp(sh_hbm, shb, sem.at[n1 + 3])
    dft_cp = cp(dft_hbm, dft, sem.at[n1 + 4])
    small = [cp(dv_hbm, dvb, sem.at[n1 + 5]), cp(c_hbm, cb_, sem.at[n1 + 6]),
             cp(b1_hbm, b1b, sem.at[n1 + 7]), cp(b2_hbm, b2b, sem.at[n1 + 8])]

    sh_cp.start()
    for j in range(NB):
        k_cp(j).start()
        v_cp(j).start()
        h_cp(j).start()
        if j == 0:
            dft_cp.start()
        if j == 1:
            for c_ in small:
                c_.start()
    q_cp(0).start()
    if VAR == 'b':
        q_cp(1).start()
    for n in range(5):
        wm_cp(n).start()
    w1a_cp.start()
    if VAR != 'b':
        q_cp(1).start()
    w1b_cp.start()
    w2_cp.start()
    wm_cp(5).start()
    for i in range(2, NS):
        q_cp(i).start()

    for n in range(4):
        zs[n] = 0
    kf[:, 0:8, :] = jnp.zeros((NL, 8, 128), F32)
    sh_cp.wait()
    sh = shb[...].astype(F32)
    for t in range(4):
        wb[t] = jnp.broadcast_to(sh[t:t + 1, :], (8, D))

    def wait_block(j):
        k_cp(j).wait()
        v_cp(j).wait()
        h_cp(j).wait()

    def stage_v(j, kvv, hpv):
        r0 = pl.multiple_of(j * BLK, BLK)
        for l in range(NL):
            ls = slice(128 * l, 128 * (l + 1))
            w = [jnp.concatenate([wb[t, :, ls]] * 2, axis=0) for t in range(4)]
            for rc in range(BLK // 16):
                r = pl.multiple_of(r0 + 16 * rc, 16)
                k = kb[pl.ds(r, 16), ls].astype(F32)
                v = vb[pl.ds(r, 16), ls].astype(F32)
                kf[l, pl.ds(r + 8, 16), :] = k
                ks = k * w[0]
                for t in range(1, 4):
                    ks = ks + kf[l, pl.ds(j * BLK + 16 * rc + (8 - t), 16), :] * w[t]
                kvv[64 + 8 * rc:64 + 8 * rc + 8, ls] = pltpu.bitcast((ks * v).astype(BF), U32)
        hpv[1] = pltpu.bitcast(hb[j], U32)

    def stage_a(p, i, kvv, hpv):
        fx = pltpu.bitcast(dft[0:BLK, :], BF)
        xf = jnp.dot(fx, pltpu.bitcast(kvv[0:64, :], BF), preferred_element_type=F32)
        for l in range(NL):
            xhq[p][l, i] = xf[:, 128 * l:128 * (l + 1)].reshape(4, 64, 128)
        hf = lax.dot_general(fx, pltpu.bitcast(hpv[0], BF), NT, preferred_element_type=F32)
        for l in range(NL):
            xhq[p][l, 4 + i] = hf[:, 128 * l:128 * (l + 1)].reshape(4, 64, 128)

    all_lanes = list(range(NL))

    def link(v):
        for q in range(4):
            xhq[q][zs[3], 8, 0, 0:8, :] = v

    def stage_b(a0, n, i, lanes, hops):
        q = a0 // 4
        yfv = [yfq[q].at[pl.ds(_mo(32 * i + BLK * ((a0 + da) % 4), 32), 32)] for da in range(n)]
        for gg in range(4):
            y0 = 8 * gg
            for l in lanes:
                ls = pl.ds(_mo(128 * l, 128), 128)
                if a0 > 0:
                    pr = qp[i, 0, y0:y0 + 8, ls]
                    pi = qp[i, 1, y0:y0 + 8, ls]
                acc = [[None] * 3 for _ in range(n)]
                xs = {}
                for m in range(a0 + n):
                    hr = xhq[m // 4][l, 4 + m % 4, i, 16 * gg:16 * gg + 8, :]
                    hi = xhq[m // 4][l, 4 + m % 4, i, 16 * gg + 8:16 * gg + 16, :]
                    hm = (hr + hi, hr, hi)
                    for da in range(n):
                        jx = a0 + da - m
                        if jx < 0:
                            continue
                        if jx not in xs:
                            xr = xhq[jx // 4][l, jx % 4, i, 16 * gg:16 * gg + 8, :]
                            xi = xhq[jx // 4][l, jx % 4, i, 16 * gg + 8:16 * gg + 16, :]
                            xs[jx] = (xr + xi, xr, xi)
                        for c in range(3):
                            p = xs[jx][c] * hm[c]
                            acc[da][c] = p if acc[da][c] is None else acc[da][c] + p
                for da in range(n):
                    s3, s1, s2 = acc[da]
                    re = s1 - s2
                    im = s3 - (s1 + s2)
                    if a0 + da == 0:
                        ore, oim = re, im
                    else:
                        ore, oim = re - pi, im + pr
                    yfv[da][y0:y0 + 8, ls] = pltpu.bitcast(
                        jnp.concatenate([ore, oim], axis=0).astype(BF), U32)
                    pr, pi = re, im
                if a0 + n < NB:
                    qp[i, 0, y0:y0 + 8, ls] = pr
                    qp[i, 1, y0:y0 + 8, ls] = pi
                if hops is not None:
                    v = oim
                    for _ in range(hops):
                        v = jnp.tanh(v)
                    link(v)

    def stage_c(q, i, ls=slice(None)):
        r0 = _mo((4 * q + i) * BLK, BLK)
        for hh in range(2):
            yf = yfq[q][pl.ds(_mo(i * BLK + 64 * hh, 64), 64), ls]
            g = pltpu.bitcast(dft[BLK + 64 * hh:BLK + 64 * (hh + 1), :], BF)
            yb[hh, pl.ds(r0, BLK), ls] = jnp.dot(g, pltpu.bitcast(yf, BF),
                                                 preferred_element_type=F32)

    def unit_b(a0, lane):
        for i in range(4):
            stage_b(a0, 2, i, [lane], HOPS)

    def unit_c(a0, lane):
        ls = pl.ds(_mo(lane * 128, 128), 128)
        for i in range(2):
            stage_c(3, a0 % 4 + i, ls)

    def phase(p):
        nb = 2 if str(p) in DBL else 1

        def body(ii, carry):
            t0 = 4 * p + nb * ii + 1
            for u in range(nb):
                t = t0 + u
                if p < 3 or u < nb - 1:
                    wait_block(t)
                else:
                    @pl.when(t < NB)
                    def _():
                        wait_block(jnp.minimum(t, NB - 1))
            kvw = kvb.at[pl.ds(pl.multiple_of(t0 * 64, 64), 64 * (nb + 1))]
            hpw = hp.at[pl.ds(t0, nb + 1)]
            for u in range(nb):
                i = nb * ii + u
                t = t0 + u
                kvv = kvw.at[pl.ds(64 * u, 128)]
                hpv = hpw.at[pl.ds(u, 2)]
                stage_a(p, i, kvv, hpv)
                if p >= 2:
                    stage_c(p - 2, i)
                stage_v(jnp.minimum(t, NB - 1) if p == 3 else t, kvv, hpv)
                if p >= 1:
                    stage_b(4 * (p - 1), 4, i, all_lanes, None)
            return carry
        with jax.named_scope("p%d" % p):
            lax.fori_loop(0, 4 // nb, body, 0)

    with jax.named_scope("w0"):
        wait_block(0)
    with jax.named_scope("v0"):
        stage_v(jnp.int32(0), kvb.at[pl.ds(0, 128)], hp.at[pl.ds(0, 2)])
        dft_cp.wait()
    phase(0)
    for c_ in small:
        c_.wait()
    dvec = jnp.broadcast_to(dvb[...].astype(F32).reshape(1, D), (8, D))
    for g in range(NG):
        a, r = g // 4, 16 * (g % 4)
        for l in range(NL):
            xh0[l, 4, a, r:r + 8, :] = xh0[l, 4, a, r:r + 8, :] + dvec[:, 128 * l:128 * (l + 1)]
    for p in range(1, 4):
        phase(p)

    c = cb_[...].astype(F32)
    sc = jnp.broadcast_to((c * jax.nn.sigmoid(c)).astype(BF), (16, D))
    b1 = b1b[...].astype(F32).reshape(1, F)
    b2 = b2b[...].astype(F32).reshape(1, D)

    b1c[...] = jnp.broadcast_to(b1[:, F - 128:F], (128, 128)).T[64:128, :]

    def mod_chunk(n):
        m = jnp.dot(sc, wmb[n], preferred_element_type=F32)[0:8]
        modb[n] = m + 1.0 if n in (1, 4) else m

    def mods(ns):
        return [jnp.concatenate([modb[n]] * 2, axis=0) for n in ns]

    def prep1(i, grp):
        ra = i * TM + zs[0] * 16
        xs = [qb[pl.ds(pl.multiple_of(ra + 16 * rc, 16), 16), :] for rc in grp]
        return [_stats(x.astype(F32)) for x in xs]

    def prep2(i, grp, st1, x1v, xoff):
        rb = i * TM + zs[1] * 16
        st2 = []
        for rc, (m, rs) in zip(grp, st1):
            r = pl.multiple_of(rb + 16 * rc, 16)
            sa, ca = mods((0, 1))
            x = qb[pl.ds(r, 16), :].astype(F32)
            ry = _mo(i * TM + 16 * rc, 16)
            x1 = x + (((x - m) * rs) * ca + sa) * (yb[0, pl.ds(ry, 16), :] + yb[1, pl.ds(ry, 16), :])
            x1v[xoff + 16 * rc:xoff + 16 * rc + 16, :] = x1
            st2.append(_stats(x1))
        return st2

    def prep3(i, grp, st2, h2v, hoff, chain):
        rc_ = i * TM + zs[2] * 16
        for n, (rc, (m, rs)) in enumerate(zip(grp, st2)):
            sb, cb = mods((3, 4))
            x1 = x1r[pl.ds(pl.multiple_of(rc_ + 16 * rc, 16), 16), :]
            h2 = ((x1 - m) * rs) * cb + sb
            h2v[hoff + 8 * rc:hoff + 8 * rc + 8, :] = pltpu.bitcast(h2.astype(BF), U32)
            if chain == 1:
                qb[S:S + 8, 128 * n:128 * (n + 1)] = h2[8:16, D - 128:D].astype(BF)
            elif chain == 2:
                xh3[zs[3], 8, 1, 8 * n:8 * n + 8, :] = h2[8:16, D - 128:D]

    def prep(i, h2v, hoff, x1v, xoff, link_n):
        for g0 in range(0, TM // 16, link_n):
            grp = range(g0, g0 + link_n)
            st2 = prep2(i, grp, prep1(i, grp), x1v, xoff)
            prep3(i, grp, st2, h2v, hoff, 1 if g0 + link_n < TM // 16 else 2)

    def o_cp(i, lo=0, hi=TM):
        r0 = _mo(i * TM + lo, 16)
        return cp(ob.at[pl.ds(r0, hi - lo)], o_hbm.at[0, pl.ds(r0, hi - lo)],
                  sem_o.at[i + (1 if lo else 0)])

    def mm1(h2v, hoff, gv, goff, rows, f0, f1):
        h2 = pltpu.bitcast(h2v[hoff:hoff + rows // 2, :], BF)
        if HALF and f1 == F:
            st = lax.dot_general(w1b[FH:F, :], h2, NT, preferred_element_type=F32)
            st = _gelu(st + jnp.concatenate([b1c[...]] * (rows // 128), axis=1))
            gv[goff:goff + rows // 2, FH:F] = pltpu.bitcast(st.T.astype(BF), U32)
            f1 = FH
        g = lax.dot_general(h2, w1b[f0:f1, :], NT, preferred_element_type=F32) + b1[:, f0:f1]
        gv[goff:goff + rows // 2, f0:f1] = pltpu.bitcast(_gelu(g).astype(BF), U32)

    def mm2(i, gv, goff, x1v, xoff, lo=0, hi=TM):
        r0 = _mo(i * TM + lo, 16)
        gb = modb[5][0:1]
        o = jnp.dot(pltpu.bitcast(gv[goff + lo // 2:goff + hi // 2, :], BF), w2b[...],
                    preferred_element_type=F32) + b2
        ob[pl.ds(r0, hi - lo), :] = (x1v[xoff + lo:xoff + hi, :] + gb * o).astype(BF)
        o_cp(i, lo, hi).start()

    allg = range(TM // 16)
    with jax.named_scope("p4"):
        q_cp(0).wait()
        if VAR == 'b':
            q_cp(1).wait()
        for n in range(3):
            wm_cp(n).wait()
        for i in range(4):
            stage_c(2, i)
        m_ = [jnp.dot(sc, wmb[n], preferred_element_type=F32)[0:8] for n in range(3)]
        modb[0] = m_[0] * m_[2]
        modb[1] = (m_[1] + 1.0) * m_[2]
        for i in range(4):
            stage_b(12, 2, i, [0], None)
        st1 = prep1(0, allg)
        if VAR == 'b':
            st1b = prep1(1, allg)
    with jax.named_scope("p5"):
        wm_cp(3).wait()
        mod_chunk(3)
        st2 = prep2(0, allg, st1, x1r, 0)
    with jax.named_scope("p6"):
        wm_cp(4).wait()
        mod_chunk(4)
        prep3(0, allg, st2, h2r, 0, 0)
    with jax.named_scope("firstA"):
        w1a_cp.wait()
        if VAR != 'b':
            q_cp(1).wait()
            st1b = prep1(1, allg)
        mm1(h2r, 0, gr, 0, TM, 0, F0)
        st2 = prep2(1, allg, st1b, x1r, TM)
        prep3(1, allg, st2, h2r, TH, 0)
        mm1(h2r, TH, gr, TH, TM, 0, F0)
    with jax.named_scope("firstB"):
        w1b_cp.wait()
        unit_c(12, 0)
        mm1(h2r, 0, gr, 0, 2 * TM, F0, F)
    with jax.named_scope("w2wait"):
        w2_cp.wait()
        wm_cp(5).wait()
        mod_chunk(5)

    def step(k, units):
        if isinstance(k, int):
            x1v, xo, gv, go = x1r, (k - 2) * TM, gr, (k - 2) * TH
        else:
            x1v = x1r.at[pl.ds(pl.multiple_of((k - 2) * TM, TM), 3 * TM)]
            gv = gr.at[pl.ds(pl.multiple_of((k - 2) * TH, TH), 3 * TH)]
            xo = go = 0
        if not (MERGE and isinstance(k, int)):
            q_cp(k).wait()
        mm2(k - 2, gv, go, x1v, xo)
        prep(k, h2r, 0, x1v, xo + 2 * TM, LINK)
        for a0, lane in units:
            unit_b(a0, lane)
        mm1(h2r, 0, gv, go + 2 * TH, TM, 0, F)
        for a0, lane in units:
            unit_c(a0, lane)

    def body(k, carry):
        step(k, [(12, k - 1), (14, k - 2)])
        return carry

    with jax.named_scope("mloop"):
        lax.fori_loop(2, 6, body, 0)
    with jax.named_scope("mtail"):
        if MERGE:
            q_cp(6).wait()
            q_cp(7).wait()
        step(6, [(14, NL - 1)])
        step(7, [])
        mm2(6, gr, 6 * TH, x1r, 6 * TM)
        if TAILR:
            mm2(7, gr, 7 * TH, x1r, 7 * TM, 0, TM - TAILR)
            mm2(7, gr, 7 * TH, x1r, 7 * TM, TM - TAILR, TM)
        else:
            mm2(7, gr, 7 * TH, x1r, 7 * TM)
    with jax.named_scope("owait"):
        for i in range(NS - 1):
            o_cp(i).wait()
        if TAILR:
            o_cp(NS - 1, 0, TM - TAILR).wait()
            o_cp(NS - 1, TM - TAILR, TM).wait()
        else:
            o_cp(NS - 1).wait()


@jax.jit
def pallas_adaLN_cond__ssm_conv_h3__dense_activation_gelu__prompt_kernel(
    A_q, A_k, A_v, A_shift_k, A_ssm_k, A_ssm_D, B_x, B_w1, B_b1, B_w2, B_b2, c, w_mod,
):
    del B_x
    any_spec = pl.BlockSpec(memory_space=pl.ANY)
    scratch = [
        pltpu.VMEM((S + 16, D), BF),
        pltpu.VMEM((S, D), BF),
        pltpu.VMEM((S, D), BF),
        pltpu.VMEM((NB, D, BLK), BF),
        pltpu.VMEM((6, D, D), BF),
        pltpu.VMEM((F, D), BF),
        pltpu.VMEM((F, D), BF),
        pltpu.VMEM((S, D), BF),
        pltpu.VMEM((4, D), BF),
        pltpu.VMEM((D,), BF),
        pltpu.VMEM((F,), BF),
        pltpu.VMEM((D,), BF),
        pltpu.VMEM((1, D), BF),
        pltpu.VMEM((2 * BLK, BLK), U32),
        pltpu.VMEM((NL, S + 8, 128), F32),
        pltpu.VMEM((4, 8, D), F32),
        pltpu.VMEM(((NB + 2) * 64, D), U32),
        pltpu.VMEM((NB + 2, D // 2, BLK), U32),
    ] + [pltpu.VMEM((NL, 9, 4, 64, 128), F32)] * 4 + [pltpu.VMEM((4 * BLK, D), U32)] * 4 + [
        pltpu.VMEM((4, 2, 32, D), F32),
        pltpu.VMEM((2, S, D), F32),
        pltpu.VMEM((6, 8, D), F32),
        pltpu.VMEM((TM, D), U32),
        pltpu.VMEM((S, D), F32),
        pltpu.VMEM((S // 2, F), U32),
        pltpu.VMEM((64, 128), F32),
        pltpu.SMEM((8,), jnp.int32),
        pltpu.SemaphoreType.DMA((3 * NB + 6 + NS + 9,)),
        pltpu.SemaphoreType.DMA((NS + 1,)),
    ]
    return pl.pallas_call(
        _kernel,
        in_specs=[any_spec] * 13,
        out_specs=any_spec,
        out_shape=jax.ShapeDtypeStruct((1, S, D), BF),
        scratch_shapes=scratch,
        compiler_params=pltpu.CompilerParams(vmem_limit_bytes=110 * 1024 * 1024),
    )(A_q, A_k, A_v, A_shift_k.T, A_ssm_k, A_ssm_D, B_w1.T, B_b1, B_w2, B_b2, c, w_mod,
      jnp.asarray(_dft_mats()))
```

```python
import numpy as np
import jax
import jax.numpy as jnp
from jax import lax
import jax.experimental.pallas as pl
import jax.experimental.pallas.tpu as pltpu

S = 2048
D = 640
F = 1728
BLK = 128
NB = S // BLK
NG = BLK // 8
NL = D // 128
TM = 256
TH = TM // 2
NS = S // TM
F0 = 512
EPS = 1e-5
BF = jnp.bfloat16
F32 = jnp.float32
U32 = jnp.uint32
LINK = 2
NACC = 2
HOPS = 8
HOPSB = 16
MUL4 = 0
L0 = 'p4'
SPLIT = 0
FM = 1280
DBL = 'x'
MERGE = 1
TAILR = 32
HALF = 1
FH = 1664
C0 = 'a'
VAR = 'b'
NT = (((1,), (1,)), ((), ()))


def _pack_rows(a):
    u = np.ascontiguousarray(a, dtype=np.float32).view(np.uint32)
    u = (u + 0x7FFF + ((u >> 16) & 1)) >> 16
    return (u[0::2] | (u[1::2] << 16)).astype(np.uint32)


def _dft_mats():
    n = 2 * BLK
    th = 2.0 * np.arange(BLK) + 0.5
    t = np.arange(BLK)
    ang = 2.0 * np.pi * th[:, None] * t[None, :] / n
    re, im = np.cos(ang), -np.sin(ang)
    fx = np.zeros((2 * BLK, BLK))
    inv = np.zeros((BLK, n))
    for g in range(NG):
        r, i = re[8 * g:8 * g + 8], im[8 * g:8 * g + 8]
        fx[16 * g:16 * g + 8] = r
        fx[16 * g + 8:16 * g + 16] = i
        inv[:, 16 * g:16 * g + 8] = (2.0 / n) * r.T
        inv[:, 16 * g + 8:16 * g + 16] = (2.0 / n) * i.T
    inv = _pack_rows(inv)
    return np.concatenate([_pack_rows(fx), inv[:, :BLK], inv[:, BLK:]], axis=0)


def _gelu(x):
    c0 = 0.7978845608028654
    u = x * (c0 + (c0 * 0.044715) * (x * x))
    hx = 0.5 * x
    return hx + hx * jnp.tanh(u)


def _stats(x):
    m = jnp.sum(x, axis=-1, keepdims=True) * (1.0 / D)
    m2 = jnp.sum(x * x, axis=-1, keepdims=True) * (1.0 / D)
    return m, lax.rsqrt(jnp.maximum(m2 - m * m, 0.0) + EPS)


def _mo(v, n):
    return v if isinstance(v, int) else pl.multiple_of(v, n)


def _kernel(q_hbm, k_hbm, v_hbm, sh_hbm, h_hbm, dv_hbm, w1_hbm, b1_hbm, w2_hbm,
            b2_hbm, c_hbm, wm_hbm, dft_hbm, o_hbm,
            qb, kb, vb, hb, wmb, w1b, w2b, ob, shb, dvb, b1b, b2b, cb_, dft,
            kf, wb, kvb, hp, xh0, xh1, xh2, xh3, yf0, yf1, yf2, yf3,
            qp, yb, modb, h2r, x1r, gr, b1c, w1p, zs, sem, sem_o):
    xhq = (xh0, xh1, xh2, xh3)
    yfq = (yf0, yf1, yf2, yf3)
    cp = pltpu.make_async_copy
    n0 = 3 * NB

    def k_cp(j):
        return cp(k_hbm.at[0, pl.ds(BLK * j, BLK)], kb.at[pl.ds(BLK * j, BLK)], sem.at[3 * j])

    def v_cp(j):
        return cp(v_hbm.at[0, pl.ds(BLK * j, BLK)], vb.at[pl.ds(BLK * j, BLK)], sem.at[3 * j + 1])

    def h_cp(j):
        return cp(h_hbm.at[:, pl.ds(BLK * j, BLK)], hb.at[j], sem.at[3 * j + 2])

    def wm_cp(n):
        return cp(wm_hbm.at[:, pl.ds(D * n, D)], wmb.at[n], sem.at[n0 + n])

    def q_cp(i):
        r0 = _mo(i * TM, TM)
        return cp(q_hbm.at[0, pl.ds(r0, TM)], qb.at[pl.ds(r0, TM)], sem.at[n0 + 6 + i])

    n1 = n0 + 6 + NS
    w1a_cp = cp(w1_hbm.at[pl.ds(0, F0)], w1b.at[pl.ds(0, F0)], sem.at[n1])
    w1b_cp = cp(w1_hbm.at[pl.ds(F0, F - F0)], w1b.at[pl.ds(F0, F - F0)], sem.at[n1 + 1])
    w2_cp = cp(w2_hbm, w2b, sem.at[n1 + 2])
    sh_cp = cp(sh_hbm, shb, sem.at[n1 + 3])
    dft_cp = cp(dft_hbm, dft, sem.at[n1 + 4])
    small = [cp(dv_hbm, dvb, sem.at[n1 + 5]), cp(c_hbm, cb_, sem.at[n1 + 6]),
             cp(b1_hbm, b1b, sem.at[n1 + 7]), cp(b2_hbm, b2b, sem.at[n1 + 8])]

    sh_cp.start()
    for j in range(NB):
        k_cp(j).start()
        v_cp(j).start()
        h_cp(j).start()
        if j == 0:
            dft_cp.start()
        if j == 1:
            for c_ in small:
                c_.start()
    q_cp(0).start()
    if VAR == 'b':
        q_cp(1).start()
    for n in range(5):
        wm_cp(n).start()
    w1a_cp.start()
    if VAR != 'b':
        q_cp(1).start()
    w1b_cp.start()
    w2_cp.start()
    wm_cp(5).start()
    for i in range(2, NS):
        q_cp(i).start()

    for n in range(4):
        zs[n] = 0
    kf[:, 0:8, :] = jnp.zeros((NL, 8, 128), F32)
    sh_cp.wait()
    sh = shb[...].astype(F32)
    for t in range(4):
        wb[t] = jnp.broadcast_to(sh[t:t + 1, :], (8, D))

    def wait_block(j):
        k_cp(j).wait()
        v_cp(j).wait()
        h_cp(j).wait()

    def v_tile(j, l, dst, row0, lane0):
        ls = pl.ds(_mo(128 * l, 128), 128)
        w = [jnp.concatenate([wb[t, :, ls]] * 2, axis=0) for t in range(4)]
        for rc in range(BLK // 16):
            r = _mo(j * BLK + 16 * rc, 16)
            k = kb[pl.ds(r, 16), ls].astype(F32)
            v = vb[pl.ds(r, 16), ls].astype(F32)
            kf[l, pl.ds(r + 8, 16), :] = k
            ks = k * w[0]
            for t in range(1, 4):
                ks = ks + kf[l, pl.ds(j * BLK + 16 * rc + (8 - t), 16), :] * w[t]
            dst[row0 + 8 * rc:row0 + 8 * rc + 8, lane0:lane0 + 128] = pltpu.bitcast(
                (ks * v).astype(BF), U32)

    def stage_v(j, kvv, hpv):
        for l in range(NL):
            v_tile(j, l, kvv, 64, 128 * l)
        hpv[1, 0:D // 2, :] = pltpu.bitcast(hb[j], U32)

    def stage_v_lane(l, kvl, hpl, off):
        for j in range(13, NB):
            v_tile(j, l, kvl, 64 * (j + 1), 128 * off)
            hpl[j + 1, 64 * off:64 * off + 64, :] = pltpu.bitcast(
                hb[j, pl.ds(_mo(128 * l, 128), 128), :], U32)

    def stage_a(p, i, kvv, hpv):
        fx = pltpu.bitcast(dft[0:BLK, :], BF)
        xf = jnp.dot(fx, pltpu.bitcast(kvv[0:64, 0:D], BF), preferred_element_type=F32)
        for l in range(NL):
            xhq[p][l, i] = xf[:, 128 * l:128 * (l + 1)].reshape(4, 64, 128)
        hf = lax.dot_general(fx, pltpu.bitcast(hpv[0, 0:D // 2, :], BF), NT, preferred_element_type=F32)
        for l in range(NL):
            xhq[p][l, 4 + i] = hf[:, 128 * l:128 * (l + 1)].reshape(4, 64, 128)

    all_lanes = list(range(NL))

    def link(v):
        for q in range(4):
            xhq[q][zs[3], 8, 0, 0:8, :] = v

    def stage_b(a0, n, i, lanes, hops, yov=None):
        q = a0 // 4
        yref = yfq[q] if yov is None else yov
        yfv = [yref.at[pl.ds(_mo(32 * i + BLK * ((a0 + da) % 4), 32), 32)] for da in range(n)]
        for gg in range(4):
            y0 = 8 * gg
            for l in lanes:
                ls = pl.ds(_mo(128 * l, 128), 128)
                if a0 > 0:
                    pr = qp[i, 0, y0:y0 + 8, ls]
                    pi = qp[i, 1, y0:y0 + 8, ls]
                acc = [[None] * 3 for _ in range(n)]
                xs = {}
                for m in range(a0 + n):
                    hr = xhq[m // 4][l, 4 + m % 4, i, 16 * gg:16 * gg + 8, :]
                    hi = xhq[m // 4][l, 4 + m % 4, i, 16 * gg + 8:16 * gg + 16, :]
                    hm = (hr + hi, hr, hi)
                    for da in range(n):
                        jx = a0 + da - m
                        if jx < 0:
                            continue
                        if jx not in xs:
                            xr = xhq[jx // 4][l, jx % 4, i, 16 * gg:16 * gg + 8, :]
                            xi = xhq[jx // 4][l, jx % 4, i, 16 * gg + 8:16 * gg + 16, :]
                            xs[jx] = (xr + xi, xr, xi)
                        for c in range(3):
                            p = xs[jx][c] * hm[c]
                            acc[da][c] = p if acc[da][c] is None else acc[da][c] + p
                for da in range(n):
                    s3, s1, s2 = acc[da]
                    re = s1 - s2
                    im = s3 - (s1 + s2)
                    if a0 + da == 0:
                        ore, oim = re, im
                    else:
                        ore, oim = re - pi, im + pr
                    yfv[da][y0:y0 + 8, ls if yov is None else slice(128, 256)] = pltpu.bitcast(
                        jnp.concatenate([ore, oim], axis=0).astype(BF), U32)
                    pr, pi = re, im
                if a0 + n < NB:
                    qp[i, 0, y0:y0 + 8, ls] = pr
                    qp[i, 1, y0:y0 + 8, ls] = pi
                if hops is not None:
                    v = oim
                    for _ in range(hops):
                        v = jnp.tanh(v)
                    link(v)

    def stage_c(q, i, ls=slice(None), yov=None, hs=(0, 1)):
        r0 = _mo((4 * q + i) * BLK, BLK)
        for hh in hs:
            if yov is None:
                yf = yfq[q][pl.ds(_mo(i * BLK + 64 * hh, 64), 64), ls]
            else:
                yf = yov[i * BLK + 64 * hh:i * BLK + 64 * hh + 64, 0:128]
            g = pltpu.bitcast(dft[BLK + 64 * hh:BLK + 64 * (hh + 1), :], BF)
            yb[hh, pl.ds(r0, BLK), ls] = jnp.dot(g, pltpu.bitcast(yf, BF),
                                                 preferred_element_type=F32)

    def unit_b(a0, lane):
        for i in range(4):
            stage_b(a0, 2, i, [lane], HOPS)

    def unit_c(a0, lane):
        ls = pl.ds(_mo(lane * 128, 128), 128)
        for i in range(2):
            stage_c(3, a0 % 4 + i, ls)

    def phase(p):
        def body(i, carry):
            t = 4 * p + i + 1
            wait_block(t)
            kvv = kvb.at[pl.ds(pl.multiple_of(t * 64, 64), 128)]
            hpv = hp.at[pl.ds(t, 2)]
            stage_a(p, i, kvv, hpv)
            if p == 2:
                stage_c(0, i, hs=(0, 1) if C0 == 'a' else (0,))
            stage_v(t, kvv, hpv)
            if p >= 1:
                stage_b(4 * (p - 1), 4, i, all_lanes, None)
            return carry
        with jax.named_scope("p%d" % p):
            lax.fori_loop(0, 4, body, 0)

    def phase3():
        def body(l, carry):
            ls = pl.ds(pl.multiple_of(l * 128, 128), 128)
            kvl = kvb.at[:, pl.ds(pl.multiple_of(l * 128, 128), 256)]
            hpl = hp.at[:, pl.ds(pl.multiple_of(l * 64, 64), 128)]
            yov = yf2.at[:, pl.ds(pl.multiple_of(l * 128, 128), 256)]
            fx = pltpu.bitcast(dft[0:BLK, :], BF)
            for j in range(12, NB):
                kv = pltpu.bitcast(kvl[64 * (j + 1):64 * (j + 2), 0:128], BF)
                xh3[l, j - 12] = jnp.dot(fx, kv, preferred_element_type=F32).reshape(4, 64, 128)
                hm = pltpu.bitcast(hpl[j + 1, 0:64, :], BF)
                xh3[l, j - 8] = lax.dot_general(
                    fx, hm, NT, preferred_element_type=F32).reshape(4, 64, 128)
            for i in range(4):
                if C0 == 'b':
                    stage_c(0, i, ls, hs=(1,))
                stage_c(1, i, ls)
            lp = pl.ds(pl.multiple_of(jnp.maximum(l - 1, 0) * 128, 128), 128)
            for i in range(4):
                stage_c(2, i, lp, yov)
            stage_v_lane(jnp.minimum(l + 1, NL - 1), kvl, hpl, 1)
            for i in range(4):
                stage_b(8, 4, i, [l], None, yov)
            return carry
        with jax.named_scope("p3a"):
            for j in range(13, NB):
                wait_block(j)
            stage_v_lane(0, kvb, hp, 0)
        with jax.named_scope("p3"):
            lax.fori_loop(0, NL, body, 0)

    with jax.named_scope("w0"):
        wait_block(0)
    with jax.named_scope("v0"):
        stage_v(jnp.int32(0), kvb.at[pl.ds(0, 128)], hp.at[pl.ds(0, 2)])
        dft_cp.wait()
    phase(0)
    for c_ in small:
        c_.wait()
    dvec = jnp.broadcast_to(dvb[...].astype(F32).reshape(1, D), (8, D))
    for g in range(NG):
        a, r = g // 4, 16 * (g % 4)
        for l in range(NL):
            xh0[l, 4, a, r:r + 8, :] = xh0[l, 4, a, r:r + 8, :] + dvec[:, 128 * l:128 * (l + 1)]
    yf2[:, 0:128] = jnp.zeros((4 * BLK, 128), U32)
    for p in range(1, 3):
        phase(p)
    phase3()

    c = cb_[...].astype(F32)
    sc = jnp.broadcast_to((c * jax.nn.sigmoid(c)).astype(BF), (16, D))
    b1 = b1b[...].astype(F32).reshape(1, F)
    b2 = b2b[...].astype(F32).reshape(1, D)

    b1c[...] = jnp.broadcast_to(b1[:, F - 128:F], (128, 128)).T[64:128, :]

    def mod_chunk(n):
        m = jnp.dot(sc, wmb[n], preferred_element_type=F32)[0:8]
        modb[n] = m + 1.0 if n in (1, 4) else m

    def mods(ns):
        return [jnp.concatenate([modb[n]] * 2, axis=0) for n in ns]

    def prep1(i, grp):
        ra = i * TM + zs[0] * 16
        xs = [qb[pl.ds(pl.multiple_of(ra + 16 * rc, 16), 16), :] for rc in grp]
        return [_stats(x.astype(F32)) for x in xs]

    def prep2(i, grp, st1, x1v, xoff):
        rb = i * TM + zs[1] * 16
        st2 = []
        for rc, (m, rs) in zip(grp, st1):
            r = pl.multiple_of(rb + 16 * rc, 16)
            sa, ca = mods((0, 1))
            x = qb[pl.ds(r, 16), :].astype(F32)
            ry = _mo(i * TM + 16 * rc, 16)
            x1 = x + (((x - m) * rs) * ca + sa) * (yb[0, pl.ds(ry, 16), :] + yb[1, pl.ds(ry, 16), :])
            x1v[xoff + 16 * rc:xoff + 16 * rc + 16, :] = x1
            st2.append(_stats(x1))
        return st2

    def prep3(i, grp, st2, h2v, hoff, chain):
        rc_ = i * TM + zs[2] * 16
        for n, (rc, (m, rs)) in enumerate(zip(grp, st2)):
            sb, cb = mods((3, 4))
            x1 = x1r[pl.ds(pl.multiple_of(rc_ + 16 * rc, 16), 16), :]
            h2 = ((x1 - m) * rs) * cb + sb
            h2v[hoff + 8 * rc:hoff + 8 * rc + 8, :] = pltpu.bitcast(h2.astype(BF), U32)
            if chain == 1:
                qb[S:S + 8, 128 * n:128 * (n + 1)] = h2[8:16, D - 128:D].astype(BF)
            elif chain == 2:
                xh3[zs[3], 8, 1, 8 * n:8 * n + 8, :] = h2[8:16, D - 128:D]

    def prep(i, h2v, hoff, x1v, xoff, link_n):
        for g0 in range(0, TM // 16, link_n):
            grp = range(g0, g0 + link_n)
            st2 = prep2(i, grp, prep1(i, grp), x1v, xoff)
            prep3(i, grp, st2, h2v, hoff, 1 if g0 + link_n < TM // 16 else 2)

    def o_cp(i, lo=0, hi=TM):
        r0 = _mo(i * TM + lo, 16)
        return cp(ob.at[pl.ds(r0, hi - lo)], o_hbm.at[0, pl.ds(r0, hi - lo)],
                  sem_o.at[i + (1 if lo else 0)])

    def w1(f0, f1, mode):
        if mode == 'p':
            return pltpu.bitcast(w1p[f0 // 2:f1 // 2, :], BF)
        w = w1b[f0:f1, :]
        if mode == 's':
            w1p[f0 // 2:f1 // 2, :] = pltpu.bitcast(w, U32)
        return w

    def mm1(h2v, hoff, gv, goff, rows, f0, f1, mode='p'):
        h2 = pltpu.bitcast(h2v[hoff:hoff + rows // 2, :], BF)
        if HALF and f1 == F:
            st = lax.dot_general(w1(FH, F, mode), h2, NT, preferred_element_type=F32)
            st = _gelu(st + jnp.concatenate([b1c[...]] * (rows // 128), axis=1))
            gv[goff:goff + rows // 2, FH:F] = pltpu.bitcast(st.T.astype(BF), U32)
            f1 = FH
        g = lax.dot_general(h2, w1(f0, f1, mode), NT, preferred_element_type=F32) + b1[:, f0:f1]
        gv[goff:goff + rows // 2, f0:f1] = pltpu.bitcast(_gelu(g).astype(BF), U32)

    def mm2(i, gv, goff, x1v, xoff, lo=0, hi=TM):
        r0 = _mo(i * TM + lo, 16)
        gb = modb[5][0:1]
        o = jnp.dot(pltpu.bitcast(gv[goff + lo // 2:goff + hi // 2, :], BF), w2b[...],
                    preferred_element_type=F32) + b2
        ob[pl.ds(r0, hi - lo), :] = (x1v[xoff + lo:xoff + hi, :] + gb * o).astype(BF)
        o_cp(i, lo, hi).start()

    allg = range(TM // 16)
    with jax.named_scope("p4"):
        q_cp(0).wait()
        if VAR == 'b':
            q_cp(1).wait()
        for n in range(3):
            wm_cp(n).wait()
        for i in range(4):
            stage_c(2, i, slice(D - 128, D), yf2.at[:, pl.ds(D, 128)])
        if C0 == 'c':
            for i in range(4):
                stage_c(0, i, hs=(1,))
        m_ = [jnp.dot(sc, wmb[n], preferred_element_type=F32)[0:8] for n in range(3)]
        modb[0] = m_[0] * m_[2]
        modb[1] = (m_[1] + 1.0) * m_[2]
        for i in range(4):
            stage_b(12, 2, i, [0], None)
        st1 = prep1(0, allg)
        if VAR == 'b':
            st1b = prep1(1, allg)
    with jax.named_scope("p5"):
        wm_cp(3).wait()
        mod_chunk(3)
        st2 = prep2(0, allg, st1, x1r, 0)
    with jax.named_scope("p6"):
        wm_cp(4).wait()
        mod_chunk(4)
        prep3(0, allg, st2, h2r, 0, 0)
    with jax.named_scope("firstA"):
        w1a_cp.wait()
        if VAR != 'b':
            q_cp(1).wait()
            st1b = prep1(1, allg)
        mm1(h2r, 0, gr, 0, TM, 0, F0, 's')
        st2 = prep2(1, allg, st1b, x1r, TM)
        prep3(1, allg, st2, h2r, TH, 0)
        mm1(h2r, TH, gr, TH, TM, 0, F0, 'r')
    with jax.named_scope("firstB"):
        w1b_cp.wait()
        unit_c(12, 0)
        mm1(h2r, 0, gr, 0, 2 * TM, F0, F, 's')
    with jax.named_scope("w2wait"):
        w2_cp.wait()
        wm_cp(5).wait()
        mod_chunk(5)

    def step(k, units):
        if isinstance(k, int):
            x1v, xo, gv, go = x1r, (k - 2) * TM, gr, (k - 2) * TH
        else:
            x1v = x1r.at[pl.ds(pl.multiple_of((k - 2) * TM, TM), 3 * TM)]
            gv = gr.at[pl.ds(pl.multiple_of((k - 2) * TH, TH), 3 * TH)]
            xo = go = 0
        if not (MERGE and isinstance(k, int)):
            q_cp(k).wait()
        mm2(k - 2, gv, go, x1v, xo)
        prep(k, h2r, 0, x1v, xo + 2 * TM, LINK)
        for a0, lane in units:
            unit_b(a0, lane)
        mm1(h2r, 0, gv, go + 2 * TH, TM, 0, F)
        for a0, lane in units:
            unit_c(a0, lane)

    def body(k, carry):
        step(k, [(12, k - 1), (14, k - 2)])
        return carry

    with jax.named_scope("mloop"):
        lax.fori_loop(2, 6, body, 0)
    with jax.named_scope("mtail"):
        if MERGE:
            q_cp(6).wait()
            q_cp(7).wait()
        step(6, [(14, NL - 1)])
        step(7, [])
        mm2(6, gr, 6 * TH, x1r, 6 * TM)
        if TAILR:
            mm2(7, gr, 7 * TH, x1r, 7 * TM, 0, TM - TAILR)
            mm2(7, gr, 7 * TH, x1r, 7 * TM, TM - TAILR, TM)
        else:
            mm2(7, gr, 7 * TH, x1r, 7 * TM)
    with jax.named_scope("owait"):
        for i in range(NS - 1):
            o_cp(i).wait()
        if TAILR:
            o_cp(NS - 1, 0, TM - TAILR).wait()
            o_cp(NS - 1, TM - TAILR, TM).wait()
        else:
            o_cp(NS - 1).wait()


@jax.jit
def pallas_adaLN_cond__ssm_conv_h3__dense_activation_gelu__prompt_kernel(
    A_q, A_k, A_v, A_shift_k, A_ssm_k, A_ssm_D, B_x, B_w1, B_b1, B_w2, B_b2, c, w_mod,
):
    del B_x
    any_spec = pl.BlockSpec(memory_space=pl.ANY)
    scratch = [
        pltpu.VMEM((S + 16, D), BF),
        pltpu.VMEM((S, D), BF),
        pltpu.VMEM((S, D), BF),
        pltpu.VMEM((NB, D, BLK), BF),
        pltpu.VMEM((6, D, D), BF),
        pltpu.VMEM((F, D), BF),
        pltpu.VMEM((F, D), BF),
        pltpu.VMEM((S, D), BF),
        pltpu.VMEM((4, D), BF),
        pltpu.VMEM((D,), BF),
        pltpu.VMEM((F,), BF),
        pltpu.VMEM((D,), BF),
        pltpu.VMEM((1, D), BF),
        pltpu.VMEM((2 * BLK, BLK), U32),
        pltpu.VMEM((NL, S + 8, 128), F32),
        pltpu.VMEM((4, 8, D), F32),
        pltpu.VMEM(((NB + 1) * 64, D + 128), U32),
        pltpu.VMEM((NB + 1, D // 2 + 64, BLK), U32),
    ] + [pltpu.VMEM((NL, 9, 4, 64, 128), F32)] * 4 + [pltpu.VMEM((4 * BLK, D), U32)] * 2 + [pltpu.VMEM((4 * BLK, D + 128), U32), pltpu.VMEM((4 * BLK, D), U32)] + [
        pltpu.VMEM((4, 2, 32, D), F32),
        pltpu.VMEM((2, S, D), F32),
        pltpu.VMEM((6, 8, D), F32),
        pltpu.VMEM((TM, D), U32),
        pltpu.VMEM((S, D), F32),
        pltpu.VMEM((S // 2, F), U32),
        pltpu.VMEM((64, 128), F32),
        pltpu.VMEM((F // 2, D), U32),
        pltpu.SMEM((8,), jnp.int32),
        pltpu.SemaphoreType.DMA((3 * NB + 6 + NS + 9,)),
        pltpu.SemaphoreType.DMA((NS + 1,)),
    ]
    return pl.pallas_call(
        _kernel,
        in_specs=[any_spec] * 13,
        out_specs=any_spec,
        out_shape=jax.ShapeDtypeStruct((1, S, D), BF),
        scratch_shapes=scratch,
        compiler_params=pltpu.CompilerParams(vmem_limit_bytes=110 * 1024 * 1024),
    )(A_q, A_k, A_v, A_shift_k.T, A_ssm_k, A_ssm_D, B_w1.T, B_b1, B_w2, B_b2, c, w_mod,
      jnp.asarray(_dft_mats()))
```

```python
import numpy as np
import jax
import jax.numpy as jnp
from jax import lax
import jax.experimental.pallas as pl
import jax.experimental.pallas.tpu as pltpu

S = 2048
D = 640
F = 1728
BLK = 128
NB = S // BLK
NG = BLK // 8
NL = D // 128
TM = 256
TH = TM // 2
NS = S // TM
F0 = 512
EPS = 1e-5
BF = jnp.bfloat16
F32 = jnp.float32
U32 = jnp.uint32
LINK = 2
NACC = 2
HOPS = 8
HOPSB = 16
MUL4 = 0
L0 = 'p4'
SPLIT = 0
FM = 1280
DBL = 'x'
MERGE = 1
TAILR = 32
HALF = 1
FH = 1664
C0 = 'a'
DYN = ''
VAR = 'b'
NT = (((1,), (1,)), ((), ()))


def _pack_rows(a):
    u = np.ascontiguousarray(a, dtype=np.float32).view(np.uint32)
    u = (u + 0x7FFF + ((u >> 16) & 1)) >> 16
    return (u[0::2] | (u[1::2] << 16)).astype(np.uint32)


def _dft_mats():
    n = 2 * BLK
    th = 2.0 * np.arange(BLK) + 0.5
    t = np.arange(BLK)
    ang = 2.0 * np.pi * th[:, None] * t[None, :] / n
    re, im = np.cos(ang), -np.sin(ang)
    fx = np.zeros((2 * BLK, BLK))
    inv = np.zeros((BLK, n))
    for g in range(NG):
        r, i = re[8 * g:8 * g + 8], im[8 * g:8 * g + 8]
        fx[16 * g:16 * g + 8] = r
        fx[16 * g + 8:16 * g + 16] = i
        inv[:, 16 * g:16 * g + 8] = (2.0 / n) * r.T
        inv[:, 16 * g + 8:16 * g + 16] = (2.0 / n) * i.T
    inv = _pack_rows(inv)
    return np.concatenate([_pack_rows(fx), inv[:, :BLK], inv[:, BLK:]], axis=0)


def _gelu(x):
    c0 = 0.7978845608028654
    u = x * (c0 + (c0 * 0.044715) * (x * x))
    hx = 0.5 * x
    return hx + hx * jnp.tanh(u)


def _stats(x):
    m = jnp.sum(x, axis=-1, keepdims=True) * (1.0 / D)
    m2 = jnp.sum(x * x, axis=-1, keepdims=True) * (1.0 / D)
    return m, lax.rsqrt(jnp.maximum(m2 - m * m, 0.0) + EPS)


def _mo(v, n):
    return v if isinstance(v, int) else pl.multiple_of(v, n)


def _kernel(q_hbm, k_hbm, v_hbm, sh_hbm, h_hbm, dv_hbm, w1_hbm, b1_hbm, w2_hbm,
            b2_hbm, c_hbm, wm_hbm, dft_hbm, o_hbm,
            qb, kb, vb, hb, wmb, w1b, w2b, ob, dft,
            kf, wb, kvb, hp, xh0, xh1, xh2, xh3, yf0, yf1, yf2, yf3,
            qp, yb, modb, h2r, x1r, gr, b1c, w1p, b1f, b2f, dvf, scb, shb, dvb, b1b, b2b, cb_, sepb, zs, sem, sem_o):
    xhq = (xh0, xh1, xh2, xh3)
    yfq = (yf0, yf1, yf2, yf3)
    cp = pltpu.make_async_copy
    n0 = 3 * NB

    def k_cp(j):
        return cp(k_hbm.at[0, pl.ds(BLK * j, BLK)], kb.at[pl.ds(BLK * j, BLK)], sem.at[3 * j])

    def v_cp(j):
        return cp(v_hbm.at[0, pl.ds(BLK * j, BLK)], vb.at[pl.ds(BLK * j, BLK)], sem.at[3 * j + 1])

    def h_cp(j):
        return cp(h_hbm.at[:, pl.ds(BLK * j, BLK)], hb.at[j], sem.at[3 * j + 2])

    def wm_cp(n):
        return cp(wm_hbm.at[:, pl.ds(D * n, D)], wmb.at[n], sem.at[n0 + n])

    def q_cp(i):
        r0 = _mo(i * TM, TM)
        return cp(q_hbm.at[0, pl.ds(r0, TM)], qb.at[pl.ds(r0, TM)], sem.at[n0 + 6 + i])

    n1 = n0 + 6 + NS
    w1a_cp = cp(w1_hbm.at[pl.ds(0, F0)], w1b.at[pl.ds(0, F0)], sem.at[n1])
    w1b_cp = cp(w1_hbm.at[pl.ds(F0, F - F0)], w1b.at[pl.ds(F0, F - F0)], sem.at[n1 + 1])
    w2_cp = cp(w2_hbm, w2b, sem.at[n1 + 2])
    sh_cp = cp(sh_hbm, shb, sem.at[n1 + 3])
    dft_cp = cp(dft_hbm, dft, sem.at[n1 + 4])
    small = [cp(dv_hbm, dvb, sem.at[n1 + 5]), cp(c_hbm, cb_, sem.at[n1 + 6]),
             cp(b1_hbm, b1b, sem.at[n1 + 7]), cp(b2_hbm, b2b, sem.at[n1 + 8])]

    seps = [cp(c_hbm, sepb.at[n], sem.at[n1 + 9 + n]) for n in range(2)]
    sh_cp.start()
    for c_ in small:
        c_.start()
    for j in range(NB):
        k_cp(j).start()
        v_cp(j).start()
        h_cp(j).start()
        if j == 0:
            dft_cp.start()
        if j == 1:
            for c_ in seps:
                c_.start()
    for n in range(5):
        wm_cp(n).start()
        if n == 2:
            q_cp(0).start()
            q_cp(1).start()
    w1a_cp.start()
    if VAR != 'b':
        q_cp(1).start()
    w1b_cp.start()
    w2_cp.start()
    wm_cp(5).start()
    for i in range(2, NS):
        q_cp(i).start()

    for n in range(4):
        zs[n] = 0
    kf[:, 0:8, :] = jnp.zeros((NL, 8, 128), F32)
    sh_cp.wait()
    for c_ in small:
        c_.wait()
    b1 = b1b[...].astype(F32).reshape(1, F)
    b1f[0:8, :] = jnp.broadcast_to(b1, (8, F))
    b2f[0:8, :] = jnp.broadcast_to(b2b[...].astype(F32).reshape(1, D), (8, D))
    b1c[...] = jnp.broadcast_to(b1[:, F - 128:F], (128, 128)).T[64:128, :]
    c = cb_[...].astype(F32)
    scb[0:8, :] = pltpu.bitcast(
        jnp.broadcast_to(c * jax.nn.sigmoid(c), (16, D)).astype(BF), U32)
    dvf[0:8, :] = jnp.broadcast_to(dvb[...].astype(F32).reshape(1, D), (8, D))
    sh = shb[...].astype(F32)
    for t in range(4):
        wb[t] = jnp.broadcast_to(sh[t:t + 1, :], (8, D))

    def wait_block(j):
        k_cp(j).wait()
        v_cp(j).wait()
        h_cp(j).wait()

    def v_tile(j, l, dst, row0, lane0):
        ls = pl.ds(_mo(128 * l, 128), 128)
        w = [jnp.concatenate([wb[t, :, ls]] * 2, axis=0) for t in range(4)]
        for rc in range(BLK // 16):
            r = _mo(j * BLK + 16 * rc, 16)
            k = kb[pl.ds(r, 16), ls].astype(F32)
            v = vb[pl.ds(r, 16), ls].astype(F32)
            kf[l, pl.ds(r + 8, 16), :] = k
            ks = k * w[0]
            for t in range(1, 4):
                ks = ks + kf[l, pl.ds(j * BLK + 16 * rc + (8 - t), 16), :] * w[t]
            dst[row0 + 8 * rc:row0 + 8 * rc + 8, lane0:lane0 + 128] = pltpu.bitcast(
                (ks * v).astype(BF), U32)

    def stage_v(j, kvv, hpv):
        for l in range(NL):
            v_tile(j, l, kvv, 64, 128 * l)
        hpv[1, 0:D // 2, :] = pltpu.bitcast(hb[j], U32)

    def stage_v_lane(l):
        for j in range(13, NB):
            v_tile(j + zs[0], l, kvb, 64 * (j + 1), 128 * l)
            hp[j + 1, 64 * l:64 * l + 64, :] = pltpu.bitcast(
                hb[j, 128 * l:128 * (l + 1), :], U32)

    def stage_a(p, i, kvv, hpv):
        fx = pltpu.bitcast(dft[0:BLK, :], BF)
        xf = jnp.dot(fx, pltpu.bitcast(kvv[0:64, 0:D], BF), preferred_element_type=F32)
        for l in range(NL):
            xhq[p][l, i] = xf[:, 128 * l:128 * (l + 1)].reshape(4, 64, 128)
        hf = lax.dot_general(fx, pltpu.bitcast(hpv[0, 0:D // 2, :], BF), NT, preferred_element_type=F32)
        for l in range(NL):
            xhq[p][l, 4 + i] = hf[:, 128 * l:128 * (l + 1)].reshape(4, 64, 128)

    all_lanes = list(range(NL))

    def link(v):
        for q in range(4):
            xhq[q][zs[3], 8, 0, 0:8, :] = v

    def stage_b(a0, n, i, lanes, hops, yov=None):
        q = a0 // 4
        yref = yfq[q] if yov is None else yov
        yfv = [yref.at[pl.ds(_mo(32 * i + BLK * ((a0 + da) % 4), 32), 32)] for da in range(n)]
        for gg in range(4):
            y0 = 8 * gg
            for l in lanes:
                ls = pl.ds(_mo(128 * l, 128), 128)
                if a0 > 0:
                    pr = qp[i, 0, y0:y0 + 8, ls]
                    pi = qp[i, 1, y0:y0 + 8, ls]
                acc = [[None] * 3 for _ in range(n)]
                xs = {}
                for m in range(a0 + n):
                    hr = xhq[m // 4][l, 4 + m % 4, i, 16 * gg:16 * gg + 8, :]
                    hi = xhq[m // 4][l, 4 + m % 4, i, 16 * gg + 8:16 * gg + 16, :]
                    hm = (hr + hi, hr, hi)
                    for da in range(n):
                        jx = a0 + da - m
                        if jx < 0:
                            continue
                        if jx not in xs:
                            xr = xhq[jx // 4][l, jx % 4, i, 16 * gg:16 * gg + 8, :]
                            xi = xhq[jx // 4][l, jx % 4, i, 16 * gg + 8:16 * gg + 16, :]
                            xs[jx] = (xr + xi, xr, xi)
                        for c in range(3):
                            p = xs[jx][c] * hm[c]
                            acc[da][c] = p if acc[da][c] is None else acc[da][c] + p
                for da in range(n):
                    s3, s1, s2 = acc[da]
                    re = s1 - s2
                    im = s3 - (s1 + s2)
                    if a0 + da == 0:
                        ore, oim = re, im
                    else:
                        ore, oim = re - pi, im + pr
                    yfv[da][y0:y0 + 8, ls if yov is None else slice(128, 256)] = pltpu.bitcast(
                        jnp.concatenate([ore, oim], axis=0).astype(BF), U32)
                    pr, pi = re, im
                if a0 + n < NB:
                    qp[i, 0, y0:y0 + 8, ls] = pr
                    qp[i, 1, y0:y0 + 8, ls] = pi
                if hops is not None:
                    v = oim
                    for _ in range(hops):
                        v = jnp.tanh(v)
                    link(v)

    def stage_c(q, i, ls=slice(None), yov=None, hs=(0, 1)):
        r0 = _mo((4 * q + i) * BLK, BLK)
        for hh in hs:
            if yov is None:
                yf = yfq[q][pl.ds(_mo(i * BLK + 64 * hh, 64), 64), ls]
            else:
                yf = yov[i * BLK + 64 * hh:i * BLK + 64 * hh + 64, 0:128]
            g = pltpu.bitcast(dft[BLK + 64 * hh:BLK + 64 * (hh + 1), :], BF)
            yb[hh, pl.ds(r0, BLK), ls] = jnp.dot(g, pltpu.bitcast(yf, BF),
                                                 preferred_element_type=F32)

    def unit_b(a0, lane):
        for i in range(4):
            stage_b(a0, 2, i, [lane], HOPS)

    def unit_c(a0, lane):
        ls = pl.ds(_mo(lane * 128, 128), 128)
        for i in range(2):
            stage_c(3, a0 % 4 + i, ls)

    def phase(p):
        def body(i, carry):
            t = 4 * p + i + 1
            wait_block(t)
            kvv = kvb.at[pl.ds(pl.multiple_of(t * 64, 64), 128)]
            hpv = hp.at[pl.ds(t, 2)]
            stage_a(p, i, kvv, hpv)
            if p == 2:
                stage_c(0, i, hs=(0, 1) if C0 == 'a' else (0,))
            stage_v(t, kvv, hpv)
            if p >= 1:
                stage_b(4 * (p - 1), 4, i, all_lanes, None)
            return carry
        with jax.named_scope("p%d" % p):
            lax.fori_loop(0, 4, body, 0)

    with jax.named_scope("w0"):
        wait_block(0)
    with jax.named_scope("v0"):
        stage_v(jnp.int32(0), kvb.at[pl.ds(0, 128)], hp.at[pl.ds(0, 2)])
        dft_cp.wait()
    phase(0)
    dvec = dvf[0:8, :]
    for g in range(NG):
        a, r = g // 4, 16 * (g % 4)
        for l in range(NL):
            xh0[l, 4, a, r:r + 8, :] = xh0[l, 4, a, r:r + 8, :] + dvec[:, 128 * l:128 * (l + 1)]
    for p in range(1, 3):
        phase(p)

    def lane_block(l):
        ls = slice(128 * l, 128 * (l + 1))
        fx = pltpu.bitcast(dft[0:BLK, :], BF)
        for j in range(12, NB):
            kv = pltpu.bitcast(kvb[64 * (j + 1):64 * (j + 2), ls], BF)
            xh3[l, j - 12] = jnp.dot(fx, kv, preferred_element_type=F32).reshape(4, 64, 128)
            hm = pltpu.bitcast(hp[j + 1, 64 * l:64 * l + 64, :], BF)
            xh3[l, j - 8] = lax.dot_general(
                fx, hm, NT, preferred_element_type=F32).reshape(4, 64, 128)
        for i in range(4):
            stage_c(1, i, ls)
        if l > 0:
            for i in range(4):
                stage_c(2, i, slice(128 * (l - 1), 128 * l))
        if l + 1 < NL:
            stage_v_lane(l + 1)
        for i in range(4):
            stage_b(8, 4, i, [l], None)

    with jax.named_scope("p3a"):
        for j in range(13, NB):
            wait_block(j)
        stage_v_lane(0)
    with jax.named_scope("p3"):
        seps[0].wait()
        lane_block(0)
        seps[1].wait()
        lane_block(1)
        for n in range(3):
            wm_cp(n).wait()
            lane_block(2 + n)

    def mod_chunk(n):
        m = jnp.dot(pltpu.bitcast(scb[0:8, :], BF), wmb[n], preferred_element_type=F32)[0:8]
        modb[n] = m + 1.0 if n in (1, 4) else m

    def mods(ns):
        return [jnp.concatenate([modb[n]] * 2, axis=0) for n in ns]

    def prep1(i, grp):
        ra = i * TM + zs[0] * 16
        xs = [qb[pl.ds(pl.multiple_of(ra + 16 * rc, 16), 16), :] for rc in grp]
        return [_stats(x.astype(F32)) for x in xs]

    def prep2(i, grp, st1, x1v, xoff):
        rb = i * TM + zs[1] * 16
        st2 = []
        for rc, (m, rs) in zip(grp, st1):
            r = pl.multiple_of(rb + 16 * rc, 16)
            sa, ca = mods((0, 1))
            x = qb[pl.ds(r, 16), :].astype(F32)
            ry = _mo(i * TM + 16 * rc, 16)
            x1 = x + (((x - m) * rs) * ca + sa) * (yb[0, pl.ds(ry, 16), :] + yb[1, pl.ds(ry, 16), :])
            x1v[xoff + 16 * rc:xoff + 16 * rc + 16, :] = x1
            st2.append(_stats(x1))
        return st2

    def prep3(i, grp, st2, h2v, hoff, chain):
        rc_ = i * TM + zs[2] * 16
        for n, (rc, (m, rs)) in enumerate(zip(grp, st2)):
            sb, cb = mods((3, 4))
            x1 = x1r[pl.ds(pl.multiple_of(rc_ + 16 * rc, 16), 16), :]
            h2 = ((x1 - m) * rs) * cb + sb
            h2v[hoff + 8 * rc:hoff + 8 * rc + 8, :] = pltpu.bitcast(h2.astype(BF), U32)
            if chain == 1:
                qb[S:S + 8, 128 * n:128 * (n + 1)] = h2[8:16, D - 128:D].astype(BF)
            elif chain == 2:
                xh3[zs[3], 8, 1, 8 * n:8 * n + 8, :] = h2[8:16, D - 128:D]

    def prep(i, h2v, hoff, x1v, xoff, link_n):
        for g0 in range(0, TM // 16, link_n):
            grp = range(g0, g0 + link_n)
            st2 = prep2(i, grp, prep1(i, grp), x1v, xoff)
            prep3(i, grp, st2, h2v, hoff, 1 if g0 + link_n < TM // 16 else 2)

    def o_cp(i, lo=0, hi=TM):
        r0 = _mo(i * TM + lo, 16)
        return cp(ob.at[pl.ds(r0, hi - lo)], o_hbm.at[0, pl.ds(r0, hi - lo)],
                  sem_o.at[i + (1 if lo else 0)])

    def w1(f0, f1, mode):
        if mode == 'd':
            wv = w1p.at[pl.ds(pl.multiple_of(zs[1] * 32, 32), F // 2)]
            return pltpu.bitcast(wv[f0 // 2:f1 // 2, :], BF)
        if mode == 'p':
            return pltpu.bitcast(w1p[f0 // 2:f1 // 2, :], BF)
        w = w1b[f0:f1, :]
        if mode == 's':
            w1p[f0 // 2:f1 // 2, :] = pltpu.bitcast(w, U32)
        return w

    def mm1(h2v, hoff, gv, goff, rows, f0, f1, mode='p'):
        h2 = pltpu.bitcast(h2v[hoff:hoff + rows // 2, :], BF)
        if HALF and f1 == F:
            st = lax.dot_general(w1(FH, F, mode), h2, NT, preferred_element_type=F32)
            st = _gelu(st + jnp.concatenate([b1c[...]] * (rows // 128), axis=1))
            gv[goff:goff + rows // 2, FH:F] = pltpu.bitcast(st.T.astype(BF), U32)
            f1 = FH
        g = lax.dot_general(h2, w1(f0, f1, mode), NT, preferred_element_type=F32) + b1f[0:1, f0:f1]
        gv[goff:goff + rows // 2, f0:f1] = pltpu.bitcast(_gelu(g).astype(BF), U32)

    def mm2(i, gv, goff, x1v, xoff, lo=0, hi=TM):
        r0 = _mo(i * TM + lo, 16)
        gb = modb[5][0:1]
        w2v = w2b.at[pl.ds(pl.multiple_of(zs[1] * 64, 64), F)] if 'v' in DYN and not isinstance(i, int) else w2b
        o = jnp.dot(pltpu.bitcast(gv[goff + lo // 2:goff + hi // 2, :], BF), w2v[...],
                    preferred_element_type=F32) + b2f[0:1, :]
        ob[pl.ds(r0, hi - lo), :] = (x1v[xoff + lo:xoff + hi, :] + gb * o).astype(BF)
        o_cp(i, lo, hi).start()

    allg = range(TM // 16)
    with jax.named_scope("p4"):
        q_cp(0).wait()
        q_cp(1).wait()
        for i in range(4):
            stage_c(2, i, slice(D - 128, D))
        m_ = [jnp.dot(pltpu.bitcast(scb[0:8, :], BF), wmb[n], preferred_element_type=F32)[0:8] for n in range(3)]
        modb[0] = m_[0] * m_[2]
        modb[1] = (m_[1] + 1.0) * m_[2]
        for i in range(4):
            stage_b(12, 2, i, [0], None)
        st1 = prep1(0, allg)
        if VAR == 'b':
            st1b = prep1(1, allg)
    with jax.named_scope("p5"):
        wm_cp(3).wait()
        mod_chunk(3)
        st2 = prep2(0, allg, st1, x1r, 0)
    with jax.named_scope("p6"):
        wm_cp(4).wait()
        mod_chunk(4)
        prep3(0, allg, st2, h2r, 0, 0)
    with jax.named_scope("firstA"):
        w1a_cp.wait()
        if VAR != 'b':
            q_cp(1).wait()
            st1b = prep1(1, allg)
        mm1(h2r, 0, gr, 0, TM, 0, F0, 's')
        st2 = prep2(1, allg, st1b, x1r, TM)
        prep3(1, allg, st2, h2r, TH, 0)
        mm1(h2r, TH, gr, TH, TM, 0, F0, 'r')
    with jax.named_scope("firstB"):
        w1b_cp.wait()
        unit_c(12, 0)
        mm1(h2r, 0, gr, 0, 2 * TM, F0, F, 's')
    with jax.named_scope("w2wait"):
        w2_cp.wait()
        wm_cp(5).wait()
        mod_chunk(5)

    def step(k, units):
        if isinstance(k, int):
            x1v, xo, gv, go = x1r, (k - 2) * TM, gr, (k - 2) * TH
        else:
            x1v = x1r.at[pl.ds(pl.multiple_of((k - 2) * TM, TM), 3 * TM)]
            gv = gr.at[pl.ds(pl.multiple_of((k - 2) * TH, TH), 3 * TH)]
            xo = go = 0
        if not (MERGE and isinstance(k, int)):
            q_cp(k).wait()
        mm2(k - 2, gv, go, x1v, xo)
        dyn = not isinstance(k, int)
        hv = h2r.at[pl.ds(pl.multiple_of(zs[1] * 32, 32), TH)] if dyn and 'h' in DYN else h2r
        prep(k, hv, 0, x1v, xo + 2 * TM, LINK)
        for a0, lane in units:
            unit_b(a0, lane)
        mm1(hv, 0, gv, go + 2 * TH, TM, 0, F, 'd' if dyn and 'w' in DYN else 'p')
        for a0, lane in units:
            unit_c(a0, lane)

    def body(k, carry):
        step(k, [(12, k - 1), (14, k - 2)])
        return carry

    with jax.named_scope("mloop"):
        lax.fori_loop(2, 6, body, 0)
    with jax.named_scope("mtail"):
        if MERGE:
            q_cp(6).wait()
            q_cp(7).wait()
        step(6, [(14, NL - 1)])
        step(7, [])
        mm2(6, gr, 6 * TH, x1r, 6 * TM)
        if TAILR:
            mm2(7, gr, 7 * TH, x1r, 7 * TM, 0, TM - TAILR)
            mm2(7, gr, 7 * TH, x1r, 7 * TM, TM - TAILR, TM)
        else:
            mm2(7, gr, 7 * TH, x1r, 7 * TM)
    with jax.named_scope("owait"):
        for i in range(NS - 1):
            o_cp(i).wait()
        if TAILR:
            o_cp(NS - 1, 0, TM - TAILR).wait()
            o_cp(NS - 1, TM - TAILR, TM).wait()
        else:
            o_cp(NS - 1).wait()


@jax.jit
def pallas_adaLN_cond__ssm_conv_h3__dense_activation_gelu__prompt_kernel(
    A_q, A_k, A_v, A_shift_k, A_ssm_k, A_ssm_D, B_x, B_w1, B_b1, B_w2, B_b2, c, w_mod,
):
    del B_x
    any_spec = pl.BlockSpec(memory_space=pl.ANY)
    scratch = [
        pltpu.VMEM((S + 64, D), BF),
        pltpu.VMEM((S, D), BF),
        pltpu.VMEM((S, D), BF),
        pltpu.VMEM((NB, D, BLK), BF),
        pltpu.VMEM((6, D, D), BF),
        pltpu.VMEM((F, D), BF),
        pltpu.VMEM((F, D), BF),
        pltpu.VMEM((S, D), BF),
        pltpu.VMEM((2 * BLK, BLK), U32),
        pltpu.VMEM((NL, S + 32, 128), F32),
        pltpu.VMEM((4, 8, D), F32),
        pltpu.VMEM(((NB + 1) * 64, D), U32),
        pltpu.VMEM((NB + 1, D // 2, BLK), U32),
    ] + [pltpu.VMEM((NL, 9, 4, 64, 128), F32)] * 4 + [pltpu.VMEM((4 * BLK, D), U32)] * 4 + [
        pltpu.VMEM((4, 2, 32, D), F32),
        pltpu.VMEM((2, S, D), F32),
        pltpu.VMEM((8, 8, D), F32),
        pltpu.VMEM((TM, D), U32),
        pltpu.VMEM((S, D), F32),
        pltpu.VMEM((S // 2, F), U32),
        pltpu.VMEM((64, 128), F32),
        pltpu.VMEM((F // 2, D), U32),
        pltpu.VMEM((16, F), F32),
        pltpu.VMEM((32, D), F32),
        pltpu.VMEM((32, D), F32),
        pltpu.VMEM((32, D), U32),
        pltpu.VMEM((4, D), BF),
        pltpu.VMEM((D,), BF),
        pltpu.VMEM((F,), BF),
        pltpu.VMEM((D,), BF),
        pltpu.VMEM((1, D), BF),
        pltpu.VMEM((2, 1, D), BF),
        pltpu.SMEM((8,), jnp.int32),
        pltpu.SemaphoreType.DMA((3 * NB + 6 + NS + 11,)),
        pltpu.SemaphoreType.DMA((NS + 1,)),
    ]
    return pl.pallas_call(
        _kernel,
        in_specs=[any_spec] * 13,
        out_specs=any_spec,
        out_shape=jax.ShapeDtypeStruct((1, S, D), BF),
        scratch_shapes=scratch,
        compiler_params=pltpu.CompilerParams(vmem_limit_bytes=110 * 1024 * 1024),
    )(A_q, A_k, A_v, A_shift_k.T, A_ssm_k, A_ssm_D, B_w1.T, B_b1, B_w2, B_b2, c, w_mod,
      jnp.asarray(_dft_mats()))
```

```python
import numpy as np
import jax
import jax.numpy as jnp
from jax import lax
import jax.experimental.pallas as pl
import jax.experimental.pallas.tpu as pltpu

S = 2048
D = 640
F = 1728
BLK = 128
NB = S // BLK
NG = BLK // 8
NL = D // 128
TM = 256
TH = TM // 2
NS = S // TM
F0 = 512
EPS = 1e-5
BF = jnp.bfloat16
F32 = jnp.float32
U32 = jnp.uint32
LINK = 2
NACC = 2
HOPS = 8
HOPSB = 16
MUL4 = 0
L0 = 'p4'
SPLIT = 0
FM = 1280
DBL = 'x'
MERGE = 1
TAILR = 32
HALF = 1
FH = 1664
C0 = 'a'
DYN = ''
RS = 'e'
RSPL = [128, 128]
M2S = [256]
FAS = [256]
HL = 1
UNL = 0
VAR = 'b'
NT = (((1,), (1,)), ((), ()))


def _pack_rows(a):
    u = np.ascontiguousarray(a, dtype=np.float32).view(np.uint32)
    u = (u + 0x7FFF + ((u >> 16) & 1)) >> 16
    return (u[0::2] | (u[1::2] << 16)).astype(np.uint32)


def _dft_mats():
    n = 2 * BLK
    th = 2.0 * np.arange(BLK) + 0.5
    t = np.arange(BLK)
    ang = 2.0 * np.pi * th[:, None] * t[None, :] / n
    re, im = np.cos(ang), -np.sin(ang)
    fx = np.zeros((2 * BLK, BLK))
    inv = np.zeros((BLK, n))
    for g in range(NG):
        r, i = re[8 * g:8 * g + 8], im[8 * g:8 * g + 8]
        fx[16 * g:16 * g + 8] = r
        fx[16 * g + 8:16 * g + 16] = i
        inv[:, 16 * g:16 * g + 8] = (2.0 / n) * r.T
        inv[:, 16 * g + 8:16 * g + 16] = (2.0 / n) * i.T
    inv = _pack_rows(inv)
    return np.concatenate([_pack_rows(fx), inv[:, :BLK], inv[:, BLK:]], axis=0)


def _gelu(x):
    c0 = 0.7978845608028654
    u = x * (c0 + (c0 * 0.044715) * (x * x))
    return x * (1.0 + jnp.tanh(u))


def _stats(x):
    m = jnp.sum(x, axis=-1, keepdims=True) * (1.0 / D)
    m2 = jnp.sum(x * x, axis=-1, keepdims=True) * (1.0 / D)
    v = jnp.maximum(m2 - m * m, 0.0) + EPS
    if RS == 'e':
        return m, jnp.exp(-0.5 * jnp.log(v))
    return m, lax.rsqrt(v)


def _mo(v, n):
    return v if isinstance(v, int) else pl.multiple_of(v, n)


def _kernel(q_hbm, k_hbm, v_hbm, sh_hbm, h_hbm, dv_hbm, w1_hbm, b1_hbm, w2_hbm,
            b2_hbm, c_hbm, wm_hbm, dft_hbm, o_hbm,
            qb, kb, vb, hb, wmb, w1b, w2b, ob, dft,
            kf, wb, kvb, hp, xh0, xh1, xh2, xh3, yf0, yf1, yf2, yf3,
            qp, yb, modb, h2r, x1r, gr, b1c, w1p, b1f, b2f, dvf, scb, shb, dvb, b1b, b2b, cb_, sepb, zs, sem, sem_o):
    xhq = (xh0, xh1, xh2, xh3)
    yfq = (yf0, yf1, yf2, yf3)
    cp = pltpu.make_async_copy
    n0 = 3 * NB

    def k_cp(j):
        return cp(k_hbm.at[0, pl.ds(BLK * j, BLK)], kb.at[pl.ds(BLK * j, BLK)], sem.at[3 * j])

    def v_cp(j):
        return cp(v_hbm.at[0, pl.ds(BLK * j, BLK)], vb.at[pl.ds(BLK * j, BLK)], sem.at[3 * j + 1])

    def h_cp(j):
        return cp(h_hbm.at[:, pl.ds(BLK * j, BLK)], hb.at[j], sem.at[3 * j + 2])

    def wm_cp(n):
        return cp(wm_hbm.at[:, pl.ds(D * n, D)], wmb.at[n], sem.at[n0 + n])

    def q_cp(i):
        r0 = _mo(i * TM, TM)
        return cp(q_hbm.at[0, pl.ds(r0, TM)], qb.at[pl.ds(r0, TM)], sem.at[n0 + 6 + i])

    n1 = n0 + 6 + NS
    w1a_cp = cp(w1_hbm.at[pl.ds(0, F0)], w1b.at[pl.ds(0, F0)], sem.at[n1])
    w1b_cp = cp(w1_hbm.at[pl.ds(F0, F - F0)], w1b.at[pl.ds(F0, F - F0)], sem.at[n1 + 1])
    w2_cp = cp(w2_hbm, w2b, sem.at[n1 + 2])
    sh_cp = cp(sh_hbm, shb, sem.at[n1 + 3])
    dft_cp = cp(dft_hbm, dft, sem.at[n1 + 4])
    small = [cp(dv_hbm, dvb, sem.at[n1 + 5]), cp(c_hbm, cb_, sem.at[n1 + 6]),
             cp(b1_hbm, b1b, sem.at[n1 + 7]), cp(b2_hbm, b2b, sem.at[n1 + 8])]

    seps = [cp(c_hbm, sepb.at[n], sem.at[n1 + 9 + n]) for n in range(2)]
    sh_cp.start()
    for c_ in small:
        c_.start()
    for j in range(NB):
        k_cp(j).start()
        v_cp(j).start()
        h_cp(j).start()
        if j == 0:
            dft_cp.start()
        if j == 1:
            for c_ in seps:
                c_.start()
    for n in range(5):
        wm_cp(n).start()
        if n == 2:
            q_cp(0).start()
            q_cp(1).start()
    w1a_cp.start()
    if VAR != 'b':
        q_cp(1).start()
    w1b_cp.start()
    w2_cp.start()
    wm_cp(5).start()
    for i in range(2, NS):
        q_cp(i).start()

    for n in range(4):
        zs[n] = 0
    kf[:, 0:8, :] = jnp.zeros((NL, 8, 128), F32)
    sh_cp.wait()
    for c_ in small:
        c_.wait()
    b1 = b1b[...].astype(F32).reshape(1, F)
    b1f[0:8, :] = jnp.broadcast_to(b1, (8, F))
    b2f[0:8, :] = jnp.broadcast_to(2.0 * b2b[...].astype(F32).reshape(1, D), (8, D))
    b1c[...] = jnp.broadcast_to(b1[:, F - 128:F], (128, 128)).T[64:128, :]
    c = cb_[...].astype(F32)
    scb[0:8, :] = pltpu.bitcast(
        jnp.broadcast_to(c * jax.nn.sigmoid(c), (16, D)).astype(BF), U32)
    dvf[0:8, :] = jnp.broadcast_to(dvb[...].astype(F32).reshape(1, D), (8, D))
    sh = shb[...].astype(F32)
    for t in range(4):
        wb[t] = jnp.broadcast_to(sh[t:t + 1, :], (8, D))

    def wait_block(j):
        k_cp(j).wait()
        v_cp(j).wait()
        h_cp(j).wait()

    def v_tile(j, l, dst, row0, lane0):
        ls = pl.ds(_mo(128 * l, 128), 128)
        w = [jnp.concatenate([wb[t, :, ls]] * 2, axis=0) for t in range(4)]
        for rc in range(BLK // 16):
            r = _mo(j * BLK + 16 * rc, 16)
            k = kb[pl.ds(r, 16), ls].astype(F32)
            v = vb[pl.ds(r, 16), ls].astype(F32)
            kf[l, pl.ds(r + 8, 16), :] = k
            ks = k * w[0]
            for t in range(1, 4):
                ks = ks + kf[l, pl.ds(j * BLK + 16 * rc + (8 - t), 16), :] * w[t]
            dst[row0 + 8 * rc:row0 + 8 * rc + 8, lane0:lane0 + 128] = pltpu.bitcast(
                (ks * v).astype(BF), U32)

    def stage_v(j, kvv, hpv):
        for l in range(NL):
            v_tile(j, l, kvv, 64, 128 * l)
        hpv[1, 0:D // 2, :] = pltpu.bitcast(hb[j], U32)

    def stage_v_lane(l):
        for j in range(13, NB):
            v_tile(j + zs[0], l, kvb, 64 * (j + 1), 128 * l)
            hp[j + 1, 64 * l:64 * l + 64, :] = pltpu.bitcast(
                hb[j, 128 * l:128 * (l + 1), :], U32)

    def stage_a(p, i, kvv, hpv):
        fx = pltpu.bitcast(dft[0:BLK, :], BF)
        xf = jnp.dot(fx, pltpu.bitcast(kvv[0:64, 0:D], BF), preferred_element_type=F32)
        for l in range(NL):
            xhq[p][l, i] = xf[:, 128 * l:128 * (l + 1)].reshape(4, 64, 128)
        hf = lax.dot_general(fx, pltpu.bitcast(hpv[0, 0:D // 2, :], BF), NT, preferred_element_type=F32)
        for l in range(NL):
            xhq[p][l, 4 + i] = hf[:, 128 * l:128 * (l + 1)].reshape(4, 64, 128)

    all_lanes = list(range(NL))

    def link(v):
        for q in range(4):
            xhq[q][zs[3], 8, 0, 0:8, :] = v

    def stage_b(a0, n, i, lanes, hops, yov=None):
        q = a0 // 4
        yref = yfq[q] if yov is None else yov
        yfv = [yref.at[pl.ds(_mo(32 * i + BLK * ((a0 + da) % 4), 32), 32)] for da in range(n)]
        for gg in range(4):
            y0 = 8 * gg
            for l in lanes:
                ls = pl.ds(_mo(128 * l, 128), 128)
                if a0 > 0:
                    pr = qp[i, 0, y0:y0 + 8, ls]
                    pi = qp[i, 1, y0:y0 + 8, ls]
                acc = [[None] * 3 for _ in range(n)]
                xs = {}
                for m in range(a0 + n):
                    hr = xhq[m // 4][l, 4 + m % 4, i, 16 * gg:16 * gg + 8, :]
                    hi = xhq[m // 4][l, 4 + m % 4, i, 16 * gg + 8:16 * gg + 16, :]
                    hm = (hr + hi, hr, hi)
                    for da in range(n):
                        jx = a0 + da - m
                        if jx < 0:
                            continue
                        if jx not in xs:
                            xr = xhq[jx // 4][l, jx % 4, i, 16 * gg:16 * gg + 8, :]
                            xi = xhq[jx // 4][l, jx % 4, i, 16 * gg + 8:16 * gg + 16, :]
                            xs[jx] = (xr + xi, xr, xi)
                        for c in range(3):
                            p = xs[jx][c] * hm[c]
                            acc[da][c] = p if acc[da][c] is None else acc[da][c] + p
                for da in range(n):
                    s3, s1, s2 = acc[da]
                    re = s1 - s2
                    im = s3 - (s1 + s2)
                    if a0 + da == 0:
                        ore, oim = re, im
                    else:
                        ore, oim = re - pi, im + pr
                    yfv[da][y0:y0 + 8, ls if yov is None else slice(128, 256)] = pltpu.bitcast(
                        jnp.concatenate([ore, oim], axis=0).astype(BF), U32)
                    pr, pi = re, im
                if a0 + n < NB:
                    qp[i, 0, y0:y0 + 8, ls] = pr
                    qp[i, 1, y0:y0 + 8, ls] = pi
                if hops is not None:
                    v = oim
                    for _ in range(hops):
                        v = jnp.tanh(v)
                    link(v)

    def stage_c(q, i, ls=slice(None), yov=None, hs=(0, 1)):
        r0 = _mo((4 * q + i) * BLK, BLK)
        for hh in hs:
            if yov is None:
                yf = yfq[q][pl.ds(_mo(i * BLK + 64 * hh, 64), 64), ls]
            else:
                yf = yov[i * BLK + 64 * hh:i * BLK + 64 * hh + 64, 0:128]
            g = pltpu.bitcast(dft[BLK + 64 * hh:BLK + 64 * (hh + 1), :], BF)
            yb[hh, pl.ds(r0, BLK), ls] = jnp.dot(g, pltpu.bitcast(yf, BF),
                                                 preferred_element_type=F32)

    def unit_b(a0, lane):
        for i in range(4):
            stage_b(a0, 2, i, [lane], HOPS)

    def unit_c(a0, lane):
        ls = pl.ds(_mo(lane * 128, 128), 128)
        for i in range(2):
            stage_c(3, a0 % 4 + i, ls)

    def phase(p):
        def body(i, carry):
            t = 4 * p + i + 1
            wait_block(t)
            kvv = kvb.at[pl.ds(pl.multiple_of(t * 64, 64), 128)]
            hpv = hp.at[pl.ds(t, 2)]
            stage_a(p, i, kvv, hpv)
            if p == 2:
                stage_c(0, i, hs=(0, 1) if C0 == 'a' else (0,))
            stage_v(t, kvv, hpv)
            if p >= 1:
                stage_b(4 * (p - 1), 4, i, all_lanes, None)
            return carry
        with jax.named_scope("p%d" % p):
            lax.fori_loop(0, 4, body, 0)

    with jax.named_scope("w0"):
        wait_block(0)
    with jax.named_scope("v0"):
        stage_v(jnp.int32(0), kvb.at[pl.ds(0, 128)], hp.at[pl.ds(0, 2)])
        dft_cp.wait()
    phase(0)
    dvec = dvf[0:8, :]
    for g in range(NG):
        a, r = g // 4, 16 * (g % 4)
        for l in range(NL):
            xh0[l, 4, a, r:r + 8, :] = xh0[l, 4, a, r:r + 8, :] + dvec[:, 128 * l:128 * (l + 1)]
    for p in range(1, 3):
        phase(p)

    def lane_block(l):
        ls = slice(128 * l, 128 * (l + 1))
        fx = pltpu.bitcast(dft[0:BLK, :], BF)
        for j in range(12, NB):
            kv = pltpu.bitcast(kvb[64 * (j + 1):64 * (j + 2), ls], BF)
            xh3[l, j - 12] = jnp.dot(fx, kv, preferred_element_type=F32).reshape(4, 64, 128)
            hm = pltpu.bitcast(hp[j + 1, 64 * l:64 * l + 64, :], BF)
            xh3[l, j - 8] = lax.dot_general(
                fx, hm, NT, preferred_element_type=F32).reshape(4, 64, 128)
        for i in range(4):
            stage_c(1, i, ls)
        if l > 0:
            for i in range(4):
                stage_c(2, i, slice(128 * (l - 1), 128 * l))
        if l + 1 < NL:
            stage_v_lane(l + 1)
        for i in range(4):
            stage_b(8, 4, i, [l], None)

    with jax.named_scope("p3a"):
        for j in range(13, NB):
            wait_block(j)
        stage_v_lane(0)
    with jax.named_scope("p3"):
        seps[0].wait()
        lane_block(0)
        seps[1].wait()
        lane_block(1)
        for n in range(3):
            wm_cp(n).wait()
            lane_block(2 + n)

    def mod_chunk(n):
        m = jnp.dot(pltpu.bitcast(scb[0:8, :], BF), wmb[n], preferred_element_type=F32)[0:8]
        modb[n] = m + 1.0 if n == 4 else (0.5 * m if n == 5 else m)

    def mods(ns):
        return [jnp.concatenate([modb[n]] * 2, axis=0) for n in ns]

    def prep1(i, grp):
        ra = i * TM + zs[0] * 16
        xs = [qb[pl.ds(pl.multiple_of(ra + 16 * rc, 16), 16), :] for rc in grp]
        return [_stats(x.astype(F32)) for x in xs]

    def prep2(i, grp, st1, x1v, xoff):
        rb = i * TM + zs[1] * 16
        st2 = []
        for rc, (m, rs) in zip(grp, st1):
            r = pl.multiple_of(rb + 16 * rc, 16)
            sa, ca = mods((0, 1))
            x = qb[pl.ds(r, 16), :].astype(F32)
            ry = _mo(i * TM + 16 * rc, 16)
            x1 = x + (((x - m) * rs) * ca + sa) * (yb[0, pl.ds(ry, 16), :] + yb[1, pl.ds(ry, 16), :])
            x1v[xoff + 16 * rc:xoff + 16 * rc + 16, :] = x1
            st2.append(_stats(x1))
        return st2

    def prep3(i, grp, st2, h2v, hoff, chain):
        rc_ = i * TM + zs[2] * 16
        for n, (rc, (m, rs)) in enumerate(zip(grp, st2)):
            sb, cb = mods((3, 4))
            x1 = x1r[pl.ds(pl.multiple_of(rc_ + 16 * rc, 16), 16), :]
            h2 = ((x1 - m) * rs) * cb + sb
            h2v[hoff + 8 * rc:hoff + 8 * rc + 8, :] = pltpu.bitcast(h2.astype(BF), U32)
            if chain == 1:
                qb[S:S + 8, 128 * n:128 * (n + 1)] = h2[8:16, D - 128:D].astype(BF)
            elif chain == 2:
                xh3[zs[3], 8, 1, 8 * n:8 * n + 8, :] = h2[8:16, D - 128:D]

    def prep(i, h2v, hoff, x1v, xoff, link_n):
        for g0 in range(0, TM // 16, link_n):
            grp = range(g0, g0 + link_n)
            st2 = prep2(i, grp, prep1(i, grp), x1v, xoff)
            prep3(i, grp, st2, h2v, hoff, 1 if g0 + link_n < TM // 16 else (0 if UNL else 2))

    def o_cp(i, lo=0, hi=TM):
        r0 = _mo(i * TM + lo, 16)
        return cp(ob.at[pl.ds(r0, hi - lo)], o_hbm.at[0, pl.ds(r0, hi - lo)],
                  sem_o.at[i + (1 if lo else 0)])

    def w1(f0, f1, mode):
        if mode == 'd':
            wv = w1p.at[pl.ds(pl.multiple_of(zs[1] * 32, 32), F // 2)]
            return pltpu.bitcast(wv[f0 // 2:f1 // 2, :], BF)
        if mode == 'p':
            return pltpu.bitcast(w1p[f0 // 2:f1 // 2, :], BF)
        w = w1b[f0:f1, :]
        if mode == 's':
            w1p[f0 // 2:f1 // 2, :] = pltpu.bitcast(w, U32)
        return w

    def mm1(h2v, hoff, gv, goff, rows, f0, f1, mode='p'):
        h2 = pltpu.bitcast(h2v[hoff:hoff + rows // 2, :], BF)
        if f1 == F:
            st = lax.dot_general(w1(FH, F, mode), h2, NT, preferred_element_type=F32)
            st = _gelu(st + jnp.concatenate([b1c[...]] * (rows // 128), axis=1))
            gv[goff:goff + rows // 2, FH:F] = pltpu.bitcast(st.T.astype(BF), U32)
            f1 = FH
        if f0 == f1:
            return
        g = lax.dot_general(h2, w1(f0, f1, mode), NT, preferred_element_type=F32) + b1f[0:1, f0:f1]
        gv[goff:goff + rows // 2, f0:f1] = pltpu.bitcast(_gelu(g).astype(BF), U32)

    def mm2(i, gv, goff, x1v, xoff, lo=0, hi=TM, whole=None):
        r0 = _mo(i * TM + lo, 16)
        gb = modb[5][0:1]
        w2v = w2b.at[pl.ds(pl.multiple_of(zs[1] * 64, 64), F)] if 'v' in DYN and not isinstance(i, int) else w2b
        o = jnp.dot(pltpu.bitcast(gv[goff + lo // 2:goff + hi // 2, :], BF), w2v[...],
                    preferred_element_type=F32) + b2f[0:1, :]
        ob[pl.ds(r0, hi - lo), :] = (x1v[xoff + lo:xoff + hi, :] + gb * o).astype(BF)
        if whole is None:
            o_cp(i, lo, hi).start()
        elif whole:
            o_cp(i).start()

    allg = range(TM // 16)
    with jax.named_scope("p4"):
        q_cp(0).wait()
        q_cp(1).wait()
        for i in range(4):
            stage_c(2, i, slice(D - 128, D))
        m_ = [jnp.dot(pltpu.bitcast(scb[0:8, :], BF), wmb[n], preferred_element_type=F32)[0:8] for n in range(3)]
        modb[0] = m_[0] * m_[2]
        modb[1] = (m_[1] + 1.0) * m_[2]
        for i in range(4):
            stage_b(12, 2, i, [0], None)
        st1 = prep1(0, allg)
        if VAR == 'b':
            st1b = prep1(1, allg)
    with jax.named_scope("p5"):
        wm_cp(3).wait()
        mod_chunk(3)
        st2 = prep2(0, allg, st1, x1r, 0)
    with jax.named_scope("p6"):
        wm_cp(4).wait()
        mod_chunk(4)
        prep3(0, allg, st2, h2r, 0, 0)
    with jax.named_scope("firstA"):
        w1a_cp.wait()
        if VAR != 'b':
            q_cp(1).wait()
            st1b = prep1(1, allg)
        mm1(h2r, 0, gr, 0, TM, 0, F0, 's')
        st2 = prep2(1, allg, st1b, x1r, TM)
        prep3(1, allg, st2, h2r, TH, 0)
        r = 0
        for rows in FAS:
            mm1(h2r, TH + r // 2, gr, TH + r // 2, rows, 0, F0, 'r')
            r += rows
    with jax.named_scope("firstB"):
        w1b_cp.wait()
        unit_c(12, 0)
        mm1(h2r, 0, gr, 0, 2 * TM, F0, F, 's')
    with jax.named_scope("w2wait"):
        w2_cp.wait()
        wm_cp(5).wait()
        mod_chunk(5)

    def step(k, units):
        if isinstance(k, int):
            x1v, xo, gv, go = x1r, (k - 2) * TM, gr, (k - 2) * TH
        else:
            x1v = x1r.at[pl.ds(pl.multiple_of((k - 2) * TM, TM), 3 * TM)]
            gv = gr.at[pl.ds(pl.multiple_of((k - 2) * TH, TH), 3 * TH)]
            xo = go = 0
        if not (MERGE and isinstance(k, int)):
            q_cp(k).wait()
        r = 0
        for rows in M2S:
            mm2(k - 2, gv, go, x1v, xo, r, r + rows, r + rows == TM)
            r += rows
        dyn = not isinstance(k, int)
        hv = h2r.at[pl.ds(pl.multiple_of(zs[1] * 32, 32), TH)] if dyn and 'h' in DYN else h2r
        prep(k, hv, 0, x1v, xo + 2 * TM, LINK)
        for a0, lane in units:
            unit_b(a0, lane)
        r = 0
        for n_, rows in enumerate(RSPL):
            if HL and n_ == len(RSPL) - 1:
                mm1(hv, 0, gv, go + 2 * TH, TM, FH, F)
            mm1(hv, r // 2, gv, go + 2 * TH + r // 2, rows, 0, FH if HL else F)
            r += rows
        for a0, lane in units:
            unit_c(a0, lane)

    def body(k, carry):
        step(k, [(12, k - 1), (14, k - 2)])
        return carry

    with jax.named_scope("mloop"):
        lax.fori_loop(2, 6, body, 0)
    with jax.named_scope("mtail"):
        if MERGE:
            q_cp(6).wait()
            q_cp(7).wait()
        step(6, [(14, NL - 1)])
        step(7, [])
        mm2(6, gr, 6 * TH, x1r, 6 * TM)
        if TAILR:
            mm2(7, gr, 7 * TH, x1r, 7 * TM, 0, TM - TAILR)
            mm2(7, gr, 7 * TH, x1r, 7 * TM, TM - TAILR, TM)
        else:
            mm2(7, gr, 7 * TH, x1r, 7 * TM)
    with jax.named_scope("owait"):
        for i in range(NS - 1):
            o_cp(i).wait()
        if TAILR:
            o_cp(NS - 1, 0, TM - TAILR).wait()
            o_cp(NS - 1, TM - TAILR, TM).wait()
        else:
            o_cp(NS - 1).wait()


@jax.jit
def pallas_adaLN_cond__ssm_conv_h3__dense_activation_gelu__prompt_kernel(
    A_q, A_k, A_v, A_shift_k, A_ssm_k, A_ssm_D, B_x, B_w1, B_b1, B_w2, B_b2, c, w_mod,
):
    del B_x
    any_spec = pl.BlockSpec(memory_space=pl.ANY)
    scratch = [
        pltpu.VMEM((S + 64, D), BF),
        pltpu.VMEM((S, D), BF),
        pltpu.VMEM((S, D), BF),
        pltpu.VMEM((NB, D, BLK), BF),
        pltpu.VMEM((6, D, D), BF),
        pltpu.VMEM((F, D), BF),
        pltpu.VMEM((F, D), BF),
        pltpu.VMEM((S, D), BF),
        pltpu.VMEM((2 * BLK, BLK), U32),
        pltpu.VMEM((NL, S + 32, 128), F32),
        pltpu.VMEM((4, 8, D), F32),
        pltpu.VMEM(((NB + 1) * 64, D), U32),
        pltpu.VMEM((NB + 1, D // 2, BLK), U32),
    ] + [pltpu.VMEM((NL, 9, 4, 64, 128), F32)] * 4 + [pltpu.VMEM((4 * BLK, D), U32)] * 4 + [
        pltpu.VMEM((4, 2, 32, D), F32),
        pltpu.VMEM((2, S, D), F32),
        pltpu.VMEM((8, 8, D), F32),
        pltpu.VMEM((TM, D), U32),
        pltpu.VMEM((S, D), F32),
        pltpu.VMEM((S // 2, F), U32),
        pltpu.VMEM((64, 128), F32),
        pltpu.VMEM((F // 2, D), U32),
        pltpu.VMEM((16, F), F32),
        pltpu.VMEM((32, D), F32),
        pltpu.VMEM((32, D), F32),
        pltpu.VMEM((32, D), U32),
        pltpu.VMEM((4, D), BF),
        pltpu.VMEM((D,), BF),
        pltpu.VMEM((F,), BF),
        pltpu.VMEM((D,), BF),
        pltpu.VMEM((1, D), BF),
        pltpu.VMEM((2, 1, D), BF),
        pltpu.SMEM((8,), jnp.int32),
        pltpu.SemaphoreType.DMA((3 * NB + 6 + NS + 11,)),
        pltpu.SemaphoreType.DMA((NS + 1,)),
    ]
    return pl.pallas_call(
        _kernel,
        in_specs=[any_spec] * 13,
        out_specs=any_spec,
        out_shape=jax.ShapeDtypeStruct((1, S, D), BF),
        scratch_shapes=scratch,
        compiler_params=pltpu.CompilerParams(vmem_limit_bytes=110 * 1024 * 1024),
    )(A_q, A_k, A_v, A_shift_k.T, A_ssm_k, A_ssm_D, B_w1.T, B_b1, B_w2, B_b2, c, w_mod,
      jnp.asarray(_dft_mats()))
```

```python
import numpy as np
import jax
import jax.numpy as jnp
from jax import lax
import jax.experimental.pallas as pl
import jax.experimental.pallas.tpu as pltpu

S = 2048
D = 640
F = 1728
BLK = 128
NB = S // BLK
NG = BLK // 8
NL = D // 128
TM = 256
TH = TM // 2
NS = S // TM
F0 = 512
FH = 1664
LINK = 2
HOPS = 8
TAILR = 32
EPS = 1e-5
BF = jnp.bfloat16
F32 = jnp.float32
U32 = jnp.uint32
NT = (((1,), (1,)), ((), ()))


def _pack_rows(a):
    u = np.ascontiguousarray(a, dtype=np.float32).view(np.uint32)
    u = (u + 0x7FFF + ((u >> 16) & 1)) >> 16
    return (u[0::2] | (u[1::2] << 16)).astype(np.uint32)


def _dft_mats():
    n = 2 * BLK
    th = 2.0 * np.arange(BLK) + 0.5
    t = np.arange(BLK)
    ang = 2.0 * np.pi * th[:, None] * t[None, :] / n
    re, im = np.cos(ang), -np.sin(ang)
    fx = np.zeros((2 * BLK, BLK))
    inv = np.zeros((BLK, n))
    for g in range(NG):
        r, i = re[8 * g:8 * g + 8], im[8 * g:8 * g + 8]
        fx[16 * g:16 * g + 8] = r
        fx[16 * g + 8:16 * g + 16] = i
        inv[:, 16 * g:16 * g + 8] = (2.0 / n) * r.T
        inv[:, 16 * g + 8:16 * g + 16] = (2.0 / n) * i.T
    inv = _pack_rows(inv)
    return np.concatenate([_pack_rows(fx), inv[:, :BLK], inv[:, BLK:]], axis=0)


def _gelu2(x):
    c0 = 0.7978845608028654
    u = x * (c0 + (c0 * 0.044715) * (x * x))
    return x * (1.0 + jnp.tanh(u))


def _stats(x):
    m = jnp.sum(x, axis=-1, keepdims=True) * (1.0 / D)
    m2 = jnp.sum(x * x, axis=-1, keepdims=True) * (1.0 / D)
    v = jnp.maximum(m2 - m * m, 0.0) + EPS
    return m, jnp.exp(-0.5 * jnp.log(v))


def _mo(v, n):
    return v if isinstance(v, int) else pl.multiple_of(v, n)


def _bf(x):
    return pltpu.bitcast(x, BF)


def _pk(x):
    return pltpu.bitcast(x, U32)


def _kernel(q_hbm, k_hbm, v_hbm, sh_hbm, h_hbm, dv_hbm, w1_hbm, b1_hbm, w2_hbm,
            b2_hbm, c_hbm, wm_hbm, dft_hbm, o_hbm,
            qb, kb, vb, hb, wmb, w1b, w2b, ob, dft,
            kf, wb, kvb, hp, xh0, xh1, xh2, xh3, yf0, yf1, yf2, yf3,
            qp, yb, modb, h2r, x1r, gr, b1c, w1p, b1f, b2f, dvf, scb,
            shb, dvb, b1b, b2b, cb_, sepb, zs, sem, sem_o):
    xhq = (xh0, xh1, xh2, xh3)
    yfq = (yf0, yf1, yf2, yf3)
    cp = pltpu.make_async_copy

    n0 = 3 * NB
    n1 = n0 + 6 + NS

    def k_cp(j):
        return cp(k_hbm.at[0, pl.ds(BLK * j, BLK)], kb.at[pl.ds(BLK * j, BLK)], sem.at[3 * j])

    def v_cp(j):
        return cp(v_hbm.at[0, pl.ds(BLK * j, BLK)], vb.at[pl.ds(BLK * j, BLK)],
                  sem.at[3 * j + 1])

    def h_cp(j):
        return cp(h_hbm.at[:, pl.ds(BLK * j, BLK)], hb.at[j], sem.at[3 * j + 2])

    def wm_cp(n):
        return cp(wm_hbm.at[:, pl.ds(D * n, D)], wmb.at[n], sem.at[n0 + n])

    def q_cp(i):
        r0 = _mo(i * TM, TM)
        return cp(q_hbm.at[0, pl.ds(r0, TM)], qb.at[pl.ds(r0, TM)], sem.at[n0 + 6 + i])

    def o_cp(i, lo=0, hi=TM):
        r0 = _mo(i * TM + lo, 16)
        return cp(ob.at[pl.ds(r0, hi - lo)], o_hbm.at[0, pl.ds(r0, hi - lo)],
                  sem_o.at[i + (1 if lo else 0)])

    w1a_cp = cp(w1_hbm.at[pl.ds(0, F0)], w1b.at[pl.ds(0, F0)], sem.at[n1])
    w1b_cp = cp(w1_hbm.at[pl.ds(F0, F - F0)], w1b.at[pl.ds(F0, F - F0)], sem.at[n1 + 1])
    w2_cp = cp(w2_hbm, w2b, sem.at[n1 + 2])
    sh_cp = cp(sh_hbm, shb, sem.at[n1 + 3])
    dft_cp = cp(dft_hbm, dft, sem.at[n1 + 4])
    small = [cp(dv_hbm, dvb, sem.at[n1 + 5]), cp(c_hbm, cb_, sem.at[n1 + 6]),
             cp(b1_hbm, b1b, sem.at[n1 + 7]), cp(b2_hbm, b2b, sem.at[n1 + 8])]
    seps = [cp(c_hbm, sepb.at[n], sem.at[n1 + 9 + n]) for n in range(2)]

    sh_cp.start()
    for c_ in small:
        c_.start()
    for j in range(NB):
        k_cp(j).start()
        v_cp(j).start()
        h_cp(j).start()
        if j == 0:
            dft_cp.start()
        if j == 1:
            for c_ in seps:
                c_.start()
    for n in range(5):
        wm_cp(n).start()
        if n == 2:
            q_cp(0).start()
            q_cp(1).start()
    w1a_cp.start()
    w1b_cp.start()
    w2_cp.start()
    wm_cp(5).start()
    for i in range(2, NS):
        q_cp(i).start()

    for n in range(4):
        zs[n] = 0
    kf[:, 0:8, :] = jnp.zeros((NL, 8, 128), F32)
    sh_cp.wait()
    for c_ in small:
        c_.wait()
    b1 = b1b[...].astype(F32).reshape(1, F)
    b1f[0:8, :] = jnp.broadcast_to(b1, (8, F))
    b2f[0:8, :] = jnp.broadcast_to(2.0 * b2b[...].astype(F32).reshape(1, D), (8, D))
    b1c[...] = jnp.broadcast_to(b1[:, F - 128:F], (128, 128)).T[64:128, :]
    c = cb_[...].astype(F32)
    scb[0:8, :] = _pk(jnp.broadcast_to(c * jax.nn.sigmoid(c), (16, D)).astype(BF))
    dvf[0:8, :] = jnp.broadcast_to(dvb[...].astype(F32).reshape(1, D), (8, D))
    sh = shb[...].astype(F32)
    for t in range(4):
        wb[t] = jnp.broadcast_to(sh[t:t + 1, :], (8, D))

    def wait_block(j):
        k_cp(j).wait()
        v_cp(j).wait()
        h_cp(j).wait()

    def v_tile(j, l, dst, row0):
        ls = slice(128 * l, 128 * (l + 1))
        w = [jnp.concatenate([wb[t, :, ls]] * 2, axis=0) for t in range(4)]
        for rc in range(BLK // 16):
            r = pl.multiple_of(j * BLK + 16 * rc, 16)
            k = kb[pl.ds(r, 16), ls].astype(F32)
            v = vb[pl.ds(r, 16), ls].astype(F32)
            kf[l, pl.ds(r + 8, 16), :] = k
            ks = k * w[0]
            for t in range(1, 4):
                ks = ks + kf[l, pl.ds(j * BLK + 16 * rc + (8 - t), 16), :] * w[t]
            dst[row0 + 8 * rc:row0 + 8 * rc + 8, ls] = _pk((ks * v).astype(BF))

    def stage_v(j, kvv, hpv):
        for l in range(NL):
            v_tile(j, l, kvv, 64)
        hpv[1] = _pk(hb[j])

    def stage_v_lane(l):
        for j in range(13, NB):
            v_tile(j + zs[0], l, kvb, 64 * (j + 1))
            hp[j + 1, 64 * l:64 * l + 64, :] = _pk(hb[j, 128 * l:128 * (l + 1), :])

    def stage_a(p, i, kvv, hpv):
        fx = _bf(dft[0:BLK, :])
        xf = jnp.dot(fx, _bf(kvv[0:64, :]), preferred_element_type=F32)
        for l in range(NL):
            xhq[p][l, i] = xf[:, 128 * l:128 * (l + 1)].reshape(4, 64, 128)
        hf = lax.dot_general(fx, _bf(hpv[0]), NT, preferred_element_type=F32)
        for l in range(NL):
            xhq[p][l, 4 + i] = hf[:, 128 * l:128 * (l + 1)].reshape(4, 64, 128)

    def stage_b(a0, n, i, lanes, paced=False):
        yfv = [yfq[a0 // 4].at[pl.ds(_mo(32 * i + BLK * ((a0 + da) % 4), 32), 32)]
               for da in range(n)]
        for gg in range(4):
            y0 = 8 * gg
            for l in lanes:
                ls = pl.ds(_mo(128 * l, 128), 128)

                def spec(j, slot0):
                    re = xhq[j // 4][l, slot0 + j % 4, i, 16 * gg:16 * gg + 8, :]
                    im = xhq[j // 4][l, slot0 + j % 4, i, 16 * gg + 8:16 * gg + 16, :]
                    return (re + im, re, im)

                if a0 > 0:
                    pr = qp[i, 0, y0:y0 + 8, ls]
                    pi = qp[i, 1, y0:y0 + 8, ls]
                acc = [[None] * 3 for _ in range(n)]
                xs = {}
                for m in range(a0 + n):
                    hm = spec(m, 4)
                    for da in range(n):
                        jx = a0 + da - m
                        if jx < 0:
                            continue
                        if jx not in xs:
                            xs[jx] = spec(jx, 0)
                        for c_ in range(3):
                            p = xs[jx][c_] * hm[c_]
                            acc[da][c_] = p if acc[da][c_] is None else acc[da][c_] + p
                for da in range(n):
                    s3, s1, s2 = acc[da]
                    re = s1 - s2
                    im = s3 - (s1 + s2)
                    if a0 + da == 0:
                        ore, oim = re, im
                    else:
                        ore, oim = re - pi, im + pr
                    yfv[da][y0:y0 + 8, ls] = _pk(
                        jnp.concatenate([ore, oim], axis=0).astype(BF))
                    pr, pi = re, im
                if a0 + n < NB:
                    qp[i, 0, y0:y0 + 8, ls] = pr
                    qp[i, 1, y0:y0 + 8, ls] = pi
                if paced:
                    v = oim
                    for _ in range(HOPS):
                        v = jnp.tanh(v)
                    for q in range(4):
                        xhq[q][zs[3], 8, 0, 0:8, :] = v

    def stage_c(q, i, ls=slice(None)):
        r0 = _mo((4 * q + i) * BLK, BLK)
        for hh in range(2):
            yf = yfq[q][pl.ds(_mo(i * BLK + 64 * hh, 64), 64), ls]
            g = _bf(dft[BLK + 64 * hh:BLK + 64 * (hh + 1), :])
            yb[hh, pl.ds(r0, BLK), ls] = jnp.dot(g, _bf(yf), preferred_element_type=F32)

    def unit_b(a0, lane):
        for i in range(4):
            stage_b(a0, 2, i, [lane], True)

    def unit_c(a0, lane):
        ls = pl.ds(_mo(lane * 128, 128), 128)
        for i in range(2):
            stage_c(3, a0 % 4 + i, ls)

    def phase(p):
        def body(i, carry):
            t = 4 * p + i + 1
            wait_block(t)
            kvv = kvb.at[pl.ds(pl.multiple_of(t * 64, 64), 128)]
            hpv = hp.at[pl.ds(t, 2)]
            stage_a(p, i, kvv, hpv)
            if p == 2:
                stage_c(0, i)
            stage_v(t, kvv, hpv)
            if p >= 1:
                stage_b(4 * (p - 1), 4, i, range(NL))
            return carry
        lax.fori_loop(0, 4, body, 0)

    wait_block(0)
    stage_v(jnp.int32(0), kvb.at[pl.ds(0, 128)], hp.at[pl.ds(0, 2)])
    dft_cp.wait()
    phase(0)
    dvec = dvf[0:8, :]
    for g in range(NG):
        a, r = g // 4, 16 * (g % 4)
        for l in range(NL):
            xh0[l, 4, a, r:r + 8, :] = xh0[l, 4, a, r:r + 8, :] + dvec[:, 128 * l:128 * (l + 1)]
    phase(1)
    phase(2)

    def lane_block(l):
        ls = slice(128 * l, 128 * (l + 1))
        fx = _bf(dft[0:BLK, :])
        for j in range(12, NB):
            kv = _bf(kvb[64 * (j + 1):64 * (j + 2), ls])
            xh3[l, j - 12] = jnp.dot(fx, kv, preferred_element_type=F32).reshape(4, 64, 128)
            hm = _bf(hp[j + 1, 64 * l:64 * l + 64, :])
            xh3[l, j - 8] = lax.dot_general(
                fx, hm, NT, preferred_element_type=F32).reshape(4, 64, 128)
        for i in range(4):
            stage_c(1, i, ls)
        if l > 0:
            for i in range(4):
                stage_c(2, i, slice(128 * (l - 1), 128 * l))
        if l + 1 < NL:
            stage_v_lane(l + 1)
        for i in range(4):
            stage_b(8, 4, i, [l])

    for j in range(13, NB):
        wait_block(j)
    stage_v_lane(0)
    seps[0].wait()
    lane_block(0)
    seps[1].wait()
    lane_block(1)
    for n in range(3):
        wm_cp(n).wait()
        lane_block(2 + n)

    def mod_vec(n):
        return jnp.dot(_bf(scb[0:8, :]), wmb[n], preferred_element_type=F32)[0:8]

    def mods(ns):
        return [jnp.concatenate([modb[n]] * 2, axis=0) for n in ns]

    def prep1(i, grp):
        ra = i * TM + zs[0] * 16
        xs = [qb[pl.ds(pl.multiple_of(ra + 16 * rc, 16), 16), :] for rc in grp]
        return [_stats(x.astype(F32)) for x in xs]

    def prep2(i, grp, st1, x1v, xoff):
        rb = i * TM + zs[1] * 16
        st2 = []
        for rc, (m, rs) in zip(grp, st1):
            sa, ca = mods((0, 1))
            x = qb[pl.ds(pl.multiple_of(rb + 16 * rc, 16), 16), :].astype(F32)
            ry = _mo(i * TM + 16 * rc, 16)
            x1 = x + (((x - m) * rs) * ca + sa) * (
                yb[0, pl.ds(ry, 16), :] + yb[1, pl.ds(ry, 16), :])
            x1v[xoff + 16 * rc:xoff + 16 * rc + 16, :] = x1
            st2.append(_stats(x1))
        return st2

    def prep3(i, grp, st2, hoff, chain):
        rx = i * TM + zs[2] * 16
        for n, (rc, (m, rs)) in enumerate(zip(grp, st2)):
            sb, cb = mods((3, 4))
            x1 = x1r[pl.ds(pl.multiple_of(rx + 16 * rc, 16), 16), :]
            h2 = ((x1 - m) * rs) * cb + sb
            h2r[hoff + 8 * rc:hoff + 8 * rc + 8, :] = _pk(h2.astype(BF))
            if chain == 1:
                qb[S:S + 8, 128 * n:128 * (n + 1)] = h2[8:16, D - 128:D].astype(BF)
            elif chain == 2:
                xh3[zs[3], 8, 1, 8 * n:8 * n + 8, :] = h2[8:16, D - 128:D]

    def prep(i, x1v, xoff):
        for g0 in range(0, TM // 16, LINK):
            grp = range(g0, g0 + LINK)
            st2 = prep2(i, grp, prep1(i, grp), x1v, xoff)
            prep3(i, grp, st2, 0, 1 if g0 + LINK < TM // 16 else 2)

    def w1(f0, f1, mode):
        if mode == 'packed':
            return _bf(w1p[f0 // 2:f1 // 2, :])
        w = w1b[f0:f1, :]
        if mode == 'save':
            w1p[f0 // 2:f1 // 2, :] = _pk(w)
        return w

    def mm1(hoff, gv, goff, rows, f0, f1, mode='packed'):
        h2 = _bf(h2r[hoff:hoff + rows // 2, :])
        if f1 == F:
            st = lax.dot_general(w1(FH, F, mode), h2, NT, preferred_element_type=F32)
            st = _gelu2(st + jnp.concatenate([b1c[...]] * (rows // 128), axis=1))
            gv[goff:goff + rows // 2, FH:F] = _pk(st.T.astype(BF))
            f1 = FH
        if f0 < f1:
            g = lax.dot_general(h2, w1(f0, f1, mode), NT,
                                preferred_element_type=F32) + b1f[0:1, f0:f1]
            gv[goff:goff + rows // 2, f0:f1] = _pk(_gelu2(g).astype(BF))

    def mm2(i, gv, goff, x1v, xoff, lo=0, hi=TM):
        r0 = _mo(i * TM + lo, 16)
        gb = modb[5][0:1]
        o = jnp.dot(_bf(gv[goff + lo // 2:goff + hi // 2, :]), w2b[...],
                    preferred_element_type=F32) + b2f[0:1, :]
        ob[pl.ds(r0, hi - lo), :] = (x1v[xoff + lo:xoff + hi, :] + gb * o).astype(BF)
        o_cp(i, lo, hi).start()

    allg = range(TM // 16)
    q_cp(0).wait()
    q_cp(1).wait()
    for i in range(4):
        stage_c(2, i, slice(D - 128, D))
    mv = [mod_vec(n) for n in range(3)]
    modb[0] = mv[0] * mv[2]
    modb[1] = (mv[1] + 1.0) * mv[2]
    for i in range(4):
        stage_b(12, 2, i, [0])
    st1a = prep1(0, allg)
    st1b = prep1(1, allg)

    wm_cp(3).wait()
    modb[3] = mod_vec(3)
    st2a = prep2(0, allg, st1a, x1r, 0)

    wm_cp(4).wait()
    modb[4] = mod_vec(4) + 1.0
    prep3(0, allg, st2a, 0, 0)

    w1a_cp.wait()
    mm1(0, gr, 0, TM, 0, F0, 'save')
    prep3(1, allg, prep2(1, allg, st1b, x1r, TM), TH, 0)
    mm1(TH, gr, TH, TM, 0, F0, 'raw')

    w1b_cp.wait()
    unit_c(12, 0)
    mm1(0, gr, 0, 2 * TM, F0, F, 'save')

    w2_cp.wait()
    wm_cp(5).wait()
    modb[5] = 0.5 * mod_vec(5)

    def step(k, units):
        if isinstance(k, int):
            x1v, xo, gv, go = x1r, (k - 2) * TM, gr, (k - 2) * TH
        else:
            x1v = x1r.at[pl.ds(pl.multiple_of((k - 2) * TM, TM), 3 * TM)]
            gv = gr.at[pl.ds(pl.multiple_of((k - 2) * TH, TH), 3 * TH)]
            xo = go = 0
        mm2(k - 2, gv, go, x1v, xo)
        prep(k, x1v, xo + 2 * TM)
        for a0, lane in units:
            unit_b(a0, lane)
        mm1(0, gv, go + 2 * TH, TM // 2, 0, FH)
        mm1(0, gv, go + 2 * TH, TM, FH, F)
        mm1(TH // 2, gv, go + 2 * TH + TH // 2, TM // 2, 0, FH)
        for a0, lane in units:
            unit_c(a0, lane)

    def body(k, carry):
        q_cp(k).wait()
        step(k, [(12, k - 1), (14, k - 2)])
        return carry

    lax.fori_loop(2, 6, body, 0)
    q_cp(6).wait()
    q_cp(7).wait()
    step(6, [(14, NL - 1)])
    step(7, [])
    mm2(6, gr, 6 * TH, x1r, 6 * TM)
    mm2(7, gr, 7 * TH, x1r, 7 * TM, 0, TM - TAILR)
    mm2(7, gr, 7 * TH, x1r, 7 * TM, TM - TAILR, TM)
    for i in range(NS - 1):
        o_cp(i).wait()
    o_cp(NS - 1, 0, TM - TAILR).wait()
    o_cp(NS - 1, TM - TAILR, TM).wait()


@jax.jit
def pallas_adaLN_cond__ssm_conv_h3__dense_activation_gelu__prompt_kernel(
    A_q: jax.Array,
    A_k: jax.Array,
    A_v: jax.Array,
    A_shift_k: jax.Array,
    A_ssm_k: jax.Array,
    A_ssm_D: jax.Array,
    B_x: jax.Array,
    B_w1: jax.Array,
    B_b1: jax.Array,
    B_w2: jax.Array,
    B_b2: jax.Array,
    c: jax.Array,
    w_mod: jax.Array,
):
    del B_x
    any_spec = pl.BlockSpec(memory_space=pl.ANY)
    scratch = [
        pltpu.VMEM((S + 64, D), BF),
        pltpu.VMEM((S, D), BF),
        pltpu.VMEM((S, D), BF),
        pltpu.VMEM((NB, D, BLK), BF),
        pltpu.VMEM((6, D, D), BF),
        pltpu.VMEM((F, D), BF),
        pltpu.VMEM((F, D), BF),
        pltpu.VMEM((S, D), BF),
        pltpu.VMEM((2 * BLK, BLK), U32),
        pltpu.VMEM((NL, S + 32, 128), F32),
        pltpu.VMEM((4, 8, D), F32),
        pltpu.VMEM(((NB + 1) * 64, D), U32),
        pltpu.VMEM((NB + 1, D // 2, BLK), U32),
    ] + [pltpu.VMEM((NL, 9, 4, 64, 128), F32)] * 4 + [pltpu.VMEM((4 * BLK, D), U32)] * 4 + [
        pltpu.VMEM((4, 2, 32, D), F32),
        pltpu.VMEM((2, S, D), F32),
        pltpu.VMEM((8, 8, D), F32),
        pltpu.VMEM((TM, D), U32),
        pltpu.VMEM((S, D), F32),
        pltpu.VMEM((S // 2, F), U32),
        pltpu.VMEM((64, 128), F32),
        pltpu.VMEM((F // 2, D), U32),
        pltpu.VMEM((16, F), F32),
        pltpu.VMEM((32, D), F32),
        pltpu.VMEM((32, D), F32),
        pltpu.VMEM((32, D), U32),
        pltpu.VMEM((4, D), BF),
        pltpu.VMEM((D,), BF),
        pltpu.VMEM((F,), BF),
        pltpu.VMEM((D,), BF),
        pltpu.VMEM((1, D), BF),
        pltpu.VMEM((2, 1, D), BF),
        pltpu.SMEM((8,), jnp.int32),
        pltpu.SemaphoreType.DMA((3 * NB + 6 + NS + 11,)),
        pltpu.SemaphoreType.DMA((NS + 1,)),
    ]
    return pl.pallas_call(
        _kernel,
        in_specs=[any_spec] * 13,
        out_specs=any_spec,
        out_shape=jax.ShapeDtypeStruct((1, S, D), BF),
        scratch_shapes=scratch,
        compiler_params=pltpu.CompilerParams(vmem_limit_bytes=110 * 1024 * 1024,
                                             disable_semaphore_checks=True),
    )(A_q, A_k, A_v, A_shift_k.T, A_ssm_k, A_ssm_D, B_w1.T, B_b1, B_w2, B_b2, c, w_mod,
      jnp.asarray(_dft_mats()))
```

```python
import numpy as np
import jax
import jax.numpy as jnp
from jax import lax
import jax.experimental.pallas as pl
import jax.experimental.pallas.tpu as pltpu

S = 2048
D = 640
F = 1728
BLK = 128
NB = S // BLK
NG = BLK // 8
NL = D // 128
TM = 256
TH = TM // 2
NS = S // TM
F0 = 256
F1 = 768
FH = 1664
LINK = 2
HOPS = 8
TAILR = 32
EPS = 1e-5
BF = jnp.bfloat16
F32 = jnp.float32
U32 = jnp.uint32
NT = (((1,), (1,)), ((), ()))


def _dft_tile(rows, r0, transposed):
    shape = (BLK, rows) if transposed else (rows, BLK)
    f = lax.broadcasted_iota(jnp.int32, shape, 1 if transposed else 0) + r0
    t = lax.broadcasted_iota(jnp.int32, shape, 0 if transposed else 1)
    j = ((f >> 4) << 3) + (f & 7)
    ph = ((4 * j + 1) * t + ((f >> 3) & 1) * 128 + 256) & 511
    z = (128 - jnp.abs(ph - 256)).astype(F32) * (2.0 * np.pi / 512.0)
    z2 = z * z
    val = 1.0 / 6227020800.0
    for d in (-39916800.0, 362880.0, -5040.0, 120.0, -6.0, 1.0):
        val = val * z2 + 1.0 / d
    val = val * z
    return (val * (1.0 / BLK) if transposed else val).astype(BF)


def _gelu2(x):
    c0 = 0.7978845608028654
    u = x * (c0 + (c0 * 0.044715) * (x * x))
    return x * (1.0 + jnp.tanh(u))


def _stats(x):
    m = jnp.sum(x, axis=-1, keepdims=True) * (1.0 / D)
    m2 = jnp.sum(x * x, axis=-1, keepdims=True) * (1.0 / D)
    v = jnp.maximum(m2 - m * m, 0.0) + EPS
    return m, jnp.exp(-0.5 * jnp.log(v))


def _mo(v, n):
    return v if isinstance(v, int) else pl.multiple_of(v, n)


def _bf(x):
    return pltpu.bitcast(x, BF)


def _pk(x):
    return pltpu.bitcast(x, U32)


def _kernel(q_hbm, k_hbm, v_hbm, sh_hbm, h_hbm, dv_hbm, w1_hbm, b1_hbm, w2_hbm,
            b2_hbm, c_hbm, wm_hbm, o_hbm,
            qb, kb, vb, hb, wmb, w1b, w2b, ob, dft,
            kf, wb, kvb, hp, xh0, xh1, xh2, xh3, yf0, yf1, yf2, yf3,
            qp, yb, modb, h2r, x1r, gr, b1c, w1p, b1f, b2f, dvf, scb,
            shb, dvb, b1b, b2b, cb_, zs, sem, sem_o):
    xhq = (xh0, xh1, xh2, xh3)
    yfq = (yf0, yf1, yf2, yf3)
    cp = pltpu.make_async_copy

    n0 = 3 * NB
    n1 = n0 + 6 + NS

    def k_cp(j):
        return cp(k_hbm.at[0, pl.ds(BLK * j, BLK)], kb.at[pl.ds(BLK * j, BLK)], sem.at[3 * j])

    def v_cp(j):
        return cp(v_hbm.at[0, pl.ds(BLK * j, BLK)], vb.at[pl.ds(BLK * j, BLK)],
                  sem.at[3 * j + 1])

    def h_cp(j):
        return cp(h_hbm.at[:, pl.ds(BLK * j, BLK)], hb.at[j], sem.at[3 * j + 2])

    def wm_cp(n):
        return cp(wm_hbm.at[:, pl.ds(D * n, D)], wmb.at[n], sem.at[n0 + n])

    def q_cp(i):
        r0 = _mo(i * TM, TM)
        return cp(q_hbm.at[0, pl.ds(r0, TM)], qb.at[pl.ds(r0, TM)], sem.at[n0 + 6 + i])

    def o_cp(i, lo=0, hi=TM):
        r0 = _mo(i * TM + lo, 16)
        return cp(ob.at[pl.ds(r0, hi - lo)], o_hbm.at[0, pl.ds(r0, hi - lo)],
                  sem_o.at[i + (1 if lo else 0)])

    w1a_cp = cp(w1_hbm.at[pl.ds(0, F0)], w1b.at[pl.ds(0, F0)], sem.at[n1])
    w1m_cp = cp(w1_hbm.at[pl.ds(F0, F1 - F0)], w1b.at[pl.ds(F0, F1 - F0)], sem.at[n1 + 8])
    w1b_cp = cp(w1_hbm.at[pl.ds(F1, F - F1)], w1b.at[pl.ds(F1, F - F1)], sem.at[n1 + 1])
    w2_cp = cp(w2_hbm, w2b, sem.at[n1 + 2])
    sh_cp = cp(sh_hbm, shb, sem.at[n1 + 3])
    dv_cp = cp(dv_hbm, dvb, sem.at[n1 + 4])
    c_cp = cp(c_hbm, cb_, sem.at[n1 + 5])
    b1_cp = cp(b1_hbm, b1b, sem.at[n1 + 6])
    b2_cp = cp(b2_hbm, b2b, sem.at[n1 + 7])

    sh_cp.start()
    dv_cp.start()
    b1_cp.start()
    for j in range(NB):
        k_cp(j).start()
        v_cp(j).start()
        h_cp(j).start()
        if j == 8:
            c_cp.start()
            b2_cp.start()
    for n in range(5):
        wm_cp(n).start()
        if n == 2:
            q_cp(0).start()
            q_cp(1).start()
    w1a_cp.start()
    w1m_cp.start()
    w1b_cp.start()
    w2_cp.start()
    wm_cp(5).start()
    for i in range(2, NS):
        q_cp(i).start()

    for n in range(4):
        zs[n] = 0
    kf[:, 0:8, :] = jnp.zeros((NL, 8, 128), F32)
    dft[0:BLK, 0:BLK] = _pk(_dft_tile(2 * BLK, 0, False))
    dft[0:BLK // 2, BLK:3 * BLK] = _pk(_dft_tile(2 * BLK, 0, True))
    sh_cp.wait()
    dv_cp.wait()
    b1_cp.wait()
    b1 = b1b[...].astype(F32).reshape(1, F)
    b1f[0:8, :] = jnp.broadcast_to(b1, (8, F))
    b1c[...] = jnp.broadcast_to(b1[:, F - 128:F], (128, 128)).T[64:128, :]
    dvf[0:8, :] = jnp.broadcast_to(dvb[...].astype(F32).reshape(1, D), (8, D))
    sh = shb[...].astype(F32)
    for t in range(4):
        wb[t] = jnp.broadcast_to(sh[t:t + 1, :], (8, D))

    def wait_block(j):
        k_cp(j).wait()
        v_cp(j).wait()
        h_cp(j).wait()

    def v_tile(j, l, dst, row0):
        ls = slice(128 * l, 128 * (l + 1))
        w = [jnp.concatenate([wb[t, :, ls]] * 2, axis=0) for t in range(4)]
        for rc in range(BLK // 16):
            r = pl.multiple_of(j * BLK + 16 * rc, 16)
            k = kb[pl.ds(r, 16), ls].astype(F32)
            v = vb[pl.ds(r, 16), ls].astype(F32)
            kf[l, pl.ds(r + 8, 16), :] = k
            ks = k * w[0]
            for t in range(1, 4):
                ks = ks + kf[l, pl.ds(j * BLK + 16 * rc + (8 - t), 16), :] * w[t]
            dst[row0 + 8 * rc:row0 + 8 * rc + 8, ls] = _pk((ks * v).astype(BF))

    def stage_v(j, kvv, hpv):
        for l in range(NL):
            v_tile(j, l, kvv, 64)
        hpv[1] = _pk(hb[j])

    def stage_v_lane(l):
        for j in range(13, NB):
            v_tile(j + zs[0], l, kvb, 64 * (j + 1))
            hp[j + 1, 64 * l:64 * l + 64, :] = _pk(hb[j, 128 * l:128 * (l + 1), :])

    def stage_a(p, i, kvv, hpv):
        fx = _bf(dft[0:BLK, 0:BLK])
        xf = jnp.dot(fx, _bf(kvv[0:64, :]), preferred_element_type=F32)
        for l in range(NL):
            xhq[p][l, i] = xf[:, 128 * l:128 * (l + 1)].reshape(4, 64, 128)
        hf = lax.dot_general(fx, _bf(hpv[0]), NT, preferred_element_type=F32)
        for l in range(NL):
            xhq[p][l, 4 + i] = hf[:, 128 * l:128 * (l + 1)].reshape(4, 64, 128)

    def stage_b(a0, n, i, lanes, paced=False):
        yfv = [yfq[a0 // 4].at[pl.ds(_mo(32 * i + BLK * ((a0 + da) % 4), 32), 32)]
               for da in range(n)]
        for gg in range(4):
            y0 = 8 * gg
            for l in lanes:
                ls = pl.ds(_mo(128 * l, 128), 128)

                def spec(j, slot0):
                    re = xhq[j // 4][l, slot0 + j % 4, i, 16 * gg:16 * gg + 8, :]
                    im = xhq[j // 4][l, slot0 + j % 4, i, 16 * gg + 8:16 * gg + 16, :]
                    return (re + im, re, im)

                if a0 > 0:
                    pr = qp[i, 0, y0:y0 + 8, ls]
                    pi = qp[i, 1, y0:y0 + 8, ls]
                acc = [[None] * 3 for _ in range(n)]
                xs = {}
                for m in range(a0 + n):
                    hm = spec(m, 4)
                    for da in range(n):
                        jx = a0 + da - m
                        if jx < 0:
                            continue
                        if jx not in xs:
                            xs[jx] = spec(jx, 0)
                        for c_ in range(3):
                            p = xs[jx][c_] * hm[c_]
                            acc[da][c_] = p if acc[da][c_] is None else acc[da][c_] + p
                for da in range(n):
                    s3, s1, s2 = acc[da]
                    re = s1 - s2
                    im = s3 - (s1 + s2)
                    if a0 + da == 0:
                        ore, oim = re, im
                    else:
                        ore, oim = re - pi, im + pr
                    yfv[da][y0:y0 + 8, ls] = _pk(
                        jnp.concatenate([ore, oim], axis=0).astype(BF))
                    pr, pi = re, im
                if a0 + n < NB:
                    qp[i, 0, y0:y0 + 8, ls] = pr
                    qp[i, 1, y0:y0 + 8, ls] = pi
                if paced:
                    v = oim
                    for _ in range(HOPS):
                        v = jnp.tanh(v)
                    for q in range(4):
                        xhq[q][zs[3], 8, 0, 0:8, :] = v

    def stage_c(q, i, ls=slice(None)):
        r0 = _mo((4 * q + i) * BLK, BLK)
        for hh in range(2):
            yf = yfq[q][pl.ds(_mo(i * BLK + 64 * hh, 64), 64), ls]
            g = _bf(dft[0:BLK // 2, BLK * (1 + hh):BLK * (2 + hh)])
            yb[hh, pl.ds(r0, BLK), ls] = jnp.dot(g, _bf(yf), preferred_element_type=F32)

    def unit_b(a0, lane):
        for i in range(4):
            stage_b(a0, 2, i, [lane], True)

    def unit_c(a0, lane):
        ls = pl.ds(_mo(lane * 128, 128), 128)
        for i in range(2):
            stage_c(3, a0 % 4 + i, ls)

    def phase(p):
        def body(i, carry):
            t = 4 * p + i + 1
            wait_block(t)
            kvv = kvb.at[pl.ds(pl.multiple_of(t * 64, 64), 128)]
            hpv = hp.at[pl.ds(t, 2)]
            stage_a(p, i, kvv, hpv)
            if p == 2:
                stage_c(0, i, slice(256, D))
            stage_v(t, kvv, hpv)
            if p >= 1:
                stage_b(4 * (p - 1), 4, i, range(NL))
            return carry
        lax.fori_loop(0, 4, body, 0)

    wait_block(0)
    stage_v(jnp.int32(0), kvb.at[pl.ds(0, 128)], hp.at[pl.ds(0, 2)])
    phase(0)
    dvec = dvf[0:8, :]
    for g in range(NG):
        a, r = g // 4, 16 * (g % 4)
        for l in range(NL):
            xh0[l, 4, a, r:r + 8, :] = xh0[l, 4, a, r:r + 8, :] + dvec[:, 128 * l:128 * (l + 1)]
    phase(1)
    phase(2)

    def stage_a_lane(l):
        ls = slice(128 * l, 128 * (l + 1))
        fx = _bf(dft[0:BLK, 0:BLK])
        for j in range(12, NB):
            kv = _bf(kvb[64 * (j + 1):64 * (j + 2), ls])
            xh3[l, j - 12] = jnp.dot(fx, kv, preferred_element_type=F32).reshape(4, 64, 128)
            hm = _bf(hp[j + 1, 64 * l:64 * l + 64, :])
            xh3[l, j - 8] = lax.dot_general(
                fx, hm, NT, preferred_element_type=F32).reshape(4, 64, 128)

    def lane_block(l):
        ls = slice(128 * l, 128 * (l + 1))
        if l > 0:
            stage_a_lane(l - 1)
        for i in range(4):
            stage_c(1, i, ls)
        for i in range(4):
            if l == 0:
                stage_c(0, i, slice(0, 256))
            else:
                stage_c(2, i, slice(128 * (l - 1), 128 * l))
        stage_v_lane(l)
        for i in range(4):
            stage_b(8, 4, i, [l])

    for j in range(13, NB):
        wait_block(j)
    c_cp.wait()
    c = cb_[...].astype(F32)
    scb[0:8, :] = _pk(jnp.broadcast_to(c * jax.nn.sigmoid(c), (16, D)).astype(BF))
    lane_block(0)
    b2_cp.wait()
    b2f[0:8, :] = jnp.broadcast_to(2.0 * b2b[...].astype(F32).reshape(1, D), (8, D))
    lane_block(1)
    for n in range(3):
        wm_cp(n).wait()
        lane_block(2 + n)

    def mod_vec(n):
        return jnp.dot(_bf(scb[0:8, :]), wmb[n], preferred_element_type=F32)[0:8]

    def mods(ns):
        return [jnp.concatenate([modb[n]] * 2, axis=0) for n in ns]

    def prep1(i, grp):
        ra = i * TM + zs[0] * 16
        xs = [qb[pl.ds(pl.multiple_of(ra + 16 * rc, 16), 16), :] for rc in grp]
        return [_stats(x.astype(F32)) for x in xs]

    def prep2(i, grp, st1, x1v, xoff):
        rb = i * TM + zs[1] * 16
        st2 = []
        for rc, (m, rs) in zip(grp, st1):
            sa, ca = mods((0, 1))
            x = qb[pl.ds(pl.multiple_of(rb + 16 * rc, 16), 16), :].astype(F32)
            ry = _mo(i * TM + 16 * rc, 16)
            x1 = x + (((x - m) * rs) * ca + sa) * (
                yb[0, pl.ds(ry, 16), :] + yb[1, pl.ds(ry, 16), :])
            x1v[xoff + 16 * rc:xoff + 16 * rc + 16, :] = x1
            st2.append(_stats(x1))
        return st2

    def prep3(i, grp, st2, hoff, chain):
        rx = i * TM + zs[2] * 16
        for n, (rc, (m, rs)) in enumerate(zip(grp, st2)):
            sb, cb = mods((3, 4))
            x1 = x1r[pl.ds(pl.multiple_of(rx + 16 * rc, 16), 16), :]
            h2 = ((x1 - m) * rs) * cb + sb
            h2r[hoff + 8 * rc:hoff + 8 * rc + 8, :] = _pk(h2.astype(BF))
            if chain == 1:
                qb[S:S + 8, 128 * n:128 * (n + 1)] = h2[8:16, D - 128:D].astype(BF)
            elif chain == 2:
                xh3[zs[3], 8, 1, 8 * n:8 * n + 8, :] = h2[8:16, D - 128:D]

    def prep(i, x1v, xoff):
        for g0 in range(0, TM // 16, LINK):
            grp = range(g0, g0 + LINK)
            st2 = prep2(i, grp, prep1(i, grp), x1v, xoff)
            prep3(i, grp, st2, 0, 1 if g0 + LINK < TM // 16 else 2)

    def w1(f0, f1, mode):
        if mode == 'packed':
            return _bf(w1p[f0 // 2:f1 // 2, :])
        w = w1b[f0:f1, :]
        if mode == 'save':
            w1p[f0 // 2:f1 // 2, :] = _pk(w)
        return w

    def mm1(hoff, gv, goff, rows, f0, f1, mode='packed'):
        h2 = _bf(h2r[hoff:hoff + rows // 2, :])
        if f1 == F:
            st = lax.dot_general(w1(FH, F, mode), h2, NT, preferred_element_type=F32)
            st = _gelu2(st + jnp.concatenate([b1c[...]] * (rows // 128), axis=1))
            gv[goff:goff + rows // 2, FH:F] = _pk(st.T.astype(BF))
            f1 = FH
        if f0 < f1:
            g = lax.dot_general(h2, w1(f0, f1, mode), NT,
                                preferred_element_type=F32) + b1f[0:1, f0:f1]
            gv[goff:goff + rows // 2, f0:f1] = _pk(_gelu2(g).astype(BF))

    def mm2(i, gv, goff, x1v, xoff, lo=0, hi=TM):
        r0 = _mo(i * TM + lo, 16)
        gb = modb[5][0:1]
        o = jnp.dot(_bf(gv[goff + lo // 2:goff + hi // 2, :]), w2b[...],
                    preferred_element_type=F32) + b2f[0:1, :]
        ob[pl.ds(r0, hi - lo), :] = (x1v[xoff + lo:xoff + hi, :] + gb * o).astype(BF)
        o_cp(i, lo, hi).start()

    allg = range(TM // 16)
    q_cp(0).wait()
    q_cp(1).wait()
    stage_a_lane(NL - 1)
    for i in range(4):
        stage_c(2, i, slice(D - 128, D))
    mv = [mod_vec(n) for n in range(3)]
    modb[0] = mv[0] * mv[2]
    modb[1] = (mv[1] + 1.0) * mv[2]
    for i in range(4):
        stage_b(12, 2, i, [0])
    st1a = prep1(0, allg)
    st1b = prep1(1, allg)

    wm_cp(3).wait()
    modb[3] = mod_vec(3)
    st2a = prep2(0, allg, st1a, x1r, 0)

    wm_cp(4).wait()
    modb[4] = mod_vec(4) + 1.0
    prep3(0, allg, st2a, 0, 0)

    w1a_cp.wait()
    mm1(0, gr, 0, TM, 0, F0, 'save')
    prep3(1, allg, prep2(1, allg, st1b, x1r, TM), TH, 0)
    mm1(TH, gr, TH, TM, 0, F0, 'raw')

    w1m_cp.wait()
    unit_c(12, 0)
    mm1(0, gr, 0, 2 * TM, F0, F1, 'save')

    w1b_cp.wait()
    mm1(0, gr, 0, 2 * TM, F1, FH - 128, 'save')
    mm1(0, gr, 0, 2 * TM, FH, F, 'save')
    for r in range(4):
        mm1(r * 64, gr, r * 64, 128, FH - 128, FH, 'save' if r == 0 else 'raw')

    w2_cp.wait()
    wm_cp(5).wait()
    modb[5] = 0.5 * mod_vec(5)

    def step(k, units):
        if isinstance(k, int):
            x1v, xo, gv, go = x1r, (k - 2) * TM, gr, (k - 2) * TH
        else:
            x1v = x1r.at[pl.ds(pl.multiple_of((k - 2) * TM, TM), 3 * TM)]
            gv = gr.at[pl.ds(pl.multiple_of((k - 2) * TH, TH), 3 * TH)]
            xo = go = 0
        mm2(k - 2, gv, go, x1v, xo)
        prep(k, x1v, xo + 2 * TM)
        for a0, lane in units:
            unit_b(a0, lane)
        mm1(0, gv, go + 2 * TH, TM // 2, 0, FH)
        mm1(0, gv, go + 2 * TH, TM, FH, F)
        mm1(TH // 2, gv, go + 2 * TH + TH // 2, TM // 2, 0, FH)
        for a0, lane in units:
            unit_c(a0, lane)

    def body(k, carry):
        q_cp(k).wait()
        step(k, [(12, k - 1), (14, k - 2)])
        return carry

    lax.fori_loop(2, 6, body, 0)
    q_cp(6).wait()
    q_cp(7).wait()
    step(6, [(14, NL - 1)])
    step(7, [])
    mm2(6, gr, 6 * TH, x1r, 6 * TM)
    mm2(7, gr, 7 * TH, x1r, 7 * TM, 0, TM - TAILR)
    mm2(7, gr, 7 * TH, x1r, 7 * TM, TM - TAILR, TM)
    for i in range(NS - 1):
        o_cp(i).wait()
    o_cp(NS - 1, 0, TM - TAILR).wait()
    o_cp(NS - 1, TM - TAILR, TM).wait()


@jax.jit
def pallas_adaLN_cond__ssm_conv_h3__dense_activation_gelu__prompt_kernel(
    A_q: jax.Array,
    A_k: jax.Array,
    A_v: jax.Array,
    A_shift_k: jax.Array,
    A_ssm_k: jax.Array,
    A_ssm_D: jax.Array,
    B_x: jax.Array,
    B_w1: jax.Array,
    B_b1: jax.Array,
    B_w2: jax.Array,
    B_b2: jax.Array,
    c: jax.Array,
    w_mod: jax.Array,
):
    del B_x
    any_spec = pl.BlockSpec(memory_space=pl.ANY)
    scratch = [
        pltpu.VMEM((S + 64, D), BF),
        pltpu.VMEM((S, D), BF),
        pltpu.VMEM((S, D), BF),
        pltpu.VMEM((NB, D, BLK), BF),
        pltpu.VMEM((6, D, D), BF),
        pltpu.VMEM((F, D), BF),
        pltpu.VMEM((F, D), BF),
        pltpu.VMEM((S, D), BF),
        pltpu.VMEM((BLK, 4 * BLK), U32),
        pltpu.VMEM((NL, S + 32, 128), F32),
        pltpu.VMEM((4, 8, D), F32),
        pltpu.VMEM(((NB + 1) * 64, D), U32),
        pltpu.VMEM((NB + 1, D // 2, BLK), U32),
    ] + [pltpu.VMEM((NL, 9, 4, 64, 128), F32)] * 4 + [pltpu.VMEM((4 * BLK, D), U32)] * 4 + [
        pltpu.VMEM((4, 2, 32, D), F32),
        pltpu.VMEM((2, S, D), F32),
        pltpu.VMEM((8, 8, D), F32),
        pltpu.VMEM((TM, D), U32),
        pltpu.VMEM((S, D), F32),
        pltpu.VMEM((S // 2, F), U32),
        pltpu.VMEM((64, 128), F32),
        pltpu.VMEM((F // 2, D), U32),
        pltpu.VMEM((16, F), F32),
        pltpu.VMEM((32, D), F32),
        pltpu.VMEM((32, D), F32),
        pltpu.VMEM((32, D), U32),
        pltpu.VMEM((4, D), BF),
        pltpu.VMEM((D,), BF),
        pltpu.VMEM((F,), BF),
        pltpu.VMEM((D,), BF),
        pltpu.VMEM((1, D), BF),
        pltpu.SMEM((8,), jnp.int32),
        pltpu.SemaphoreType.DMA((3 * NB + 6 + NS + 9,)),
        pltpu.SemaphoreType.DMA((NS + 1,)),
    ]
    return pl.pallas_call(
        _kernel,
        in_specs=[any_spec] * 12,
        out_specs=any_spec,
        out_shape=jax.ShapeDtypeStruct((1, S, D), BF),
        scratch_shapes=scratch,
        compiler_params=pltpu.CompilerParams(vmem_limit_bytes=110 * 1024 * 1024,
                                             disable_semaphore_checks=True),
    )(A_q, A_k, A_v, A_shift_k.T, A_ssm_k, A_ssm_D, B_w1.T, B_b1, B_w2, B_b2, c, w_mod)
```

```python
import numpy as np
import jax
import jax.numpy as jnp
from jax import lax
import jax.experimental.pallas as pl
import jax.experimental.pallas.tpu as pltpu

S = 2048
D = 640
F = 1728
BLK = 128
NB = S // BLK
NG = BLK // 8
NL = D // 128
TM = 256
TH = TM // 2
NS = S // TM
F0 = 256
F1 = 768
FH = 1664
LINK = 2
HOPS = 8
TAILR = 32
EPS = 1e-5
BF = jnp.bfloat16
F32 = jnp.float32
U32 = jnp.uint32
NT = (((1,), (1,)), ((), ()))


def _dft_table(transposed):
    shape = (BLK, 2 * BLK) if transposed else (2 * BLK, BLK)
    f = lax.broadcasted_iota(jnp.int32, shape, 1 if transposed else 0)
    t = lax.broadcasted_iota(jnp.int32, shape, 0 if transposed else 1)
    j = ((f >> 4) << 3) + (f & 7)
    ph = ((4 * j + 1) * t + ((f >> 3) & 1) * 128 + 256) & 511
    z = (128 - jnp.abs(ph - 256)).astype(F32) * (2.0 * np.pi / 512.0)
    z2 = z * z
    val = 1.0 / 6227020800.0
    for d in (-39916800.0, 362880.0, -5040.0, 120.0, -6.0, 1.0):
        val = val * z2 + 1.0 / d
    val = val * z
    return (val * (1.0 / BLK) if transposed else val).astype(BF)


def _gelu2(x):
    c0 = 0.7978845608028654
    u = x * (c0 + (c0 * 0.044715) * (x * x))
    return x * (1.0 + jnp.tanh(u))


def _stats(x):
    m = jnp.sum(x, axis=-1, keepdims=True) * (1.0 / D)
    m2 = jnp.sum(x * x, axis=-1, keepdims=True) * (1.0 / D)
    v = jnp.maximum(m2 - m * m, 0.0) + EPS
    return m, jnp.exp(-0.5 * jnp.log(v))


def _mo(v, n):
    return v if isinstance(v, int) else pl.multiple_of(v, n)


def _bf(x):
    return pltpu.bitcast(x, BF)


def _pk(x):
    return pltpu.bitcast(x, U32)


def _kernel(q_hbm, k_hbm, v_hbm, sh_hbm, h_hbm, dv_hbm, w1_hbm, b1_hbm, w2_hbm,
            b2_hbm, c_hbm, wm_hbm, o_hbm,
            qb, kb, vb, hb, wmb, w1b, w2b, ob, dft,
            kf, wb, kvb, hp, xh0, xh1, xh2, xh3, yf0, yf1, yf2, yf3,
            qp, yb, modb, h2r, x1r, gr, b1c, w1p, b1f, b2f, dvf, scb,
            shb, dvb, b1b, b2b, cb_, zs, sem, sem_o):
    xhq = (xh0, xh1, xh2, xh3)
    yfq = (yf0, yf1, yf2, yf3)
    cp = pltpu.make_async_copy

    n0 = 3 * NB
    n1 = n0 + 6 + NS

    def k_cp(j):
        return cp(k_hbm.at[0, pl.ds(BLK * j, BLK)], kb.at[pl.ds(BLK * j, BLK)], sem.at[3 * j])

    def v_cp(j):
        return cp(v_hbm.at[0, pl.ds(BLK * j, BLK)], vb.at[pl.ds(BLK * j, BLK)],
                  sem.at[3 * j + 1])

    def h_cp(j):
        return cp(h_hbm.at[:, pl.ds(BLK * j, BLK)], hb.at[j], sem.at[3 * j + 2])

    def wm_cp(n):
        return cp(wm_hbm.at[:, pl.ds(D * n, D)], wmb.at[n], sem.at[n0 + n])

    def q_cp(i):
        r0 = _mo(i * TM, TM)
        return cp(q_hbm.at[0, pl.ds(r0, TM)], qb.at[pl.ds(r0, TM)], sem.at[n0 + 6 + i])

    def o_cp(i, lo=0, hi=TM):
        r0 = _mo(i * TM + lo, 16)
        return cp(ob.at[pl.ds(r0, hi - lo)], o_hbm.at[0, pl.ds(r0, hi - lo)],
                  sem_o.at[i + (1 if lo else 0)])

    w1a_cp = cp(w1_hbm.at[pl.ds(0, F0)], w1b.at[pl.ds(0, F0)], sem.at[n1])
    w1m_cp = cp(w1_hbm.at[pl.ds(F0, F1 - F0)], w1b.at[pl.ds(F0, F1 - F0)], sem.at[n1 + 8])
    w1b_cp = cp(w1_hbm.at[pl.ds(F1, F - F1)], w1b.at[pl.ds(F1, F - F1)], sem.at[n1 + 1])
    w2_cp = cp(w2_hbm, w2b, sem.at[n1 + 2])
    sh_cp = cp(sh_hbm, shb, sem.at[n1 + 3])
    dv_cp = cp(dv_hbm, dvb, sem.at[n1 + 4])
    c_cp = cp(c_hbm, cb_, sem.at[n1 + 5])
    b1_cp = cp(b1_hbm, b1b, sem.at[n1 + 6])
    b2_cp = cp(b2_hbm, b2b, sem.at[n1 + 7])

    sh_cp.start()
    dv_cp.start()
    b1_cp.start()
    for j in range(NB):
        k_cp(j).start()
        v_cp(j).start()
        h_cp(j).start()
        if j == 8:
            c_cp.start()
            b2_cp.start()
    for n in range(5):
        wm_cp(n).start()
        if n == 2:
            q_cp(0).start()
            q_cp(1).start()
    w1a_cp.start()
    w1m_cp.start()
    w1b_cp.start()
    w2_cp.start()
    wm_cp(5).start()
    for i in range(2, NS):
        q_cp(i).start()

    for n in range(4):
        zs[n] = 0
    kf[:, 0:8, :] = jnp.zeros((NL, 8, 128), F32)
    dft[0:BLK, 0:BLK] = _pk(_dft_table(False))
    dft[0:BLK // 2, BLK:3 * BLK] = _pk(_dft_table(True))
    sh_cp.wait()
    dv_cp.wait()
    b1_cp.wait()
    b1 = b1b[...].astype(F32).reshape(1, F)
    b1f[0:8, :] = jnp.broadcast_to(b1, (8, F))
    b1c[...] = jnp.broadcast_to(b1[:, F - 128:F], (128, 128)).T[64:128, :]
    dvf[0:8, :] = jnp.broadcast_to(dvb[...].astype(F32).reshape(1, D), (8, D))
    sh = shb[...].astype(F32)
    for t in range(4):
        wb[t] = jnp.broadcast_to(sh[t:t + 1, :], (8, D))

    def wait_block(j):
        k_cp(j).wait()
        v_cp(j).wait()
        h_cp(j).wait()

    def v_tile(j, l, dst, row0):
        ls = slice(128 * l, 128 * (l + 1))
        w = [jnp.concatenate([wb[t, :, ls]] * 2, axis=0) for t in range(4)]
        for rc in range(BLK // 16):
            r = pl.multiple_of(j * BLK + 16 * rc, 16)
            k = kb[pl.ds(r, 16), ls].astype(F32)
            v = vb[pl.ds(r, 16), ls].astype(F32)
            kf[l, pl.ds(r + 8, 16), :] = k
            ks = k * w[0]
            for t in range(1, 4):
                ks = ks + kf[l, pl.ds(j * BLK + 16 * rc + (8 - t), 16), :] * w[t]
            dst[row0 + 8 * rc:row0 + 8 * rc + 8, ls] = _pk((ks * v).astype(BF))

    def stage_v(j, kvv, hpv):
        for l in range(NL):
            v_tile(j, l, kvv, 64)
        hpv[1] = _pk(hb[j])

    def stage_v_lane(l):
        for j in range(13, NB):
            v_tile(j + zs[0], l, kvb, 64 * (j + 1))
            hp[j + 1, 64 * l:64 * l + 64, :] = _pk(hb[j, 128 * l:128 * (l + 1), :])

    def stage_a(p, i, kvv, hpv):
        fx = _bf(dft[0:BLK, 0:BLK])
        xf = jnp.dot(fx, _bf(kvv[0:64, :]), preferred_element_type=F32)
        for l in range(NL):
            xhq[p][l, i] = xf[:, 128 * l:128 * (l + 1)].reshape(4, 64, 128)
        hf = lax.dot_general(fx, _bf(hpv[0]), NT, preferred_element_type=F32)
        for l in range(NL):
            xhq[p][l, 4 + i] = hf[:, 128 * l:128 * (l + 1)].reshape(4, 64, 128)

    def stage_b(a0, n, i, lanes, paced=False):
        yfv = [yfq[a0 // 4].at[pl.ds(_mo(32 * i + BLK * ((a0 + da) % 4), 32), 32)]
               for da in range(n)]
        for gg in range(4):
            y0 = 8 * gg
            for l in lanes:
                ls = pl.ds(_mo(128 * l, 128), 128)

                def spec(j, slot0):
                    re = xhq[j // 4][l, slot0 + j % 4, i, 16 * gg:16 * gg + 8, :]
                    im = xhq[j // 4][l, slot0 + j % 4, i, 16 * gg + 8:16 * gg + 16, :]
                    return (re + im, re, im)

                if a0 > 0:
                    pr = qp[i, 0, y0:y0 + 8, ls]
                    pi = qp[i, 1, y0:y0 + 8, ls]
                acc = [[None] * 3 for _ in range(n)]
                xs = {}
                for m in range(a0 + n):
                    hm = spec(m, 4)
                    for da in range(n):
                        jx = a0 + da - m
                        if jx < 0:
                            continue
                        if jx not in xs:
                            xs[jx] = spec(jx, 0)
                        for c_ in range(3):
                            p = xs[jx][c_] * hm[c_]
                            acc[da][c_] = p if acc[da][c_] is None else acc[da][c_] + p
                for da in range(n):
                    s3, s1, s2 = acc[da]
                    re = s1 - s2
                    im = s3 - (s1 + s2)
                    if a0 + da == 0:
                        ore, oim = re, im
                    else:
                        ore, oim = re - pi, im + pr
                    yfv[da][y0:y0 + 8, ls] = _pk(
                        jnp.concatenate([ore, oim], axis=0).astype(BF))
                    pr, pi = re, im
                if a0 + n < NB:
                    qp[i, 0, y0:y0 + 8, ls] = pr
                    qp[i, 1, y0:y0 + 8, ls] = pi
                if paced:
                    v = oim
                    for _ in range(HOPS):
                        v = jnp.tanh(v)
                    for q in range(4):
                        xhq[q][zs[3], 8, 0, 0:8, :] = v

    def stage_c(q, i, ls=slice(None)):
        r0 = _mo((4 * q + i) * BLK, BLK)
        for hh in range(2):
            yf = yfq[q][pl.ds(_mo(i * BLK + 64 * hh, 64), 64), ls]
            g = _bf(dft[0:BLK // 2, BLK * (1 + hh):BLK * (2 + hh)])
            yb[hh, pl.ds(r0, BLK), ls] = jnp.dot(g, _bf(yf), preferred_element_type=F32)

    def unit_b(a0, lane):
        for i in range(4):
            stage_b(a0, 2, i, [lane], True)

    def unit_c(a0, lane):
        ls = pl.ds(_mo(lane * 128, 128), 128)
        for i in range(2):
            stage_c(3, a0 % 4 + i, ls)

    def phase(p):
        def body(i, carry):
            t = 4 * p + i + 1
            wait_block(t)
            kvv = kvb.at[pl.ds(pl.multiple_of(t * 64, 64), 128)]
            hpv = hp.at[pl.ds(t, 2)]
            stage_a(p, i, kvv, hpv)
            if p == 2:
                stage_c(0, i, slice(256, D))
            stage_v(t, kvv, hpv)
            if p >= 1:
                stage_b(4 * (p - 1), 4, i, range(NL))
            return carry
        lax.fori_loop(0, 4, body, 0)

    wait_block(0)
    stage_v(jnp.int32(0), kvb.at[pl.ds(0, 128)], hp.at[pl.ds(0, 2)])
    phase(0)
    dvec = dvf[0:8, :]
    for g in range(NG):
        a, r = g // 4, 16 * (g % 4)
        for l in range(NL):
            xh0[l, 4, a, r:r + 8, :] = xh0[l, 4, a, r:r + 8, :] + dvec[:, 128 * l:128 * (l + 1)]
    phase(1)
    phase(2)

    def stage_a_lane(l):
        ls = slice(128 * l, 128 * (l + 1))
        fx = _bf(dft[0:BLK, 0:BLK])
        for j in range(12, NB):
            kv = _bf(kvb[64 * (j + 1):64 * (j + 2), ls])
            xh3[l, j - 12] = jnp.dot(fx, kv, preferred_element_type=F32).reshape(4, 64, 128)
            hm = _bf(hp[j + 1, 64 * l:64 * l + 64, :])
            xh3[l, j - 8] = lax.dot_general(
                fx, hm, NT, preferred_element_type=F32).reshape(4, 64, 128)

    def lane_block(l):
        ls = slice(128 * l, 128 * (l + 1))
        if l > 0:
            stage_a_lane(l - 1)
        for i in range(4):
            stage_c(1, i, ls)
        for i in range(4):
            if l == 0:
                stage_c(0, i, slice(0, 256))
            else:
                stage_c(2, i, slice(128 * (l - 1), 128 * l))
        stage_v_lane(l)
        for i in range(4):
            stage_b(8, 4, i, [l])

    for j in range(13, NB):
        wait_block(j)
    c_cp.wait()
    c = cb_[...].astype(F32)
    scb[0:8, :] = _pk(jnp.broadcast_to(c * jax.nn.sigmoid(c), (16, D)).astype(BF))
    lane_block(0)
    b2_cp.wait()
    b2f[0:8, :] = jnp.broadcast_to(2.0 * b2b[...].astype(F32).reshape(1, D), (8, D))
    lane_block(1)
    for n in range(3):
        wm_cp(n).wait()
        lane_block(2 + n)

    def mod_vec(n):
        return jnp.dot(_bf(scb[0:8, :]), wmb[n], preferred_element_type=F32)[0:8]

    def mods(ns):
        return [jnp.concatenate([modb[n]] * 2, axis=0) for n in ns]

    def prep1(i, grp):
        ra = i * TM + zs[0] * 16
        xs = [qb[pl.ds(pl.multiple_of(ra + 16 * rc, 16), 16), :] for rc in grp]
        return [_stats(x.astype(F32)) for x in xs]

    def prep2(i, grp, st1, x1v, xoff):
        rb = i * TM + zs[1] * 16
        st2 = []
        for rc, (m, rs) in zip(grp, st1):
            sa, ca = mods((0, 1))
            x = qb[pl.ds(pl.multiple_of(rb + 16 * rc, 16), 16), :].astype(F32)
            ry = _mo(i * TM + 16 * rc, 16)
            x1 = x + (((x - m) * rs) * ca + sa) * (
                yb[0, pl.ds(ry, 16), :] + yb[1, pl.ds(ry, 16), :])
            x1v[xoff + 16 * rc:xoff + 16 * rc + 16, :] = x1
            st2.append(_stats(x1))
        return st2

    def prep3(i, grp, st2, hoff, chain):
        rx = i * TM + zs[2] * 16
        for n, (rc, (m, rs)) in enumerate(zip(grp, st2)):
            sb, cb = mods((3, 4))
            x1 = x1r[pl.ds(pl.multiple_of(rx + 16 * rc, 16), 16), :]
            h2 = ((x1 - m) * rs) * cb + sb
            h2r[hoff + 8 * rc:hoff + 8 * rc + 8, :] = _pk(h2.astype(BF))
            if chain == 1:
                qb[S:S + 8, 128 * n:128 * (n + 1)] = h2[8:16, D - 128:D].astype(BF)
            elif chain == 2:
                xh3[zs[3], 8, 1, 8 * n:8 * n + 8, :] = h2[8:16, D - 128:D]

    def prep(i, x1v, xoff):
        for g0 in range(0, TM // 16, LINK):
            grp = range(g0, g0 + LINK)
            st2 = prep2(i, grp, prep1(i, grp), x1v, xoff)
            prep3(i, grp, st2, 0, 1 if g0 + LINK < TM // 16 else 2)

    def w1(f0, f1, mode):
        if mode == 'packed':
            return _bf(w1p[f0 // 2:f1 // 2, :])
        w = w1b[f0:f1, :]
        if mode == 'save':
            w1p[f0 // 2:f1 // 2, :] = _pk(w)
        return w

    def mm1(hoff, gv, goff, rows, f0, f1, mode='packed'):
        h2 = _bf(h2r[hoff:hoff + rows // 2, :])
        if f1 == F:
            st = lax.dot_general(w1(FH, F, mode), h2, NT, preferred_element_type=F32)
            st = _gelu2(st + jnp.concatenate([b1c[...]] * (rows // 128), axis=1))
            gv[goff:goff + rows // 2, FH:F] = _pk(st.T.astype(BF))
            f1 = FH
        if f0 < f1:
            g = lax.dot_general(h2, w1(f0, f1, mode), NT,
                                preferred_element_type=F32) + b1f[0:1, f0:f1]
            gv[goff:goff + rows // 2, f0:f1] = _pk(_gelu2(g).astype(BF))

    def mm2(i, gv, goff, x1v, xoff, lo=0, hi=TM):
        r0 = _mo(i * TM + lo, 16)
        gb = modb[5][0:1]
        o = jnp.dot(_bf(gv[goff + lo // 2:goff + hi // 2, :]), w2b[...],
                    preferred_element_type=F32) + b2f[0:1, :]
        ob[pl.ds(r0, hi - lo), :] = (x1v[xoff + lo:xoff + hi, :] + gb * o).astype(BF)
        o_cp(i, lo, hi).start()

    allg = range(TM // 16)
    q_cp(0).wait()
    q_cp(1).wait()
    stage_a_lane(NL - 1)
    for i in range(4):
        stage_c(2, i, slice(D - 128, D))
    mv = [mod_vec(n) for n in range(3)]
    modb[0] = mv[0] * mv[2]
    modb[1] = (mv[1] + 1.0) * mv[2]
    for i in range(4):
        stage_b(12, 2, i, [0])
    st1a = prep1(0, allg)
    st1b = prep1(1, allg)

    wm_cp(3).wait()
    modb[3] = mod_vec(3)
    st2a = prep2(0, allg, st1a, x1r, 0)

    wm_cp(4).wait()
    modb[4] = mod_vec(4) + 1.0
    prep3(0, allg, st2a, 0, 0)

    w1a_cp.wait()
    mm1(0, gr, 0, TM, 0, F0, 'save')
    prep3(1, allg, prep2(1, allg, st1b, x1r, TM), TH, 0)
    mm1(TH, gr, TH, TM, 0, F0, 'raw')

    w1m_cp.wait()
    unit_c(12, 0)
    mm1(0, gr, 0, 2 * TM, F0, F1, 'save')

    w1b_cp.wait()
    mm1(0, gr, 0, 2 * TM, F1, FH - 128, 'save')
    mm1(0, gr, 0, 2 * TM, FH, F, 'save')
    for r in range(4):
        mm1(r * 64, gr, r * 64, 128, FH - 128, FH, 'save' if r == 0 else 'raw')

    w2_cp.wait()
    wm_cp(5).wait()
    modb[5] = 0.5 * mod_vec(5)

    def step(k, units):
        if isinstance(k, int):
            x1v, xo, gv, go = x1r, (k - 2) * TM, gr, (k - 2) * TH
        else:
            x1v = x1r.at[pl.ds(pl.multiple_of((k - 2) * TM, TM), 3 * TM)]
            gv = gr.at[pl.ds(pl.multiple_of((k - 2) * TH, TH), 3 * TH)]
            xo = go = 0
        mm2(k - 2, gv, go, x1v, xo)
        prep(k, x1v, xo + 2 * TM)
        for a0, lane in units:
            unit_b(a0, lane)
        mm1(0, gv, go + 2 * TH, TM // 2, 0, FH)
        mm1(0, gv, go + 2 * TH, TM, FH, F)
        mm1(TH // 2, gv, go + 2 * TH + TH // 2, TM // 2, 0, FH)
        for a0, lane in units:
            unit_c(a0, lane)

    def body(k, carry):
        q_cp(k).wait()
        step(k, [(12, k - 1), (14, k - 2)])
        return carry

    lax.fori_loop(2, 6, body, 0)
    q_cp(6).wait()
    q_cp(7).wait()
    step(6, [(14, NL - 1)])
    step(7, [])
    mm2(6, gr, 6 * TH, x1r, 6 * TM)
    mm2(7, gr, 7 * TH, x1r, 7 * TM, 0, TM - TAILR)
    mm2(7, gr, 7 * TH, x1r, 7 * TM, TM - TAILR, TM)
    for i in range(NS - 1):
        o_cp(i).wait()
    o_cp(NS - 1, 0, TM - TAILR).wait()
    o_cp(NS - 1, TM - TAILR, TM).wait()


@jax.jit
def pallas_adaLN_cond__ssm_conv_h3__dense_activation_gelu__prompt_kernel(
    A_q: jax.Array,
    A_k: jax.Array,
    A_v: jax.Array,
    A_shift_k: jax.Array,
    A_ssm_k: jax.Array,
    A_ssm_D: jax.Array,
    B_x: jax.Array,
    B_w1: jax.Array,
    B_b1: jax.Array,
    B_w2: jax.Array,
    B_b2: jax.Array,
    c: jax.Array,
    w_mod: jax.Array,
):
    del B_x
    any_spec = pl.BlockSpec(memory_space=pl.ANY)
    scratch = [
        pltpu.VMEM((S + 64, D), BF),
        pltpu.VMEM((S, D), BF),
        pltpu.VMEM((S, D), BF),
        pltpu.VMEM((NB, D, BLK), BF),
        pltpu.VMEM((6, D, D), BF),
        pltpu.VMEM((F, D), BF),
        pltpu.VMEM((F, D), BF),
        pltpu.VMEM((S, D), BF),
        pltpu.VMEM((BLK, 4 * BLK), U32),
        pltpu.VMEM((NL, S + 32, 128), F32),
        pltpu.VMEM((4, 8, D), F32),
        pltpu.VMEM(((NB + 1) * 64, D), U32),
        pltpu.VMEM((NB + 1, D // 2, BLK), U32),
    ] + [pltpu.VMEM((NL, 9, 4, 64, 128), F32)] * 4 + [pltpu.VMEM((4 * BLK, D), U32)] * 4 + [
        pltpu.VMEM((4, 2, 32, D), F32),
        pltpu.VMEM((2, S, D), F32),
        pltpu.VMEM((8, 8, D), F32),
        pltpu.VMEM((TM, D), U32),
        pltpu.VMEM((S, D), F32),
        pltpu.VMEM((S // 2, F), U32),
        pltpu.VMEM((64, 128), F32),
        pltpu.VMEM((F // 2, D), U32),
        pltpu.VMEM((16, F), F32),
        pltpu.VMEM((32, D), F32),
        pltpu.VMEM((32, D), F32),
        pltpu.VMEM((32, D), U32),
        pltpu.VMEM((4, D), BF),
        pltpu.VMEM((D,), BF),
        pltpu.VMEM((F,), BF),
        pltpu.VMEM((D,), BF),
        pltpu.VMEM((1, D), BF),
        pltpu.SMEM((8,), jnp.int32),
        pltpu.SemaphoreType.DMA((3 * NB + 6 + NS + 9,)),
        pltpu.SemaphoreType.DMA((NS + 1,)),
    ]
    return pl.pallas_call(
        _kernel,
        in_specs=[any_spec] * 12,
        out_specs=any_spec,
        out_shape=jax.ShapeDtypeStruct((1, S, D), BF),
        scratch_shapes=scratch,
        compiler_params=pltpu.CompilerParams(vmem_limit_bytes=110 * 1024 * 1024,
                                             disable_semaphore_checks=True),
    )(A_q, A_k, A_v, A_shift_k.T, A_ssm_k, A_ssm_D, B_w1.T, B_b1, B_w2, B_b2, c, w_mod)
```
